```python
import os as _os
_os.environ.setdefault('JAX_PLATFORMS', 'cpu')
import jax
import jax.numpy as jnp

def _softmax(x, axis=-1):
    return jax.nn.softmax(x, axis=axis)

def _gelu(x):
    return jax.nn.gelu(x, approximate=True)

def _silu(x):
    return jax.nn.silu(x)

def _sigmoid(x):
    return jax.nn.sigmoid(x)

def _layernorm(x, axis=-1, eps=1e-05):
    m = jnp.mean(x, axis=axis, keepdims=True)
    v = jnp.var(x, axis=axis, keepdims=True)
    return (x - m) / jnp.sqrt(v + eps)

def _scatter_add(tgt, idx, src, axis=0):
    return tgt.at[idx].add(src)

def _segment_sum(src, seg, n):
    return jax.ops.segment_sum(src, seg, n)

class _Rng:

    def __init__(self, key):
        self._k = key

    def _next(self):
        self._k, sub = jax.random.split(self._k)
        return sub

    def normal(self, shape):
        return jax.random.normal(self._next(), shape, dtype=jnp.bfloat16)

    def randint(self, lo, hi, shape):
        return jax.random.randint(self._next(), shape, lo, hi, dtype=jnp.int32)

    def uniform(self, shape, lo=0.0, hi=1.0):
        return jax.random.uniform(self._next(), shape, jnp.bfloat16, lo, hi)

    def permutation(self, n):
        return jax.random.permutation(self._next(), n)
kernel_name = 'adaLN_cond__softmax_full_mha__mixer_gmlp__prompt'

def setup_inputs():
    _rng = _Rng(jax.random.key(int.from_bytes(__import__("os").urandom(4), "little")))
    _w = lambda a: (lambda t: t.astype(jnp.bfloat16) if jnp.issubdtype(t.dtype, jnp.floating) else t)(jnp.asarray(a))

    def _A_setup():
        B, S, D = (1, 2048, 512)
        return {'x': _w((lambda *s: _rng.normal(s) * 0.05)(B, S, D)), 'wqkv': _w((lambda *s: _rng.normal(s) * 0.05)(D, 3 * D)), 'wo': _w((lambda *s: _rng.normal(s) * 0.05)(D, D))}
    _A_in = _A_setup()

    def _B_setup():
        B, S, D, F = (1, 2048, 512, 1792)
        Fh = F // 2
        return {'x': _w((lambda *s: _rng.normal(s) * 0.05)(B, S, D)), 'w_in': _w((lambda *s: _rng.normal(s) * 0.4)(D, 2 * Fh)), 'w_sp': _w(0.01 * (lambda *s: _rng.normal(s) * 0.4)(S, S)), 'b_sp': _w(1.0 + 0.01 * (lambda *s: _rng.normal(s) * 0.05)(S)), 'w_out': _w((lambda *s: _rng.normal(s) * 0.05)(Fh, D))}
    _B_in = _B_setup()
    return {'A_x': _A_in['x'], 'A_wqkv': _A_in['wqkv'], 'A_wo': _A_in['wo'], 'B_x': _B_in['x'], 'B_w_in': _B_in['w_in'], 'B_w_sp': _B_in['w_sp'], 'B_b_sp': _B_in['b_sp'], 'B_w_out': _B_in['w_out'], 'c': _w((lambda *s: _rng.normal(s) * 0.05)(1, 512) * 8.0), 'w_mod': _w((lambda *s: _rng.normal(s) * 0.05)(512, 6 * 512) * 512 ** (-0.5) * 8.0)}

def reference(A_x, A_wqkv, A_wo, B_x, B_w_in, B_w_sp, B_b_sp, B_w_out, c, w_mod):

    def _A_ref(x, wqkv, wo):
        B, S, D = x.shape
        H = 32
        Dh = D // H
        qkv = (lambda x, *d: x.transpose(*d))((x @ wqkv).reshape(B, S, 3, H, Dh), 2, 0, 3, 1, 4)
        q, k, v = (qkv[0], qkv[1], qkv[2])
        scale = Dh ** (-0.5)
        scores = jnp.einsum('bhqd,bhkd->bhqk', q, k) * scale
        p = _softmax(scores, axis=-1)
        o = jnp.einsum('bhqk,bhkd->bhqd', p, v)
        return (lambda x, *d: x.transpose(*d))(o, 0, 2, 1, 3).reshape(B, S, D) @ wo

    def _B_ref(x, w_in, w_sp, b_sp, w_out):
        B, S, D = x.shape
        F = w_in.shape[-1]
        Fh = F // 2
        z = _gelu(jnp.einsum('bsd,df->bsf', x, w_in))
        z1 = z[..., :Fh].copy()
        z2 = _layernorm(z[..., Fh:], axis=-1)
        g = jnp.einsum('ts,bsf->btf', w_sp, z2) + b_sp[None, :, None]
        return jnp.einsum('bsf,fd->bsd', z1 * g, w_out)
    x = A_x
    mod = (_silu(c) @ w_mod).reshape(c.shape[0], 6, 1, -1)
    sa, ca, ga, sb, cb, gb = (mod[:, 0].copy(), mod[:, 1].copy(), mod[:, 2].copy(), mod[:, 3].copy(), mod[:, 4].copy(), mod[:, 5].copy())
    h = _layernorm(x, axis=-1) * (1 + ca) + sa
    x = x + ga * _A_ref(h, A_wqkv, A_wo)
    h = _layernorm(x, axis=-1) * (1 + cb) + sb
    x = x + gb * _B_ref(h, B_w_in, B_w_sp, B_b_sp, B_w_out)
    return x
```

```python
import jax
import jax.numpy as jnp
import jax.experimental.pallas as pl
import jax.experimental.pallas.tpu as pltpu

S = 2048
D = 512
H = 32
DH = 16
FH = 896
EPS = 1e-5
LOG2E = 1.4426950408889634
QSCALE = (DH ** -0.5) * LOG2E

TQ = 512
CK = 128
NC = S // CK
NQ = S // TQ
T = H * NQ
RB = 512
NRB = S // RB

BF = jnp.bfloat16
F32 = jnp.float32


def _pk(x):
    return pltpu.bitcast(x, jnp.uint32)


def _upk(x):
    return pltpu.bitcast(x, BF)


def _ln(x):
    m = jnp.mean(x, axis=-1, keepdims=True)
    xc = x - m
    v = jnp.mean(xc * xc, axis=-1, keepdims=True)
    return xc * jax.lax.rsqrt(v + EPS)


def _gelu(x):
    c0 = 0.7978845608028654
    inner = x * (c0 + (c0 * 0.044715) * (x * x))
    hx = 0.5 * x
    return hx + hx * jnp.tanh(inner)


def _kernel(x_hbm, wqkv_hbm, wo_hbm, win_hbm, wsp_hbm, bsp_ref, wout_hbm, c_ref, wmod_hbm,
            out_hbm,
            x_v, wqkv_v, wo_v, win_v, wsp_v, wout_v, wmod_v, mod_v,
            k_s, qt_s, vt_s, s0, s1, ot_s, x1_s, z1_s, z2_s, out_v, sems):
    cp_wmod = pltpu.make_async_copy(wmod_hbm, wmod_v, sems.at[0])
    cp_x = pltpu.make_async_copy(x_hbm.at[0], x_v, sems.at[1])
    cp_wqkv = pltpu.make_async_copy(wqkv_hbm, wqkv_v, sems.at[2])
    cp_wo = pltpu.make_async_copy(wo_hbm, wo_v, sems.at[3])
    cp_win = pltpu.make_async_copy(win_hbm, win_v, sems.at[4])
    cp_wsp = pltpu.make_async_copy(wsp_hbm, wsp_v, sems.at[5])
    cp_wout = pltpu.make_async_copy(wout_hbm, wout_v, sems.at[6])
    cp_wmod.start()
    cp_x.start()
    cp_wqkv.start()

    c = c_ref[...].astype(F32)
    sc = (c * jax.nn.sigmoid(c)).astype(BF)
    sc = jnp.broadcast_to(sc, (16, D))
    cp_wmod.wait()
    mod_v[...] = jnp.dot(sc, wmod_v[...], preferred_element_type=F32)[:8]

    def mod_row(j):
        return mod_v[0:1, j * D:(j + 1) * D]

    cp_x.wait()
    cp_wqkv.wait()
    cp_wo.start()
    cp_win.start()
    cp_wsp.start()
    cp_wout.start()

    def p1_body(i, carry):
        r0 = pl.multiple_of(i * RB, RB)
        x = x_v[pl.ds(r0, RB), :].astype(F32)
        h = (_ln(x) * (1.0 + mod_row(1)) + mod_row(0)).astype(BF)
        qkv = jnp.dot(h, wqkv_v[...], preferred_element_type=F32)
        q = (qkv[:, :D] * QSCALE).astype(BF)
        k = qkv[:, D:2 * D].astype(BF)
        v = qkv[:, 2 * D:].astype(BF)
        qt_s[:, pl.ds(r0, RB)] = _pk(q.T)
        vt_s[:, pl.ds(r0, RB)] = _pk(v.T)
        r0h = pl.multiple_of(i * (RB // 2), RB // 2)
        for g in range(4):
            k_s[g, pl.ds(r0h, RB // 2), :] = _pk(k[:, g * 128:(g + 1) * 128])
        return carry

    jax.lax.fori_loop(0, NRB, p1_body, 0)

    def wq(t):
        t = jnp.minimum(t, T - 1)
        h = t % H
        qb = t // H
        q = qt_s[pl.ds(pl.multiple_of(h * 8, 8), 8), pl.ds(pl.multiple_of(qb * TQ, TQ), TQ)]
        hp = h % 8
        blocks = [jnp.where(hp == j, q, jnp.zeros_like(q)) for j in range(8)]
        return _upk(jnp.concatenate(blocks, axis=0)), h // 8

    def a_chunk(w, g, ck, sbuf, m):
        kc = _upk(k_s[g, pl.ds(ck * CK // 2, CK // 2), :])
        st = jnp.dot(kc, w, preferred_element_type=F32)
        sbuf[pl.ds(ck * CK, CK), :] = st
        for j in range(CK // 8):
            m = jnp.maximum(m, st[8 * j:8 * j + 8])
        return m

    def b_chunk(h, ck, sbuf, mb, l, acc):
        s = sbuf[pl.ds(ck * CK, CK), :]
        p = jnp.exp2(s.reshape(CK // 8, 8, TQ) - mb[None]).reshape(CK, TQ)
        for j in reversed(range(CK // 16)):
            l = l + (p[16 * j:16 * j + 8] + p[16 * j + 8:16 * j + 16])
        vc = _upk(vt_s[pl.ds(pl.multiple_of(h * 8, 8), 8), pl.ds(ck * CK, CK)])
        acc = acc + jnp.dot(vc, p.astype(BF), preferred_element_type=F32)
        return l, acc

    neg = jnp.full((8, TQ), -jnp.inf, F32)

    def fin(t, l, acc):
        h = t % H
        qb = t // H
        lsum = l.sum(axis=0, keepdims=True)
        o = acc * (1.0 / lsum)
        ot_s[pl.ds(pl.multiple_of(h * 8, 8), 8), pl.ds(pl.multiple_of(qb * TQ, TQ), TQ)] = (
            _pk(o.astype(BF)))

    FM = 2

    def half(t, m_cur, s_cur, s_next):
        never = t < 0
        w, g = wq(t + 1)
        mb = jnp.broadcast_to(m_cur.max(axis=0, keepdims=True), (8, TQ))
        m = neg
        l = jnp.zeros((8, TQ), F32)
        acc = jnp.zeros((16, TQ), F32)
        mh = []
        for c_ in range(NC):
            m = a_chunk(w, g, c_, s_next, m)
            mh.append(m)
            mbc = mb
            if c_ - FM >= 0:
                mbc = jnp.where(never, mh[c_ - FM], mb)
            l, acc = b_chunk(t % H, c_, s_cur, mbc, l, acc)
        fin(t, l, acc)
        return m

    w0, g0 = wq(0)
    m0 = neg
    for c_ in range(NC):
        m0 = a_chunk(w0, g0, c_, s0, m0)

    def p2_body(i, m):
        m = half(2 * i, m, s0, s1)
        m = half(2 * i + 1, m, s1, s0)
        return m

    jax.lax.fori_loop(0, T // 2, p2_body, m0)

    cp_wo.wait()
    cp_win.wait()

    def p3_body(i, carry):
        r0 = pl.multiple_of(i * RB, RB)
        ot = _upk(ot_s[:, pl.ds(r0, RB)])
        attn = jnp.dot(ot.T, wo_v[...], preferred_element_type=F32)
        x1 = x_v[pl.ds(r0, RB), :].astype(F32) + mod_row(2) * attn
        x1_s[pl.ds(r0, RB), :] = x1
        h2 = (_ln(x1) * (1.0 + mod_row(4)) + mod_row(3)).astype(BF)
        z = _gelu(jnp.dot(h2, win_v[...], preferred_element_type=F32))
        z1_s[pl.ds(r0, RB), :] = z[:, :FH]
        r0h = pl.multiple_of(i * (RB // 2), RB // 2)
        z2_s[pl.ds(r0h, RB // 2), :] = _pk(_ln(z[:, FH:]).astype(BF))
        return carry

    jax.lax.fori_loop(0, NRB, p3_body, 0)

    cp_wsp.wait()
    cp_wout.wait()

    def out_copy(i):
        r0 = i * RB
        return pltpu.make_async_copy(out_v.at[pl.ds(r0, RB), :],
                                     out_hbm.at[0, pl.ds(r0, RB), :], sems.at[7 + i])

    for i in range(NRB):
        r0 = i * RB
        gsp = jnp.dot(wsp_v[pl.ds(r0, RB), :], _upk(z2_s[...]), preferred_element_type=F32)
        brow = bsp_ref[:, pl.ds(r0, RB)].astype(F32)
        bcol = jnp.broadcast_to(brow, (128, RB)).T
        bfull = jnp.concatenate([bcol] * (FH // 128), axis=1)
        u = (z1_s[pl.ds(r0, RB), :] * (gsp + bfull)).astype(BF)
        y = jnp.dot(u, wout_v[...], preferred_element_type=F32)
        out_v[pl.ds(r0, RB), :] = (x1_s[pl.ds(r0, RB), :] + mod_row(5) * y).astype(BF)
        out_copy(i).start()
    for i in range(NRB):
        out_copy(i).wait()


@jax.jit
def pallas_adaLN_cond__softmax_full_mha__mixer_gmlp__prompt_kernel(
    A_x: jax.Array,
    A_wqkv: jax.Array,
    A_wo: jax.Array,
    B_x: jax.Array,
    B_w_in: jax.Array,
    B_w_sp: jax.Array,
    B_b_sp: jax.Array,
    B_w_out: jax.Array,
    c: jax.Array,
    w_mod: jax.Array,
):
    del B_x
    any_spec = pl.BlockSpec(memory_space=pl.ANY)
    vmem_spec = pl.BlockSpec(memory_space=pltpu.VMEM)
    u32 = jnp.uint32
    scratch = [
        pltpu.VMEM((S, D), BF),
        pltpu.VMEM((D, 3 * D), BF),
        pltpu.VMEM((D, D), BF),
        pltpu.VMEM((D, 2 * FH), BF),
        pltpu.VMEM((S, S), BF),
        pltpu.VMEM((FH, D), BF),
        pltpu.VMEM((D, 6 * D), BF),
        pltpu.VMEM((8, 6 * D), F32),
        pltpu.VMEM((4, S // 2, 128), u32),
        pltpu.VMEM((D // 2, S), u32),
        pltpu.VMEM((D // 2, S), u32),
        pltpu.VMEM((S, TQ), F32),
        pltpu.VMEM((S, TQ), F32),
        pltpu.VMEM((D // 2, S), u32),
        pltpu.VMEM((S, D), F32),
        pltpu.VMEM((S, FH), F32),
        pltpu.VMEM((S // 2, FH), u32),
        pltpu.VMEM((S, D), BF),
        pltpu.SemaphoreType.DMA((7 + NRB,)),
    ]
    return pl.pallas_call(
        _kernel,
        out_shape=jax.ShapeDtypeStruct((1, S, D), BF),
        in_specs=[any_spec, any_spec, any_spec, any_spec, any_spec, vmem_spec, any_spec,
                  vmem_spec, any_spec],
        out_specs=any_spec,
        scratch_shapes=scratch,
        compiler_params=pltpu.CompilerParams(vmem_limit_bytes=100 * 1024 * 1024),
    )(A_x, A_wqkv, A_wo, B_w_in, B_w_sp, B_b_sp.reshape(1, S), B_w_out, c, w_mod)
```

```python
import jax
import jax.numpy as jnp
import jax.experimental.pallas as pl
import jax.experimental.pallas.tpu as pltpu

S = 2048; D = 512; H = 32; DH = 16; FH = 896
EPS = 1e-5
LOG2E = 1.4426950408889634
QSCALE = (DH ** -0.5) * LOG2E

TQ = 512
CK = 128
NC = S // CK
NQ = S // TQ
T = H * NQ
RB1 = 512
RB3 = 512
RB4 = 512
SPI = 8
FM = 3
G = 3
KSW = 2
PH = 15
PEEL = 8
Z1P3 = 0
NT3 = 0
HOOK = 2
OT = 128

BF = jnp.bfloat16
F32 = jnp.float32


def _pk(x):
    return pltpu.bitcast(x, jnp.uint32)


def _upk(x):
    return pltpu.bitcast(x, BF)


def _mo(x, n):
    return x if isinstance(x, int) else pl.multiple_of(x, n)


def _ln(x):
    m = jnp.mean(x, axis=-1, keepdims=True)
    xc = x - m
    v = jnp.mean(xc * xc, axis=-1, keepdims=True)
    return xc * jax.lax.rsqrt(v + EPS)


def _gelu(x):
    c0 = 0.7978845608028654
    inner = x * (c0 + (c0 * 0.044715) * (x * x))
    hx = 0.5 * x
    return hx + hx * jnp.tanh(inner)


def _dot_nt(a, w_ref, c0, n, tile):
    return [jnp.dot(a, w_ref[:, c0 + j:c0 + j + tile], preferred_element_type=F32)
            for j in range(0, n, tile)]


def _out_blocks():
    blocks = [(i * RB4, RB4) for i in range(S // RB4 - 1)]
    r0 = S - RB4
    blocks += [(r0 + j * OT, OT) for j in range(RB4 // OT)]
    return blocks


def _kernel(x_hbm, wqkv_hbm, wo_hbm, win_hbm, wsp_hbm, bsp_hbm, wout_hbm, c_hbm, wmod_hbm,
            out_hbm,
            x_v, wqkv_v, wo_v, win_v, wsp_v, wout_v, wmod_v, c_v, bsp_v, mod_v,
            k_s, qt_s, vt_s, s0, s1, ot_s, x1_s, h2_s, z2_s, z1_s, out_v, z_s, sems, osems):
    z_s[0] = 0
    def cols(src, dst, c0, n, sem):
        return pltpu.make_async_copy(src.at[:, pl.ds(c0, n)], dst.at[:, pl.ds(c0, n)], sem)

    def xrows(r0, n, sem):
        return pltpu.make_async_copy(x_hbm.at[0, pl.ds(r0, n), :], x_v.at[pl.ds(r0, n), :], sem)

    NJ = 4
    JW = D // NJ
    cp_c = pltpu.make_async_copy(c_hbm, c_v, sems.at[0])
    cp_x0 = xrows(0, RB1, sems.at[1])
    cp_ms = [cols(wmod_hbm, wmod_v, j * JW, JW, sems.at[14 + j]) for j in range(NJ)]
    cp_mc = [cols(wmod_hbm, wmod_v, D + j * JW, JW, sems.at[18 + j]) for j in range(NJ)]
    cp_w = [pltpu.make_async_copy(wqkv_hbm.at[pl.ds(j * JW, JW), :], wqkv_v.at[pl.ds(j * JW, JW), :],
                                  sems.at[2 + j]) for j in range(NJ)]
    cp_x1 = xrows(RB1, RB1, sems.at[6])
    cp_x23 = xrows(2 * RB1, 2 * RB1, sems.at[7])
    cp_wmod_b = cols(wmod_hbm, wmod_v, 2 * D, 4 * D, sems.at[8])
    cp_wo = pltpu.make_async_copy(wo_hbm, wo_v, sems.at[9])
    cp_win = pltpu.make_async_copy(win_hbm, win_v, sems.at[10])
    cp_wsp = pltpu.make_async_copy(wsp_hbm, wsp_v, sems.at[11])
    cp_wout = pltpu.make_async_copy(wout_hbm, wout_v, sems.at[12])
    cp_bsp = pltpu.make_async_copy(bsp_hbm, bsp_v, sems.at[13])
    order = [cp_c, cp_x0, cp_ms[0], cp_mc[0]]
    for j in range(NJ):
        if j + 1 < NJ:
            order += [cp_ms[j + 1], cp_mc[j + 1]]
        order.append(cp_w[j])
    order += [cp_x1, cp_x23, cp_wmod_b, cp_wo, cp_win, cp_wsp, cp_wout, cp_bsp]
    for cp in order:
        cp.start()

    cp_c.wait()
    cp_x0.wait()
    c = c_v[...].astype(F32)
    sc = (c * jax.nn.sigmoid(c)).astype(BF)
    sc = jnp.broadcast_to(sc, (16, D))

    def norm1(i):
        return _ln(x_v[pl.ds(i * RB1, RB1), :].astype(F32))

    def mod_row(j):
        return mod_v[0:1, j * D:(j + 1) * D]

    def modulate1(n):
        return (n * (1.0 + mod_row(1)) + mod_row(0)).astype(BF)

    n0 = norm1(0)

    def h0_piece(j):
        for c0 in (j * JW, D + j * JW):
            mod_v[:, c0:c0 + JW] = jnp.dot(sc, wmod_v[:, c0:c0 + JW], preferred_element_type=F32)[:8]
        sa = mod_v[0:1, j * JW:(j + 1) * JW]
        ca = mod_v[0:1, D + j * JW:D + (j + 1) * JW]
        return (n0[:, j * JW:(j + 1) * JW] * (1.0 + ca) + sa).astype(BF)

    cp_ms[0].wait()
    cp_mc[0].wait()
    hj = h0_piece(0)
    qkv0 = None
    for j in range(NJ):
        if j + 1 < NJ:
            cp_ms[j + 1].wait()
            cp_mc[j + 1].wait()
        else:
            cp_x1.wait()
        cp_w[j].wait()
        part = jnp.dot(hj, wqkv_v[j * JW:(j + 1) * JW, :], preferred_element_type=F32)
        qkv0 = part if qkv0 is None else qkv0 + part
        if j + 1 < NJ:
            hj = h0_piece(j + 1)
        else:
            h = modulate1(norm1(1))

    def proj_k(i, h):
        k = qkv0[:, D:2 * D] if i == 0 else jnp.dot(h, wqkv_v[:, D:2 * D], preferred_element_type=F32)
        k = k.astype(BF)
        for g in range(4):
            k_s[8 * g, pl.ds(i * RB1 // 2, RB1 // 2), :] = _pk(k[:, g * 128:(g + 1) * 128])

    def rot_k(i):
        for g in range(4):
            kg = k_s[8 * g, pl.ds(i * RB1 // 2, RB1 // 2), :]
            for j in range(1, 8):
                k_s[8 * g + j, pl.ds(i * RB1 // 2, RB1 // 2), :] = pltpu.roll(kg, 128 - 16 * j, axis=1)

    def proj_q(i, h):
        q = qkv0[:, :D] if i == 0 else jnp.dot(h, wqkv_v[:, :D], preferred_element_type=F32)
        q = (q * QSCALE).astype(BF)
        qt_s[:, pl.ds(i * RB1, RB1)] = _pk(q.T)

    def proj_v(i, h):
        v = qkv0[:, 2 * D:] if i == 0 else jnp.dot(h, wqkv_v[:, 2 * D:], preferred_element_type=F32)
        v = v.astype(BF)
        vt_s[:, pl.ds(i * RB1, RB1)] = _pk(v.T)

    cp_x23.wait()
    proj_k(0, None)
    rot_k(0)
    proj_q(0, None)
    proj_v(0, None)
    for i in range(1, S // RB1):
        hn = modulate1(norm1(i + 1)) if i + 1 < S // RB1 else None
        proj_k(i, h)
        rot_k(i)
        proj_v(i, h)
        proj_q(i, h)
        h = hn

    def hq(t):
        return t // NQ, t % NQ

    def wq(t):
        h, qb = hq(t)
        q = qt_s[pl.ds(_mo(h * 8, 8), 8), pl.ds(_mo(qb * TQ, TQ), TQ)]
        return _upk(q), h

    def a_chunk(w, h, c_, sbuf, m):
        kc = _upk(k_s[h, pl.ds(c_ * CK // 2, CK // 2), :])
        st = jnp.dot(kc[:, :DH], w, preferred_element_type=F32)
        sbuf[pl.ds(c_ * CK, CK), :] = st
        for j in range(CK // 8):
            m = jnp.maximum(m, st[8 * j:8 * j + 8])
        return m

    def b_chunk(t, ck, sbuf, mb, l, acc):
        h, _ = hq(t)
        s = sbuf[pl.ds(ck * CK, CK), :]
        p = jnp.exp2(s.reshape(CK // 8, 8, TQ) - mb[None]).reshape(CK, TQ)
        for j in reversed(range(CK // 16)):
            l = l + (p[16 * j:16 * j + 8] + p[16 * j + 8:16 * j + 16])
        vc = _upk(vt_s[pl.ds(_mo(h * 8, 8), 8), pl.ds(ck * CK, CK)])
        acc = acc + jnp.dot(vc, p.astype(BF), preferred_element_type=F32)
        return l, acc

    neg = jnp.full((8, TQ), -jnp.inf, F32)
    zl = jnp.zeros((8, TQ), F32)
    za = jnp.zeros((16, TQ), F32)

    def fin(t, l, acc):
        h, qb = hq(t)
        lsum = l.sum(axis=0, keepdims=True)
        o = acc * (1.0 / lsum)
        ot_s[pl.ds(_mo(h * 8, 8), 8), pl.ds(_mo(qb * TQ, TQ), TQ)] = (
            _pk(o.astype(BF)))

    def red_m(m):
        return jnp.broadcast_to(m.max(axis=0, keepdims=True), (8, TQ))

    bufs = (s0, s1)

    def run_steps(t0, nsteps, state, never, last=False, hooks=None):
        m_pre, m_fin = state
        mh_prev = None
        for s_ in range(nsteps):
            t = t0 + s_
            s_cur, s_next = bufs[s_ % 2], bufs[1 - s_ % 2]
            do_a = not (last and s_ == nsteps - 1)
            if do_a:
                w, hn = wq(t + 1)
            m = neg
            mh = []
            l, acc = zl, za
            mb = red_m(m_pre)
            for c_ in range(NC):
                if do_a:
                    m = a_chunk(w, hn, c_, s_next, m)
                if hooks is not None and s_ in hooks:
                    hooks[s_](c_)
                mh.append(m)
                if c_ == KSW:
                    mb2 = red_m(m_fin)
                    alpha = jnp.exp2(mb - mb2)
                    l = l * alpha
                    acc = (acc.reshape(2, 8, TQ) * alpha[None]).reshape(16, TQ)
                    mb = mb2
                mbc = mb
                if c_ - FM >= 0:
                    if do_a:
                        mbc = jnp.where(never, mh[c_ - FM], mb)
                elif mh_prev is not None:
                    mbc = jnp.where(never, mh_prev[NC + c_ - FM], mb)
                l, acc = b_chunk(t, c_, s_cur, mbc, l, acc)
            fin(t, l, acc)
            m_pre, m_fin = mh[NC - 1 - G], m
            mh_prev = mh
        return m_pre, m_fin

    if PH & 2:
        w0, h0 = wq(0)
        m0 = neg
        for c_ in range(NC):
            m0 = a_chunk(w0, h0, c_, s0, m0)

        def p2_body(i, state):
            t0 = i * SPI
            return run_steps(t0, SPI, state, t0 < 0)

        st = jax.lax.fori_loop(0, ((T - PEEL) // SPI), p2_body, (m0, m0))

    cp_wmod_b.wait()
    cp_wo.wait()
    cp_win.wait()
    cp_wsp.wait()
    cp_wout.wait()
    cp_bsp.wait()
    def mod_piece(c_):
        c0 = 2 * D + c_ * 128
        mod_v[:, c0:c0 + 128] = jnp.dot(sc, wmod_v[:, c0:c0 + 128], preferred_element_type=F32)[:8]

    attn0 = []
    PR = RB3 * HOOK // NC
    o0_box = []

    def wo_piece(c_):
        if not o0_box:
            o0_box.append(_upk(ot_s[:, pl.ds(0, RB3 * HOOK)]).T)
        attn0.append(jnp.dot(o0_box[0][c_ * PR:(c_ + 1) * PR], wo_v[...], preferred_element_type=F32))

    hooks = {0: mod_piece}
    if HOOK:
        hooks[PEEL - 1] = wo_piece
    run_steps(T - PEEL, PEEL, st, z_s[0] != 0, last=True, hooks=hooks)
    if HOOK:
        attn0 = jnp.concatenate(attn0, axis=0)

    def p3a(i):
        r0 = i * RB3
        if i >= HOOK:
            ot = _upk(ot_s[:, pl.ds(r0, RB3)])
        if i < HOOK:
            attn = attn0[r0:r0 + RB3]
        elif NT3:
            attn = jnp.concatenate(_dot_nt(ot.T, wo_v, 0, D, NT3), axis=1)
        else:
            attn = jnp.dot(ot.T, wo_v[...], preferred_element_type=F32)
        x1 = x_v[pl.ds(r0, RB3), :].astype(F32) + mod_row(2) * attn
        x1_s[pl.ds(r0, RB3), :] = x1
        h2 = (_ln(x1) * (1.0 + mod_row(4)) + mod_row(3)).astype(BF)
        h2_s[pl.ds(r0 // 2, RB3 // 2), :] = _pk(h2)
        return h2

    def p3b(i, h2):
        r0 = i * RB3
        if NT3:
            z2 = jnp.concatenate([_gelu(z) for z in _dot_nt(h2, win_v, FH, FH, NT3)], axis=1)
        else:
            z2 = _gelu(jnp.dot(h2, win_v[:, FH:], preferred_element_type=F32))
        z2_s[pl.ds(r0 // 2, RB3 // 2), :] = _pk(_ln(z2).astype(BF))
        if i < Z1P3:
            z1_s[pl.ds(r0, RB3), :] = jnp.dot(h2, win_v[:, :FH], preferred_element_type=F32)

    if PH & 4:
        N3 = S // RB3
        P3D = 3
        h2s = {}
        for i in range(min(P3D, N3)):
            h2s[i] = p3a(i)
        for i in range(N3):
            if i + P3D < N3:
                h2s[i + P3D] = p3a(i + P3D)
            p3b(i, h2s.pop(i))

    oblocks = _out_blocks()

    def out_copy(j):
        r0, n = oblocks[j]
        return pltpu.make_async_copy(out_v.at[pl.ds(r0, n), :],
                                     out_hbm.at[0, pl.ds(r0, n), :], osems.at[j])

    brow_all = bsp_v[...].reshape(1, S).astype(F32)
    j = 0
    for i in range(S // RB4):
        r0 = i * RB4
        if PH & 8:
            if r0 < Z1P3 * RB3:
                z1 = _gelu(z1_s[pl.ds(r0, RB4), :])
            else:
                h2 = _upk(h2_s[pl.ds(r0 // 2, RB4 // 2), :])
                z1 = _gelu(jnp.dot(h2, win_v[:, :FH], preferred_element_type=F32))
            gsp = jnp.dot(wsp_v[pl.ds(r0, RB4), :], _upk(z2_s[...]), preferred_element_type=F32)
            brow = brow_all[:, r0:r0 + RB4]
            bcol = jnp.broadcast_to(brow, (128, RB4)).T
            bfull = jnp.concatenate([bcol] * (FH // 128), axis=1)
            u = (z1 * (gsp + bfull)).astype(BF)
        while j < len(oblocks) and oblocks[j][0] < r0 + RB4:
            o0, n = oblocks[j]
            if PH & 8:
                y = jnp.dot(u[o0 - r0:o0 - r0 + n], wout_v[...], preferred_element_type=F32)
                out_v[pl.ds(o0, n), :] = (x1_s[pl.ds(o0, n), :] + mod_row(5) * y).astype(BF)
            out_copy(j).start()
            j += 1
    for j in range(len(oblocks)):
        out_copy(j).wait()


@jax.jit
def pallas_adaLN_cond__softmax_full_mha__mixer_gmlp__prompt_kernel(
    A_x, A_wqkv, A_wo, B_x, B_w_in, B_w_sp, B_b_sp, B_w_out, c, w_mod):
    del B_x
    any_spec = pl.BlockSpec(memory_space=pl.ANY)
    u32 = jnp.uint32
    scratch = [
        pltpu.VMEM((S, D), BF), pltpu.VMEM((D, 3 * D), BF), pltpu.VMEM((D, D), BF),
        pltpu.VMEM((D, 2 * FH), BF), pltpu.VMEM((S, S), BF), pltpu.VMEM((FH, D), BF),
        pltpu.VMEM((D, 6 * D), BF), pltpu.VMEM((1, D), BF), pltpu.VMEM((S,), BF),
        pltpu.VMEM((8, 6 * D), F32),
        pltpu.VMEM((H, S // 2, 128), u32), pltpu.VMEM((D // 2, S), u32), pltpu.VMEM((D // 2, S), u32),
        pltpu.VMEM((S, TQ), F32), pltpu.VMEM((S, TQ), F32), pltpu.VMEM((D // 2, S), u32),
        pltpu.VMEM((S, D), F32), pltpu.VMEM((S // 2, D), u32), pltpu.VMEM((S // 2, FH), u32),
        pltpu.VMEM((S, FH), F32),
        pltpu.VMEM((S, D), BF),
        pltpu.SMEM((1,), jnp.int32),
        pltpu.SemaphoreType.DMA((22,)),
        pltpu.SemaphoreType.DMA((len(_out_blocks()),)),
    ]
    return pl.pallas_call(
        _kernel,
        out_shape=jax.ShapeDtypeStruct((1, S, D), BF),
        in_specs=[any_spec] * 9,
        out_specs=any_spec,
        scratch_shapes=scratch,
        compiler_params=pltpu.CompilerParams(vmem_limit_bytes=100 * 1024 * 1024),
    )(A_x, A_wqkv, A_wo, B_w_in, B_w_sp, B_b_sp, B_w_out, c, w_mod)
```

```python
import jax
import jax.numpy as jnp
import jax.experimental.pallas as pl
import jax.experimental.pallas.tpu as pltpu

S = 2048; D = 512; H = 32; DH = 16; FH = 896
EPS = 1e-5
LOG2E = 1.4426950408889634
QSCALE = (DH ** -0.5) * LOG2E

TQ = 512
CK = 128
NC = S // CK
NQ = S // TQ
T = H * NQ
RB1 = 512
RB3 = 512
RB4 = 512
SPI = 8
FM = 3
G = 3
KSW = 2
PH = 15
PEEL = 8
Z1P3 = 0
NT3 = 0
HOOK = 2
NG = 8
NV = 16 * NG
NVP = 128
KM = S - NV
FOFF = 0
KFD = 8
NOQB = 0
TD = 3
XS = 3
DMAJ = 1
NP = 2
CHAIN = 1
KTOK = 1
NOKB = 0
OT = 128

BF = jnp.bfloat16
F32 = jnp.float32


def _pk(x):
    return pltpu.bitcast(x, jnp.uint32)


def _upk(x):
    return pltpu.bitcast(x, BF)


def _mo(x, n):
    return x if isinstance(x, int) else pl.multiple_of(x, n)


def _ln(x):
    m = jnp.mean(x, axis=-1, keepdims=True)
    xc = x - m
    v = jnp.mean(xc * xc, axis=-1, keepdims=True)
    return xc * jax.lax.rsqrt(v + EPS)


def _gelu(x):
    c0 = 0.7978845608028654
    inner = x * (c0 + (c0 * 0.044715) * (x * x))
    hx = 0.5 * x
    return hx + hx * jnp.tanh(inner)


def _dot_nt(a, w_ref, c0, n, tile):
    return [jnp.dot(a, w_ref[:, c0 + j:c0 + j + tile], preferred_element_type=F32)
            for j in range(0, n, tile)]


def _out_blocks():
    blocks = [(i * RB4, RB4) for i in range(S // RB4 - 1)]
    r0 = S - RB4
    blocks += [(r0 + j * OT, OT) for j in range(RB4 // OT)]
    return blocks


def _kernel(x_hbm, wqkv_hbm, wo_hbm, win_hbm, wsp_hbm, bsp_hbm, wout_hbm, c_hbm, wmod_hbm,
            out_hbm,
            x_v, wqkv_v, wo_v, win_v, wsp_v, wout_v, wmod_v, c_v, bsp_v, mod_v,
            k_s, qt_s, vt_s, kt_s, kb0, kb1, qb_s, acc_s, l_s, mb_s, s0, s1, ot_s, x1_s, h2_s, z2_s, z1_s, q0_s, out_v, z_s, sems, osems):
    z_s[0] = 0
    def cols(src, dst, c0, n, sem):
        return pltpu.make_async_copy(src.at[:, pl.ds(c0, n)], dst.at[:, pl.ds(c0, n)], sem)

    def xrows(r0, n, sem):
        return pltpu.make_async_copy(x_hbm.at[0, pl.ds(r0, n), :], x_v.at[pl.ds(r0, n), :], sem)

    NJ = 4
    JW = D // NJ
    cp_c = pltpu.make_async_copy(c_hbm, c_v, sems.at[0])
    cp_x0 = xrows(0, RB1, sems.at[1])
    cp_ms = [cols(wmod_hbm, wmod_v, j * JW, JW, sems.at[14 + j]) for j in range(NJ)]
    cp_mc = [cols(wmod_hbm, wmod_v, D + j * JW, JW, sems.at[18 + j]) for j in range(NJ)]
    cp_w = [pltpu.make_async_copy(wqkv_hbm.at[pl.ds(j * JW, JW), :], wqkv_v.at[pl.ds(j * JW, JW), :],
                                  sems.at[2 + j]) for j in range(NJ)]
    cp_x1 = xrows(RB1, RB1, sems.at[6])
    cp_x23 = xrows(2 * RB1, 2 * RB1, sems.at[7])
    cp_wmod_b = cols(wmod_hbm, wmod_v, 2 * D, 4 * D, sems.at[8])
    cp_wo = pltpu.make_async_copy(wo_hbm, wo_v, sems.at[9])
    cp_win = pltpu.make_async_copy(win_hbm, win_v, sems.at[10])
    cp_wsp = pltpu.make_async_copy(wsp_hbm, wsp_v, sems.at[11])
    cp_wout = pltpu.make_async_copy(wout_hbm, wout_v, sems.at[12])
    cp_bsp = pltpu.make_async_copy(bsp_hbm, bsp_v, sems.at[13])
    order = [cp_c, cp_x0, cp_ms[0], cp_mc[0]]
    for j in range(NJ):
        if j + 1 < NJ:
            order += [cp_ms[j + 1], cp_mc[j + 1]]
        order.append(cp_w[j])
    order += [cp_x1, cp_x23, cp_wmod_b, cp_wo, cp_win, cp_wsp, cp_wout, cp_bsp]
    for cp in order:
        cp.start()

    cp_c.wait()
    cp_x0.wait()
    c = c_v[...].astype(F32)
    sc = (c * jax.nn.sigmoid(c)).astype(BF)
    sc = jnp.broadcast_to(sc, (16, D))

    def norm1(i):
        return _ln(x_v[pl.ds(i * RB1, RB1), :].astype(F32))

    def mod_row(j):
        return mod_v[0:1, j * D:(j + 1) * D]

    def modulate1(n):
        return (n * (1.0 + mod_row(1)) + mod_row(0)).astype(BF)

    n0 = norm1(0)

    def h0_piece(j):
        for c0 in (j * JW, D + j * JW):
            mod_v[:, c0:c0 + JW] = jnp.dot(sc, wmod_v[:, c0:c0 + JW], preferred_element_type=F32)[:8]
        sa = mod_v[0:1, j * JW:(j + 1) * JW]
        ca = mod_v[0:1, D + j * JW:D + (j + 1) * JW]
        return (n0[:, j * JW:(j + 1) * JW] * (1.0 + ca) + sa).astype(BF)

    cp_ms[0].wait()
    cp_mc[0].wait()
    hj = h0_piece(0)
    qkv0 = None
    for j in range(NJ):
        if j + 1 < NJ:
            cp_ms[j + 1].wait()
            cp_mc[j + 1].wait()
        else:
            cp_x1.wait()
        cp_w[j].wait()
        part = jnp.dot(hj, wqkv_v[j * JW:(j + 1) * JW, :], preferred_element_type=F32)
        if j == 0:
            q0_s[...] = part
        elif j + 1 < NJ:
            q0_s[...] = q0_s[...] + part
        else:
            qkv0 = q0_s[...] + part
        if j + 1 < NJ:
            hj = h0_piece(j + 1)
        else:
            h = modulate1(norm1(1))

    def proj_k(i, h):
        k = qkv0[:, D:2 * D] if i == 0 else jnp.dot(h, wqkv_v[:, D:2 * D], preferred_element_type=F32)
        k = k.astype(BF)
        for g in range(4):
            k_s[8 * g, pl.ds(i * RB1 // 2, RB1 // 2), :] = _pk(k[:, g * 128:(g + 1) * 128])
        if i == S // RB1 - 1:
            kt_s[...] = _pk(k[RB1 - NVP:].T)

    def rot_k(i):
        for g in range(4):
            kg = k_s[8 * g, pl.ds(i * RB1 // 2, RB1 // 2), :]
            for j in range(1, 8):
                k_s[8 * g + j, pl.ds(i * RB1 // 2, RB1 // 2), :] = pltpu.roll(kg, 128 - 16 * j, axis=1)

    def proj_q(i, h):
        q = qkv0[:, :D] if i == 0 else jnp.dot(h, wqkv_v[:, :D], preferred_element_type=F32)
        q = (q * QSCALE).astype(BF)
        qt_s[:, pl.ds(i * RB1, RB1)] = _pk(q.T)

    def proj_v(i, h):
        v = qkv0[:, 2 * D:] if i == 0 else jnp.dot(h, wqkv_v[:, 2 * D:], preferred_element_type=F32)
        v = v.astype(BF)
        vt_s[:, pl.ds(i * RB1, RB1)] = _pk(v.T)

    cp_x23.wait()
    proj_k(0, None)
    rot_k(0)
    proj_q(0, None)
    proj_v(0, None)
    for i in range(1, S // RB1):
        hn = modulate1(norm1(i + 1)) if i + 1 < S // RB1 else None
        proj_k(i, h)
        rot_k(i)
        proj_v(i, h)
        proj_q(i, h)
        h = hn

    def q_rows(h, qb):
        return qt_s[pl.ds(_mo(h * 8, 8), 8), qb * TQ:(qb + 1) * TQ]

    def clamp_h(h):
        return min(h, H - 1) if isinstance(h, int) else jnp.minimum(h, H - 1)

    def make_qb(h, qb, slot, ds_, tok=None, never=None):
        qf = _upk(q_rows(h, qb)).astype(F32)
        for d in ds_:
            val = jnp.broadcast_to(qf[d:d + 1], (8, TQ))
            if tok is not None:
                val = jnp.where(never, tok, val)
            qb_s[slot, d] = val

    def make_kb(h, d, kb, tok=None, never=None):
        kt = _upk(kt_s[pl.ds(_mo(h * 8, 8), 8), :]).astype(F32)
        row = jnp.broadcast_to(kt[d:d + 1], (8, NVP))
        if tok is not None:
            row = jnp.where(never, tok[:, :NVP], row)
        val = jnp.concatenate([row] * 16, axis=0).T
        kb[d] = val
        return val[NVP - 8:]

    a_len = [7 if (c * NG) // NC != ((c + 1) * NG) // NC else 8 for c in range(NC)]
    a_off = [sum(a_len[:c]) for c in range(NC)]
    assert sum(a_len) * 16 == KM
    v_sched = [[] for _ in range(NC)]
    for u in range(2 * NG):
        v_sched[(u * NC) // (2 * NG)].append(u)

    def fence(val, on, never):
        return jnp.where(never, pltpu.bitcast(val, jnp.uint32), on)

    def v_piece(u, tl, kb, slot, sbuf):
        kr = 8 * u
        ts = [kb[d, pl.ds(NVP - NV + kr, 8), :] * qb_s[slot, d, :, tl * 128:(tl + 1) * 128]
              for d in range(DH)]
        a0, a1 = ts[0], ts[1]
        for d in range(2, DH, 2):
            a0 = a0 + ts[d]
            a1 = a1 + ts[d + 1]
        acc = a0 + a1
        sbuf[pl.ds(KM + kr, 8), tl * 128:(tl + 1) * 128] = acc
        return acc

    def v_unit_dmajor(u, kb, slot, sbuf):
        kr = 8 * u
        toks = []
        acc = None
        for d in range(DH):
            kk = kb[d, pl.ds(NVP - NV + kr, 8), :]
            t_ = jnp.concatenate([kk] * 4, axis=1) * qb_s[slot, d]
            acc = t_ if acc is None else acc + t_
            if (d + 1) % (DH // NP) == 0:
                toks.append((acc[:, 0:128] + acc[:, 128:256]) + (acc[:, 256:384] + acc[:, 384:512]))
        sbuf[pl.ds(KM + kr, 8), :] = acc
        return toks, acc

    def a_tick(w, h, c_, kb, slot, sbuf, m, never=None, extra=()):
        if DMAJ:
            units = [v_unit_dmajor(u, kb, slot, sbuf) for u in v_sched[c_]]
            pieces = [(None, tk) for toks, _ in units for tk in toks]
        else:
            pieces = [(tl, v_piece(u, tl, kb, slot, sbuf)) for u in v_sched[c_] for tl in range(4)]
        r0, n = a_off[c_] * 16, a_len[c_] * 16
        kc = k_s[h, pl.ds(r0 // 2, n // 2), :]
        if never is not None:
            parts = [kc[8 * j:8 * j + 8] for j in range(n // 16)]
            for i_, (_, pv) in enumerate(pieces):
                j = max(0, n // 16 - FOFF - len(pieces) + i_)
                parts[j] = fence(pv, parts[j], never[0])
            for val in extra:
                parts[0] = fence(val, parts[0], never[1])
            kc = jnp.concatenate(parts, axis=0)
        st = jnp.dot(_upk(kc)[:, :DH], w, preferred_element_type=F32)
        sbuf[pl.ds(r0, n), :] = st
        for j in range(n // 8):
            m = jnp.maximum(m, st[8 * j:8 * j + 8])
        if DMAJ:
            for _, acc_ in units:
                m = jnp.maximum(m, acc_)
        elif pieces:
            parts = [m[:, i_ * 128:(i_ + 1) * 128] for i_ in range(4)]
            for tl, pv in pieces:
                parts[tl] = jnp.maximum(parts[tl], pv)
            m = jnp.concatenate(parts, axis=1)
        return m

    def b_chunk(h, ck, sbuf, mb, l, acc, alpha=None):
        s = sbuf[pl.ds(ck * CK, CK), :]
        p = jnp.exp2(s.reshape(CK // 8, 8, TQ) - mb[None]).reshape(CK, TQ)
        if XS & 2:
            l = None if ck == 0 else l_s[...]
            if alpha is not None:
                l = l * alpha
        for j in reversed(range(CK // 16)):
            pr = p[16 * j:16 * j + 8] + p[16 * j + 8:16 * j + 16]
            l = pr if l is None else l + pr
        if XS & 2:
            l_s[...] = l
        vc = _upk(vt_s[pl.ds(_mo(h * 8, 8), 8), pl.ds(ck * CK, CK)])
        pv = jnp.dot(vc, p.astype(BF), preferred_element_type=F32)
        if XS & 1:
            if ck == 0:
                acc = pv
            else:
                acc = acc_s[...]
                if alpha is not None:
                    acc = (acc.reshape(2, 8, TQ) * alpha[None]).reshape(16, TQ)
                acc = acc + pv
            acc_s[...] = acc
        else:
            acc = acc + pv
        return l, acc

    neg = jnp.full((8, TQ), -jnp.inf, F32)
    zl = jnp.zeros((8, TQ), F32)
    za = jnp.zeros((16, TQ), F32)

    def fin(h, qb, l, acc):
        lsum = l.sum(axis=0, keepdims=True)
        o = acc * (1.0 / lsum)
        ot_s[pl.ds(_mo(h * 8, 8), 8), qb * TQ:(qb + 1) * TQ] = _pk(o.astype(BF))

    def red_m(m):
        return jnp.broadcast_to(m.max(axis=0, keepdims=True), (8, TQ))

    bufs = (s0, s1)
    kbs = (kb0, kb1)

    def run_steps(h0, state, never, last=False, hooks=None):
        m_pre, m_fin = state
        mh_prev = None
        pend = {}
        for s_ in range(SPI):
            hb, qb = h0 + s_ // NQ, s_ % NQ
            ua = s_ + 1
            ha, qa = h0 + ua // NQ, ua % NQ
            s_cur, s_next = bufs[s_ % 2], bufs[1 - s_ % 2]
            do_a = not (last and s_ == SPI - 1)
            if do_a:
                w = _upk(q_rows(ha, qa))
            kb_use = kbs[(ua // NQ) % 2]
            kb_make = kbs[1 - (ua // NQ) % 2]
            m = neg
            mh = []
            l, acc = zl, za
            mb = red_m(m_pre)
            for c_ in range(NC):
                gt = s_ * NC + c_
                if do_a:
                    m = a_tick(w, ha, c_, kb_use, s_, s_next, m, never, pend.pop(gt, ()))
                if hooks is not None and s_ in hooks:
                    hooks[s_](c_)
                mh.append(m)
                if c_ - TD >= 0:
                    tok = mh[c_ - TD]
                elif mh_prev is not None:
                    tok = mh_prev[NC + c_ - TD]
                else:
                    tok = None
                if not last and not NOQB and s_ >= 1:
                    un = s_ + SPI
                    make_qb(clamp_h(h0 + un // NQ), un % NQ, s_ - 1, [c_], tok, never[0])
                hk = ha + 1
                ok = (not last) or (h0 + ua // NQ + 1 < H)
                atick = qa * NC + c_
                if ok and not NOKB and atick % 4 == 0:
                    val = make_kb(hk, atick // 4, kb_make, tok if KTOK else None, never[0])
                    if gt + KFD < SPI * NC:
                        pend.setdefault(gt + KFD, []).append(val)
                alpha = None
                if c_ == KSW:
                    mb2 = red_m(m_fin)
                    alpha = jnp.exp2(mb - mb2)
                    if not XS & 2:
                        l = l * alpha
                    if not XS & 1:
                        acc = (acc.reshape(2, 8, TQ) * alpha[None]).reshape(16, TQ)
                    mb = mb2
                    if XS & 4:
                        mb_s[...] = mb
                if XS & 4 and c_ > KSW:
                    mb = mb_s[...]
                mbc = mb
                nv_ = never[c_ % 2] if CHAIN else never[0]
                if c_ - FM >= 0:
                    if do_a:
                        mbc = jnp.where(nv_, mh[c_ - FM], mb)
                elif mh_prev is not None:
                    mbc = jnp.where(nv_, mh_prev[NC + c_ - FM], mb)
                if CHAIN:
                    mb = mbc
                l, acc = b_chunk(hb, c_, s_cur, mbc, l, acc, alpha)
            fin(hb, qb, l, acc)
            m_pre, m_fin = mh[NC - 1 - G], m
            mh_prev = mh
        if not last and not NOQB:
            un = 2 * SPI
            make_qb(clamp_h(h0 + un // NQ), un % NQ, SPI - 1, range(DH))
        return m_pre, m_fin

    if PH & 2:
        make_qb(0, 0, SPI, range(DH))
        for u_ in range(1, SPI + 1):
            make_qb(u_ // NQ, u_ % NQ, u_ - 1, range(DH))
        for d in range(DH):
            make_kb(0, d, kb0)
        for d in range(4):
            make_kb(1, d, kb1)
        w0 = _upk(q_rows(0, 0))
        m0 = neg
        for c_ in range(NC):
            m0 = a_tick(w0, 0, c_, kb0, SPI, s0, m0)

        def p2_body(i, state):
            return run_steps(2 * i, state, (i < 0, i < -1))

        st = jax.lax.fori_loop(0, ((T - PEEL) // SPI), p2_body, (m0, m0))

    cp_wmod_b.wait()
    cp_wo.wait()
    cp_win.wait()
    cp_wsp.wait()
    cp_wout.wait()
    cp_bsp.wait()
    if PH == 2:
        out_v[0:16, :] = _upk(ot_s[0:8, 0:512])
        out_v[16:32, :] = (st[0] + st[1]).astype(BF)[0:1] + jnp.zeros((16, D), BF)
        cpo = pltpu.make_async_copy(out_v, out_hbm.at[0], osems.at[0])
        cpo.start()
        cpo.wait()
        return

    def mod_piece(c_):
        c0 = 2 * D + c_ * 128
        mod_v[:, c0:c0 + 128] = jnp.dot(sc, wmod_v[:, c0:c0 + 128], preferred_element_type=F32)[:8]

    attn0 = []
    PR = RB3 * HOOK // NC
    o0_box = []

    def wo_piece(c_):
        if not o0_box:
            o0_box.append(_upk(ot_s[:, pl.ds(0, RB3 * HOOK)]).T)
        attn0.append(jnp.dot(o0_box[0][c_ * PR:(c_ + 1) * PR], wo_v[...], preferred_element_type=F32))

    hooks = {0: mod_piece}
    if HOOK:
        hooks[PEEL - 1] = wo_piece
    run_steps(H - 2, st, (z_s[0] != 0, z_s[0] > 1), last=True, hooks=hooks)
    if HOOK:
        attn0 = jnp.concatenate(attn0, axis=0)

    def p3a(i):
        r0 = i * RB3
        if i >= HOOK:
            ot = _upk(ot_s[:, pl.ds(r0, RB3)])
        if i < HOOK:
            attn = attn0[r0:r0 + RB3]
        elif NT3:
            attn = jnp.concatenate(_dot_nt(ot.T, wo_v, 0, D, NT3), axis=1)
        else:
            attn = jnp.dot(ot.T, wo_v[...], preferred_element_type=F32)
        x1 = x_v[pl.ds(r0, RB3), :].astype(F32) + mod_row(2) * attn
        x1_s[pl.ds(r0, RB3), :] = x1
        h2 = (_ln(x1) * (1.0 + mod_row(4)) + mod_row(3)).astype(BF)
        h2_s[pl.ds(r0 // 2, RB3 // 2), :] = _pk(h2)
        return h2

    def p3b(i, h2):
        r0 = i * RB3
        if NT3:
            z2 = jnp.concatenate([_gelu(z) for z in _dot_nt(h2, win_v, FH, FH, NT3)], axis=1)
        else:
            z2 = _gelu(jnp.dot(h2, win_v[:, FH:], preferred_element_type=F32))
        z2_s[pl.ds(r0 // 2, RB3 // 2), :] = _pk(_ln(z2).astype(BF))
        if i < Z1P3:
            z1_s[pl.ds(r0, RB3), :] = jnp.dot(h2, win_v[:, :FH], preferred_element_type=F32)

    if PH & 4:
        N3 = S // RB3
        P3D = 3
        h2s = {}
        for i in range(min(P3D, N3)):
            h2s[i] = p3a(i)
        for i in range(N3):
            if i + P3D < N3:
                h2s[i + P3D] = p3a(i + P3D)
            p3b(i, h2s.pop(i))

    oblocks = _out_blocks()

    def out_copy(j):
        r0, n = oblocks[j]
        return pltpu.make_async_copy(out_v.at[pl.ds(r0, n), :],
                                     out_hbm.at[0, pl.ds(r0, n), :], osems.at[j])

    brow_all = bsp_v[...].reshape(1, S).astype(F32)
    j = 0
    for i in range(S // RB4):
        r0 = i * RB4
        if PH & 8:
            if r0 < Z1P3 * RB3:
                z1 = _gelu(z1_s[pl.ds(r0, RB4), :])
            else:
                h2 = _upk(h2_s[pl.ds(r0 // 2, RB4 // 2), :])
                z1 = _gelu(jnp.dot(h2, win_v[:, :FH], preferred_element_type=F32))
            gsp = jnp.dot(wsp_v[pl.ds(r0, RB4), :], _upk(z2_s[...]), preferred_element_type=F32)
            brow = brow_all[:, r0:r0 + RB4]
            bcol = jnp.broadcast_to(brow, (128, RB4)).T
            bfull = jnp.concatenate([bcol] * (FH // 128), axis=1)
            u = (z1 * (gsp + bfull)).astype(BF)
        while j < len(oblocks) and oblocks[j][0] < r0 + RB4:
            o0, n = oblocks[j]
            if PH & 8:
                y = jnp.dot(u[o0 - r0:o0 - r0 + n], wout_v[...], preferred_element_type=F32)
                out_v[pl.ds(o0, n), :] = (x1_s[pl.ds(o0, n), :] + mod_row(5) * y).astype(BF)
            out_copy(j).start()
            j += 1
    for j in range(len(oblocks)):
        out_copy(j).wait()


@jax.jit
def pallas_adaLN_cond__softmax_full_mha__mixer_gmlp__prompt_kernel(
    A_x, A_wqkv, A_wo, B_x, B_w_in, B_w_sp, B_b_sp, B_w_out, c, w_mod):
    del B_x
    any_spec = pl.BlockSpec(memory_space=pl.ANY)
    u32 = jnp.uint32
    scratch = [
        pltpu.VMEM((S, D), BF), pltpu.VMEM((D, 3 * D), BF), pltpu.VMEM((D, D), BF),
        pltpu.VMEM((D, 2 * FH), BF), pltpu.VMEM((S, S), BF), pltpu.VMEM((FH, D), BF),
        pltpu.VMEM((D, 6 * D), BF), pltpu.VMEM((1, D), BF), pltpu.VMEM((S,), BF),
        pltpu.VMEM((8, 6 * D), F32),
        pltpu.VMEM((H, S // 2, 128), u32), pltpu.VMEM((D // 2, S), u32), pltpu.VMEM((D // 2, S), u32),
        pltpu.VMEM((D // 2, NVP), u32), pltpu.VMEM((DH, NVP, 128), F32), pltpu.VMEM((DH, NVP, 128), F32),
        pltpu.VMEM((SPI + 1, DH, 8, TQ), F32),
        pltpu.VMEM((16, TQ), F32), pltpu.VMEM((8, TQ), F32), pltpu.VMEM((8, TQ), F32),
        pltpu.VMEM((S, TQ), F32), pltpu.VMEM((S, TQ), F32), pltpu.VMEM((D // 2, S), u32),
        pltpu.VMEM((S, D), F32), pltpu.VMEM((S // 2, D), u32), pltpu.VMEM((S // 2, FH), u32),
        pltpu.VMEM((S, FH), F32),
        pltpu.VMEM((RB1, 3 * D), F32),
        pltpu.VMEM((S, D), BF),
        pltpu.SMEM((1,), jnp.int32),
        pltpu.SemaphoreType.DMA((22,)),
        pltpu.SemaphoreType.DMA((len(_out_blocks()),)),
    ]
    return pl.pallas_call(
        _kernel,
        out_shape=jax.ShapeDtypeStruct((1, S, D), BF),
        in_specs=[any_spec] * 9,
        out_specs=any_spec,
        scratch_shapes=scratch,
        compiler_params=pltpu.CompilerParams(vmem_limit_bytes=100 * 1024 * 1024),
    )(A_x, A_wqkv, A_wo, B_w_in, B_w_sp, B_b_sp, B_w_out, c, w_mod)
```

```python
import jax
import jax.numpy as jnp
import jax.experimental.pallas as pl
import jax.experimental.pallas.tpu as pltpu

S = 2048; D = 512; H = 32; DH = 16; FH = 896
EPS = 1e-5
LOG2E = 1.4426950408889634
QSCALE = (DH ** -0.5) * LOG2E

TQ = 512
CK = 128
NC = S // CK
NQ = S // TQ
T = H * NQ
RB1 = 512
RB3 = 512
RB4 = 512
SPI = 8
PH = 15
HPI = SPI // NQ
NG = 15
KU = 2
TU = 4 // KU
NPG = 4
KFD = 8
TD = 3
XS = 3
PLO = 0
P1O = 1
KEEP = 1
SH = 1
VB = 7
FORCE_FB = 0
L_MIN = 2.0 ** -64
L_MAX = 2.0 ** 20
OT = 128

BF = jnp.bfloat16
F32 = jnp.float32


def _pk(x):
    return pltpu.bitcast(x, jnp.uint32)


def _upk(x):
    return pltpu.bitcast(x, BF)


def _mo(x, n):
    return x if isinstance(x, int) else pl.multiple_of(x, n)


def _ln(x):
    m = jnp.mean(x, axis=-1, keepdims=True)
    xc = x - m
    v = jnp.mean(xc * xc, axis=-1, keepdims=True)
    return xc * jax.lax.rsqrt(v + EPS)


def _gelu(x):
    c0 = 0.7978845608028654
    inner = x * (c0 + (c0 * 0.044715) * (x * x))
    hx = 0.5 * x
    return hx + hx * jnp.tanh(inner)


def _dot_nt(a, w_ref, c0, n, tile):
    return [jnp.dot(a, w_ref[:, c0 + j:c0 + j + tile], preferred_element_type=F32)
            for j in range(0, n, tile)]


def _out_blocks():
    blocks = [(i * RB4, RB4) for i in range(S // RB4 - 1)]
    r0 = S - RB4
    blocks += [(r0 + j * OT, OT) for j in range(RB4 // OT)]
    return blocks


def _kernel(x_hbm, wqkv_hbm, wo_hbm, win_hbm, wsp_hbm, bsp_hbm, wout_hbm, c_hbm, wmod_hbm,
            out_hbm,
            x_v, wqkv_v, wo_v, win_v, wsp_v, wout_v, wmod_v, c_v, bsp_v, mod_v,
            k_s, kr_s, qt_s, vt_s, ksel_s, kt_s, qn_s, kn_s, kb0, kb1, qb_s, acc_s, l_s, car_s, s0, ot_s, x1_s, h2_s, z2_s, q0_s, out_v, z_s, sems, osems):
    z_s[0] = 0
    def cols(src, dst, c0, n, sem):
        return pltpu.make_async_copy(src.at[:, pl.ds(c0, n)], dst.at[:, pl.ds(c0, n)], sem)

    def xrows(r0, n, sem):
        return pltpu.make_async_copy(x_hbm.at[0, pl.ds(r0, n), :], x_v.at[pl.ds(r0, n), :], sem)

    NJ = 4
    JW = D // NJ
    cp_c = pltpu.make_async_copy(c_hbm, c_v, sems.at[0])
    cp_x0 = xrows(0, RB1, sems.at[1])
    cp_ms = [cols(wmod_hbm, wmod_v, j * JW, JW, sems.at[14 + j]) for j in range(NJ)]
    cp_mc = [cols(wmod_hbm, wmod_v, D + j * JW, JW, sems.at[18 + j]) for j in range(NJ)]
    cp_w = [pltpu.make_async_copy(wqkv_hbm.at[pl.ds(j * JW, JW), :], wqkv_v.at[pl.ds(j * JW, JW), :],
                                  sems.at[2 + j]) for j in range(NJ)]
    cp_x1 = xrows(RB1, RB1, sems.at[6])
    cp_x23 = xrows(2 * RB1, 2 * RB1, sems.at[7])
    cp_wmod_b = cols(wmod_hbm, wmod_v, 2 * D, 4 * D, sems.at[8])
    cp_wo = pltpu.make_async_copy(wo_hbm, wo_v, sems.at[9])
    cp_win = pltpu.make_async_copy(win_hbm, win_v, sems.at[10])
    cp_wsp = pltpu.make_async_copy(wsp_hbm, wsp_v, sems.at[11])
    cp_wout = pltpu.make_async_copy(wout_hbm, wout_v, sems.at[12])
    cp_bsp = pltpu.make_async_copy(bsp_hbm, bsp_v, sems.at[13])
    order = [cp_c, cp_x0, cp_ms[0], cp_mc[0]]
    for j in range(NJ):
        if j + 1 < NJ:
            order += [cp_ms[j + 1], cp_mc[j + 1]]
        order.append(cp_w[j])
    order.insert(len(order) - 1, cp_x1)
    order += [cp_x23, cp_wmod_b, cp_wo, cp_win, cp_wsp, cp_wout, cp_bsp]
    for cp in order:
        cp.start()

    cp_c.wait()
    cp_x0.wait()
    c = c_v[...].astype(F32)
    sc = (c * jax.nn.sigmoid(c)).astype(BF)
    sc = jnp.broadcast_to(sc, (16, D))

    def norm1(i):
        return _ln(x_v[pl.ds(i * RB1, RB1), :].astype(F32))

    def mod_row(j):
        return mod_v[0:1, j * D:(j + 1) * D]

    def modulate1(n):
        return (n * (1.0 + mod_row(1)) + mod_row(0)).astype(BF)

    n0 = norm1(0)

    def h0_piece(j):
        for c0 in (j * JW, D + j * JW):
            mod_v[:, c0:c0 + JW] = jnp.dot(sc, wmod_v[:, c0:c0 + JW], preferred_element_type=F32)[:8]
        sa = mod_v[0:1, j * JW:(j + 1) * JW]
        ca = mod_v[0:1, D + j * JW:D + (j + 1) * JW]
        return (n0[:, j * JW:(j + 1) * JW] * (1.0 + ca) + sa).astype(BF)

    cp_ms[0].wait()
    cp_mc[0].wait()
    hj = h0_piece(0)
    qkv0 = None
    for j in range(NJ):
        if j + 1 < NJ:
            cp_ms[j + 1].wait()
            cp_mc[j + 1].wait()
        if j == NJ - 2:
            cp_x1.wait()
        cp_w[j].wait()
        part = jnp.dot(hj, wqkv_v[j * JW:(j + 1) * JW, :], preferred_element_type=F32)
        if j == 0:
            q0_s[...] = part
        elif j + 1 < NJ:
            q0_s[...] = q0_s[...] + part
        else:
            qkv0 = q0_s[...] + part
        if j + 1 < NJ:
            hj = h0_piece(j + 1)
        if j >= NJ - 2:
            hr = RB1 // 2
            r1 = RB1 + (j - (NJ - 2)) * hr
            h2_s[pl.ds((j - (NJ - 2)) * hr // 2, hr // 2), :] = _pk(
                modulate1(_ln(x_v[pl.ds(r1, hr), :].astype(F32))))

    def head_sq(xt):
        xf = xt.astype(F32)
        return (xf * xf).reshape(H, DH, xt.shape[1]).sum(axis=1)

    def proj_k(i, h):
        k = qkv0[:, D:2 * D] if i == 0 else jnp.dot(h, wqkv_v[:, D:2 * D], preferred_element_type=F32)
        k = k.astype(BF)
        kp = _pk(k)
        for g in range(4):
            kr_s[g, pl.ds(i * RB1 // 2, RB1 // 2), :] = kp[:, g * 128:(g + 1) * 128]
        for t_ in range(RB1 // CK):
            ksel_s[pl.ds((i * (RB1 // CK) + t_) * 8, 8), :] = kp[t_ * 64 + 8 * VB:t_ * 64 + 8 * VB + 8]
        kn = head_sq(k.T)
        kn_s[...] = kn if i == 0 else jnp.maximum(kn_s[...], kn)

    lane = jax.lax.broadcasted_iota(jnp.int32, (8, 128), 1)
    one_pk = _pk(jnp.where(jax.lax.broadcasted_iota(jnp.int32, (16, 128), 1) == 2 * DH, 1.0, 0.0).astype(BF))

    def rot_k(i):
        n8 = RB1 // 16
        keep = jnp.broadcast_to((lane < 2 * DH)[None], (n8, 8, 128))
        fill = jnp.broadcast_to(one_pk[None], (n8, 8, 128))
        for g in range(4):
            kg = kr_s[g, pl.ds(i * RB1 // 2, RB1 // 2), :]
            for j in range(4):
                kj = kg if j == 0 else pltpu.roll(kg, 128 - 32 * j, axis=1)
                kj = jnp.where(keep, kj.reshape(n8, 8, 128), fill).reshape(RB1 // 2, 128)
                k_s[4 * g + j, pl.ds(i * RB1 // 2, RB1 // 2), :] = kj

    def proj_q(i, h):
        q = qkv0[:, :D] if i == 0 else jnp.dot(h, wqkv_v[:, :D], preferred_element_type=F32)
        qt = (q * QSCALE).astype(BF).T
        qt_s[:, pl.ds(i * RB1, RB1)] = _pk(qt)
        qn_s[:, pl.ds(i * RB1, RB1)] = head_sq(qt)

    def make_ref(i):
        kmax = jnp.max(kn_s[...], axis=1, keepdims=True)
        bound = jnp.sqrt(qn_s[:, pl.ds(i * RB1, RB1)] * kmax) * (1.0 + 2.0 ** -6)
        qn_s[:, pl.ds(i * RB1, RB1)] = (-bound).astype(BF).astype(F32)

    def proj_v(i, h):
        v = qkv0[:, 2 * D:] if i == 0 else jnp.dot(h, wqkv_v[:, 2 * D:], preferred_element_type=F32)
        v = v.astype(BF)
        vt_s[:, pl.ds(i * RB1, RB1)] = _pk(v.T)

    cp_x23.wait()
    NB1 = S // RB1
    hs = {1: _upk(h2_s[pl.ds(0, RB1 // 2), :])}
    proj_k(0, None)
    rot_k(0)
    proj_q(0, None)
    proj_v(0, None)
    if P1O == 0:
        for i in range(1, NB1):
            if i + 1 < NB1:
                hs[i + 1] = modulate1(norm1(i + 1))
            proj_k(i, hs[i])
            rot_k(i)
        kt_s[...] = _pk(_upk(ksel_s[...]).T)
        make_ref(0)
        for i in range(1, NB1):
            proj_q(i, hs[i])
            make_ref(i)
        for i in range(1, NB1):
            proj_v(i, hs[i])
    else:
        hs[2] = modulate1(norm1(2))
        proj_k(1, hs[1]); rot_k(1)
        proj_q(1, hs[1])
        hs[3] = modulate1(norm1(3))
        proj_k(2, hs[2]); rot_k(2)
        proj_k(3, hs[3]); rot_k(3)
        kt_s[...] = _pk(_upk(ksel_s[...]).T)
        make_ref(0); make_ref(1)
        proj_q(2, hs[2]); make_ref(2)
        proj_q(3, hs[3]); make_ref(3)
        for i in range(1, NB1):
            proj_v(i, hs[i])

    def q_rows(h, qb):
        return qt_s[pl.ds(_mo(h * 8, 8), 8), qb * TQ:(qb + 1) * TQ]

    def nref_row(h, qb):
        return qn_s[pl.ds(h, 1), qb * TQ:(qb + 1) * TQ]

    def clamp_h(h):
        return min(h, H - 1) if isinstance(h, int) else jnp.minimum(h, H - 1)

    row0 = jax.lax.broadcasted_iota(jnp.int32, (16, TQ), 0) == 0

    def make_w(h, qb, par):
        aug = jnp.where(row0, jnp.broadcast_to(nref_row(h, qb), (16, TQ)), 0.0).astype(BF)
        q = _upk(q_rows(h, qb))
        z = jnp.zeros((DH, TQ), BF)
        return jnp.concatenate([z, q, aug] if par else [q, z, aug], axis=0)

    def make_qb(h, qb, slot, ds_, tok=None, never=None):
        qf = _upk(q_rows(h, qb)).astype(F32)
        for d in ds_:
            row = nref_row(h, qb) if d == DH else qf[d:d + 1]
            val = jnp.broadcast_to(row, (8, TQ))
            if tok is not None:
                val = jnp.where(never, tok, val)
            qb_s[slot, d] = val

    def make_kb(h, j, kb, tok=None, never=None):
        d, half = j // 2, j % 2
        kt = _upk(kt_s[pl.ds(_mo(h * 8, 8), 8), half * 128:(half + 1) * 128]).astype(F32)
        row = jnp.broadcast_to(kt[d:d + 1], (8, 128))
        if tok is not None:
            row = jnp.where(never, tok[:, :128], row)
        val = jnp.concatenate([row] * 16, axis=0).T
        kb[d, pl.ds(half * 128, 128), :] = val
        return val[120:]

    v_tiles = sorted(set(NC - 1 - (k_ * (NC - 1)) // NG for k_ in range(NG))) if NG else []
    assert len(v_tiles) == NG and 0 not in v_tiles

    def fence(val, on, never):
        return jnp.where(never, pltpu.bitcast(val, jnp.uint32), on)

    def v_unit(tile, ui, kb, slot):
        per = 4 // TU
        kr = 16 * tile + 8 * KU * (ui // per)
        c0 = (ui % per) * TU * 128
        acc = None
        toks = []
        for d in range(DH):
            kk = kb[d, pl.ds(kr, 8 * KU), :]
            kk = jnp.concatenate([kk] * TU, axis=1).reshape(KU, 8, TU * 128)
            t_ = kk * qb_s[slot, d, :, c0:c0 + TU * 128][None]
            acc = t_ + qb_s[slot, DH, :, c0:c0 + TU * 128][None] if acc is None else acc + t_
            if (d + 1) % (DH // NPG) == 0:
                ts = [acc[a_, :, b_ * 128:(b_ + 1) * 128] for a_ in range(KU) for b_ in range(TU)]
                toks.append((ts[0] + ts[1]) + (ts[2] + ts[3]))
        return acc.reshape(8 * KU, TU * 128), toks

    def tile_blocks(tile):
        return [j for j in reversed(range(8)) if not (tile in v_tiles and j == VB)]

    def v_rows(tile, kb, slot):
        us = [v_unit(tile, ui, kb, slot) for ui in range(2)]
        vrows = jnp.concatenate([us[0][0], us[1][0]], axis=1 if KU == 2 else 0)
        return vrows, us[0][1] + us[1][1]

    def qk_run(w, h, items, toks, never, extra=()):
        parts = [k_s[h, pl.ds(t_ * 64 + 8 * j, 8), :] for t_, j in items]
        n_ = len(parts) - PLO
        for i_, tk in enumerate(toks):
            j = PLO + (i_ * n_) // len(toks)
            parts[j] = fence(tk, parts[j], never[i_ % 2])
        for val in extra:
            parts[0] = fence(val, parts[0], never[2])
        st = jnp.dot(_upk(jnp.concatenate(parts, axis=0))[:, :3 * DH], w, preferred_element_type=F32)
        return [st[16 * i_:16 * i_ + 16] for i_ in range(len(items))]

    def b_tile(h, ck, s, l, acc):
        p = jnp.exp2(s)
        if XS & 2:
            l = None if ck == 0 else l_s[...]
        for j in reversed(range(CK // 16)):
            pr = p[16 * j:16 * j + 8] + p[16 * j + 8:16 * j + 16]
            l = pr if l is None else l + pr
        if XS & 2:
            l_s[...] = l
        vc = _upk(vt_s[pl.ds(_mo(h * 8, 8), 8), pl.ds(ck * CK, CK)])
        pv = jnp.dot(vc, p.astype(BF), preferred_element_type=F32)
        if ck == 0:
            acc = pv
        else:
            acc = (acc_s[...] if XS & 1 else acc) + pv
        if XS & 1:
            acc_s[...] = acc
        return l, acc

    def fin(h, qb, l, acc):
        lsum = l.sum(axis=0, keepdims=True)
        o = acc * (1.0 / lsum)
        ot_s[pl.ds(_mo(h * 8, 8), 8), qb * TQ:(qb + 1) * TQ] = _pk(o.astype(BF))
        return lsum

    kbs = (kb0, kb1)

    car_items = [(0, j) for j in tile_blocks(0)] + [(1, j) for j in tile_blocks(1)[:SH]]

    def run_steps(hp0, state, never):
        h0 = 2 * hp0
        lo, hi = state
        pend = {}
        lh = []
        sc_ = {}
        for i_, (t_, j) in enumerate(car_items):
            sc_[(0, t_, j)] = car_s[pl.ds(16 * i_, 16), :]
        ws = {}

        def step_hq(s_):
            return clamp_h(h0 + s_ // NQ) if s_ >= SPI else h0 + s_ // NQ, s_ % NQ

        def pair_of(s_):
            p_ = hp0 + s_ // (2 * NQ)
            return jnp.minimum(p_, H // 2 - 1) if s_ >= SPI else p_

        def get_w(s_):
            if s_ not in ws:
                ws[s_] = make_w(*step_hq(s_), (s_ // NQ) % 2)
            return ws[s_]

        for s_ in range(SPI):
            h, qb = step_hq(s_)
            kb_use = kbs[(s_ // NQ) % 2]
            kb_make = kbs[1 - (s_ // NQ) % 2]
            l = acc = None
            for c_ in range(NC):
                gt = s_ * NC + c_
                g1, g2 = gt + 1, gt + 2
                it1 = [(g1 // NC, g1 % NC, j) for j in tile_blocks(g1 % NC)[SH:]]
                it2 = [(g2 // NC, g2 % NC, j) for j in tile_blocks(g2 % NC)[:SH]]
                toks = []
                if c_ + 1 < NC and (c_ + 1) in v_tiles:
                    sc_[(s_, c_ + 1, VB)], toks = v_rows(c_ + 1, kb_use, s_)
                runs = [it1 + it2] if g1 // NC == g2 // NC else [it1, it2]
                for ri, its in enumerate(runs):
                    if not its:
                        continue
                    sr = its[0][0]
                    outs = qk_run(get_w(sr), pair_of(sr), [(t_, j) for _, t_, j in its],
                                  toks if ri == 0 else [], never,
                                  pend.pop(gt, ()) if ri == 0 else ())
                    sc_.update(zip(its, outs))
                tok = lh[-TD] if len(lh) >= TD else None
                if s_ >= 1:
                    un = s_ - 1 + SPI
                    ds_ = [c_, DH] if c_ == NC - 1 else [c_]
                    make_qb(clamp_h(h0 + un // NQ), un % NQ, s_ - 1, ds_, tok, never[0])
                ht = (s_ % NQ) * NC + c_
                if ht % 2 == 0:
                    val = make_kb(clamp_h(h + 1), ht // 2, kb_make, tok, never[0])
                    if gt + KFD < SPI * NC:
                        pend.setdefault(gt + KFD, []).append(val)
                s_cur = jnp.concatenate([sc_.pop((s_, c_, j)) for j in range(8)], axis=0)
                l, acc = b_tile(h, c_, s_cur, l, acc)
                lh.append(l)
            lsum = fin(h, qb, l, acc)
            lo = jnp.minimum(lo, lsum)
            hi = jnp.maximum(hi, lsum)
        for i_, (t_, j) in enumerate(car_items):
            car_s[pl.ds(16 * i_, 16), :] = sc_.pop((SPI, t_, j))
        un = 2 * SPI - 1
        make_qb(clamp_h(h0 + un // NQ), un % NQ, SPI - 1, range(DH + 1))
        return lo, hi

    for u_ in range(SPI):
        make_qb(u_ // NQ, u_ % NQ, u_, range(DH + 1))
    for j in range(2 * DH):
        make_kb(0, j, kb0)
    for i_, o_ in enumerate(qk_run(make_w(0, 0, 0), 0, car_items, [], None)):
        car_s[pl.ds(16 * i_, 16), :] = o_

    def p2_body(i, state):
        return run_steps((HPI // 2) * i, state, (i < 0, i < -1, i < -2))

    one = jnp.ones((1, TQ), F32)
    lo, hi = jax.lax.fori_loop(0, (T // SPI), p2_body, (one, one))

    cp_wmod_b.wait()
    cp_wo.wait()
    cp_win.wait()
    cp_wsp.wait()
    cp_wout.wait()
    cp_bsp.wait()

    ok = jnp.logical_and(lo >= L_MIN, hi <= L_MAX)
    n_bad = jnp.sum(jnp.where(ok, 0.0, 1.0))

    @pl.when(jnp.logical_or(n_bad > 0.0, FORCE_FB > 0))
    def _():
        def exact_step(t, carry):
            h = t // NQ
            c0 = pl.multiple_of((t % NQ) * TQ, TQ)
            r8 = pl.multiple_of(h * 8, 8)
            q = qt_s[pl.ds(r8, 8), pl.ds(c0, TQ)]
            zq = jnp.zeros_like(q)
            odd = h % 2 == 1
            w = _upk(jnp.concatenate([jnp.where(odd, zq, q), jnp.where(odd, q, zq)], axis=0))
            s0[...] = jnp.dot(_upk(k_s[h // 2])[:, :2 * DH], w, preferred_element_type=F32)
            st = s0[...]
            p = jnp.exp2(st - jnp.max(st, axis=0, keepdims=True))
            lsum = jnp.sum(p, axis=0, keepdims=True)
            o = jnp.dot(_upk(vt_s[pl.ds(r8, 8), :]), p.astype(BF), preferred_element_type=F32)
            ot_s[pl.ds(r8, 8), pl.ds(c0, TQ)] = _pk((o * (1.0 / lsum)).astype(BF))
            return carry

        if KEEP:
            s0[0:16, :] = acc_s[...]
            s0[16:24, :] = l_s[...]

        jax.lax.fori_loop(0, T, exact_step, 0)

    mod_v[:, 2 * D:] = jnp.dot(sc, wmod_v[:, 2 * D:], preferred_element_type=F32)[:8]

    def p3a(i):
        r0 = i * RB3
        ot = _upk(ot_s[:, pl.ds(r0, RB3)])
        attn = jnp.dot(ot.T, wo_v[...], preferred_element_type=F32)
        x1 = x_v[pl.ds(r0, RB3), :].astype(F32) + mod_row(2) * attn
        x1_s[pl.ds(r0, RB3), :] = x1
        h2 = (_ln(x1) * (1.0 + mod_row(4)) + mod_row(3)).astype(BF)
        h2_s[pl.ds(r0 // 2, RB3 // 2), :] = _pk(h2)
        return h2

    def p3b(i, h2):
        r0 = i * RB3
        z2 = _gelu(jnp.dot(h2, win_v[:, FH:], preferred_element_type=F32))
        z2_s[pl.ds(r0 // 2, RB3 // 2), :] = _pk(_ln(z2).astype(BF))

    if PH & 4:
        N3 = S // RB3
        P3D = 3
        h2s = {}
        for i in range(min(P3D, N3)):
            h2s[i] = p3a(i)
        for i in range(N3):
            if i + P3D < N3:
                h2s[i + P3D] = p3a(i + P3D)
            p3b(i, h2s.pop(i))

    oblocks = _out_blocks()

    def out_copy(j):
        r0, n = oblocks[j]
        return pltpu.make_async_copy(out_v.at[pl.ds(r0, n), :],
                                     out_hbm.at[0, pl.ds(r0, n), :], osems.at[j])

    brow_all = bsp_v[...].reshape(1, S).astype(F32)
    j = 0
    for i in range(S // RB4):
        r0 = i * RB4
        if PH & 8:
            h2 = _upk(h2_s[pl.ds(r0 // 2, RB4 // 2), :])
            z1 = _gelu(jnp.dot(h2, win_v[:, :FH], preferred_element_type=F32))
            gsp = jnp.dot(wsp_v[pl.ds(r0, RB4), :], _upk(z2_s[...]), preferred_element_type=F32)
            brow = brow_all[:, r0:r0 + RB4]
            bcol = jnp.broadcast_to(brow, (128, RB4)).T
            bfull = jnp.concatenate([bcol] * (FH // 128), axis=1)
            u = (z1 * (gsp + bfull)).astype(BF)
        while j < len(oblocks) and oblocks[j][0] < r0 + RB4:
            o0, n = oblocks[j]
            if PH & 8:
                y = jnp.dot(u[o0 - r0:o0 - r0 + n], wout_v[...], preferred_element_type=F32)
                out_v[pl.ds(o0, n), :] = (x1_s[pl.ds(o0, n), :] + mod_row(5) * y).astype(BF)
            out_copy(j).start()
            j += 1
    for j in range(len(oblocks)):
        out_copy(j).wait()


@jax.jit
def pallas_adaLN_cond__softmax_full_mha__mixer_gmlp__prompt_kernel(
    A_x, A_wqkv, A_wo, B_x, B_w_in, B_w_sp, B_b_sp, B_w_out, c, w_mod):
    del B_x
    any_spec = pl.BlockSpec(memory_space=pl.ANY)
    u32 = jnp.uint32
    scratch = [
        pltpu.VMEM((S, D), BF), pltpu.VMEM((D, 3 * D), BF), pltpu.VMEM((D, D), BF),
        pltpu.VMEM((D, 2 * FH), BF), pltpu.VMEM((S, S), BF), pltpu.VMEM((FH, D), BF),
        pltpu.VMEM((D, 6 * D), BF), pltpu.VMEM((1, D), BF), pltpu.VMEM((S,), BF),
        pltpu.VMEM((8, 6 * D), F32),
        pltpu.VMEM((H // 2, S // 2, 128), u32), pltpu.VMEM((4, S // 2, 128), u32),
        pltpu.VMEM((D // 2, S), u32), pltpu.VMEM((D // 2, S), u32),
        pltpu.VMEM((128, D), u32), pltpu.VMEM((D // 2, 256), u32),
        pltpu.VMEM((H, S), F32), pltpu.VMEM((H, RB1), F32),
        pltpu.VMEM((DH, 256, 128), F32), pltpu.VMEM((DH, 256, 128), F32),
        pltpu.VMEM((SPI, DH + 1, 8, TQ), F32),
        pltpu.VMEM((16, TQ), F32), pltpu.VMEM((8, TQ), F32), pltpu.VMEM((CK + 16 * SH, TQ), F32),
        pltpu.VMEM((S, TQ), F32), pltpu.VMEM((D // 2, S), u32),
        pltpu.VMEM((S, D), F32), pltpu.VMEM((S // 2, D), u32), pltpu.VMEM((S // 2, FH), u32),
        pltpu.VMEM((RB1, 3 * D), F32),
        pltpu.VMEM((S, D), BF),
        pltpu.SMEM((1,), jnp.int32),
        pltpu.SemaphoreType.DMA((22,)),
        pltpu.SemaphoreType.DMA((len(_out_blocks()),)),
    ]
    return pl.pallas_call(
        _kernel,
        out_shape=jax.ShapeDtypeStruct((1, S, D), BF),
        in_specs=[any_spec] * 9,
        out_specs=any_spec,
        scratch_shapes=scratch,
        compiler_params=pltpu.CompilerParams(vmem_limit_bytes=100 * 1024 * 1024),
    )(A_x, A_wqkv, A_wo, B_w_in, B_w_sp, B_b_sp, B_w_out, c, w_mod)
```

```python
import jax
import jax.numpy as jnp
import jax.experimental.pallas as pl
import jax.experimental.pallas.tpu as pltpu

S = 2048; D = 512; H = 32; DH = 16; FH = 896
EPS = 1e-5
LOG2E = 1.4426950408889634
QSCALE = (DH ** -0.5) * LOG2E

TQ = 512
CK = 128
NC = S // CK
NQ = S // TQ
T = H * NQ
RB1 = 512
RB3 = 512
RB4 = 512
SPI = 8
PH = 15
HPI = SPI // NQ
NG = 16
KU = 2
TU = 4 // KU
NPG = 3
KFD = 8
TD = 3
WS = 1
QF = 1
XS = 3
PLO = 0
KBE = 10
NOCSE = 0
DROP = 0
XP = 0
KEEPK = 0
P1O = 1
KEEP = 1
SH = 1
VB = 7
FORCE_FB = 0
L_MIN = 2.0 ** -64
L_MAX = 2.0 ** 20
OT = 128

BF = jnp.bfloat16
F32 = jnp.float32


def _pk(x):
    return pltpu.bitcast(x, jnp.uint32)


def _upk(x):
    return pltpu.bitcast(x, BF)


def _mo(x, n):
    return x if isinstance(x, int) else pl.multiple_of(x, n)


def _ln(x):
    m = jnp.mean(x, axis=-1, keepdims=True)
    xc = x - m
    v = jnp.mean(xc * xc, axis=-1, keepdims=True)
    return xc * jax.lax.rsqrt(v + EPS)


def _gelu(x):
    c0 = 0.7978845608028654
    inner = x * (c0 + (c0 * 0.044715) * (x * x))
    hx = 0.5 * x
    return hx + hx * jnp.tanh(inner)


def _dot_nt(a, w_ref, c0, n, tile):
    return [jnp.dot(a, w_ref[:, c0 + j:c0 + j + tile], preferred_element_type=F32)
            for j in range(0, n, tile)]


def _out_blocks():
    blocks = [(i * RB4, RB4) for i in range(S // RB4 - 1)]
    r0 = S - RB4
    blocks += [(r0 + j * OT, OT) for j in range(RB4 // OT)]
    return blocks


def _kernel(x_hbm, wqkv_hbm, wo_hbm, win_hbm, wsp_hbm, bsp_hbm, wout_hbm, c_hbm, wmod_hbm,
            out_hbm,
            x_v, wqkv_v, wo_v, win_v, wsp_v, wout_v, wmod_v, c_v, bsp_v, mod_v,
            k_s, ka_s, va_s, w_s, qf_s, kr_s, qt_s, vt_s, ksel_s, kt_s, qn_s, kn_s, kb0, kb1, qb_s, acc_s, l_s, car_s, s0, ot_s, x1_s, h2_s, z2_s, q0_s, out_v, z_s, sems, osems):
    z_s[0] = 0
    def cols(src, dst, c0, n, sem):
        return pltpu.make_async_copy(src.at[:, pl.ds(c0, n)], dst.at[:, pl.ds(c0, n)], sem)

    def xrows(r0, n, sem):
        return pltpu.make_async_copy(x_hbm.at[0, pl.ds(r0, n), :], x_v.at[pl.ds(r0, n), :], sem)

    NJ = 4
    JW = D // NJ
    cp_c = pltpu.make_async_copy(c_hbm, c_v, sems.at[0])
    cp_x0 = xrows(0, RB1, sems.at[1])
    cp_ms = [cols(wmod_hbm, wmod_v, j * JW, JW, sems.at[14 + j]) for j in range(NJ)]
    cp_mc = [cols(wmod_hbm, wmod_v, D + j * JW, JW, sems.at[18 + j]) for j in range(NJ)]
    cp_w = [pltpu.make_async_copy(wqkv_hbm.at[pl.ds(j * JW, JW), :], wqkv_v.at[pl.ds(j * JW, JW), :],
                                  sems.at[2 + j]) for j in range(NJ)]
    cp_x1 = xrows(RB1, RB1, sems.at[6])
    cp_x23 = xrows(2 * RB1, 2 * RB1, sems.at[7])
    cp_wmod_b = cols(wmod_hbm, wmod_v, 2 * D, 4 * D, sems.at[8])
    cp_wo = pltpu.make_async_copy(wo_hbm, wo_v, sems.at[9])
    cp_win = pltpu.make_async_copy(win_hbm, win_v, sems.at[10])
    cp_wsp = pltpu.make_async_copy(wsp_hbm, wsp_v, sems.at[11])
    cp_wout = pltpu.make_async_copy(wout_hbm, wout_v, sems.at[12])
    cp_bsp = pltpu.make_async_copy(bsp_hbm, bsp_v, sems.at[13])
    order = [cp_c, cp_x0, cp_ms[0], cp_mc[0]]
    for j in range(NJ):
        if j + 1 < NJ:
            order += [cp_ms[j + 1], cp_mc[j + 1]]
        order.append(cp_w[j])
    order.insert(len(order) - 1, cp_x1)
    order += [cp_x23, cp_wmod_b, cp_wo, cp_win, cp_wsp, cp_wout, cp_bsp]
    for cp in order:
        cp.start()

    cp_c.wait()
    cp_x0.wait()
    c = c_v[...].astype(F32)
    sc = (c * jax.nn.sigmoid(c)).astype(BF)
    sc = jnp.broadcast_to(sc, (16, D))

    def norm1(i):
        return _ln(x_v[pl.ds(i * RB1, RB1), :].astype(F32))

    def mod_row(j):
        return mod_v[0:1, j * D:(j + 1) * D]

    def modulate1(n):
        return (n * (1.0 + mod_row(1)) + mod_row(0)).astype(BF)

    n0 = norm1(0)

    def h0_piece(j):
        for c0 in (j * JW, D + j * JW):
            mod_v[:, c0:c0 + JW] = jnp.dot(sc, wmod_v[:, c0:c0 + JW], preferred_element_type=F32)[:8]
        sa = mod_v[0:1, j * JW:(j + 1) * JW]
        ca = mod_v[0:1, D + j * JW:D + (j + 1) * JW]
        return (n0[:, j * JW:(j + 1) * JW] * (1.0 + ca) + sa).astype(BF)

    cp_ms[0].wait()
    cp_mc[0].wait()
    hj = h0_piece(0)
    qkv0 = None
    for j in range(NJ):
        if j + 1 < NJ:
            cp_ms[j + 1].wait()
            cp_mc[j + 1].wait()
        if j == NJ - 2:
            cp_x1.wait()
        cp_w[j].wait()
        part = jnp.dot(hj, wqkv_v[j * JW:(j + 1) * JW, :], preferred_element_type=F32)
        if j == 0:
            q0_s[...] = part
        elif j + 1 < NJ:
            q0_s[...] = q0_s[...] + part
        else:
            qkv0 = q0_s[...] + part
        if j + 1 < NJ:
            hj = h0_piece(j + 1)
        if j >= NJ - 2:
            hr = RB1 // 2
            r1 = RB1 + (j - (NJ - 2)) * hr
            h2_s[pl.ds((j - (NJ - 2)) * hr // 2, hr // 2), :] = _pk(
                modulate1(_ln(x_v[pl.ds(r1, hr), :].astype(F32))))

    def head_sq(xt):
        xf = xt.astype(F32)
        return (xf * xf).reshape(H, DH, xt.shape[1]).sum(axis=1)

    def proj_k(i, h):
        k = qkv0[:, D:2 * D] if i == 0 else jnp.dot(h, wqkv_v[:, D:2 * D], preferred_element_type=F32)
        k = k.astype(BF)
        kp = _pk(k)
        for g in range(4):
            kr_s[g, pl.ds(i * RB1 // 2, RB1 // 2), :] = kp[:, g * 128:(g + 1) * 128]
        for t_ in range(RB1 // CK):
            ksel_s[pl.ds((i * (RB1 // CK) + t_) * 8, 8), :] = kp[t_ * 64 + 8 * VB:t_ * 64 + 8 * VB + 8]
        kn = head_sq(k.T)
        kn_s[...] = kn if i == 0 else jnp.maximum(kn_s[...], kn)

    lane = jax.lax.broadcasted_iota(jnp.int32, (8, 128), 1)
    one_pk = _pk(jnp.where(jax.lax.broadcasted_iota(jnp.int32, (16, 128), 1) == 2 * DH, 1.0, 0.0).astype(BF))

    def rot_k(i):
        n8 = RB1 // 16
        keep = jnp.broadcast_to((lane < 2 * DH)[None], (n8, 8, 128))
        fill = jnp.broadcast_to(one_pk[None], (n8, 8, 128))
        for g in range(4):
            kg = kr_s[g, pl.ds(i * RB1 // 2, RB1 // 2), :]
            for j in range(4):
                kj = kg if j == 0 else pltpu.roll(kg, 128 - 32 * j, axis=1)
                kj = jnp.where(keep, kj.reshape(n8, 8, 128), fill).reshape(RB1 // 2, 128)
                k_s[4 * g + j, pl.ds(i * RB1 // 2, RB1 // 2), :] = kj
                if g == 0 and j == 0:
                    ka_s[pl.ds(i * RB1 // 2, RB1 // 2), :] = kj

    def proj_q(i, h):
        q = qkv0[:, :D] if i == 0 else jnp.dot(h, wqkv_v[:, :D], preferred_element_type=F32)
        qt = (q * QSCALE).astype(BF).T
        qt_s[:, pl.ds(i * RB1, RB1)] = _pk(qt)
        qn_s[:, pl.ds(i * RB1, RB1)] = head_sq(qt)

    def make_ref(i):
        kmax = jnp.max(kn_s[...], axis=1, keepdims=True)
        bound = jnp.sqrt(qn_s[:, pl.ds(i * RB1, RB1)] * kmax) * (1.0 + 2.0 ** -6)
        qn_s[:, pl.ds(i * RB1, RB1)] = (-bound).astype(BF).astype(F32)

    def proj_v(i, h):
        v = qkv0[:, 2 * D:] if i == 0 else jnp.dot(h, wqkv_v[:, 2 * D:], preferred_element_type=F32)
        v = v.astype(BF)
        vp = _pk(v.T)
        vt_s[:, pl.ds(i * RB1, RB1)] = vp
        va_s[:, pl.ds(i * RB1, RB1)] = vp[:16]

    cp_x23.wait()
    NB1 = S // RB1
    hs = {1: _upk(h2_s[pl.ds(0, RB1 // 2), :])}
    proj_k(0, None)
    rot_k(0)
    proj_q(0, None)
    proj_v(0, None)
    if P1O == 0:
        for i in range(1, NB1):
            if i + 1 < NB1:
                hs[i + 1] = modulate1(norm1(i + 1))
            proj_k(i, hs[i])
            rot_k(i)
        kt_s[...] = _pk(_upk(ksel_s[...]).T)
        make_ref(0)
        for i in range(1, NB1):
            proj_q(i, hs[i])
            make_ref(i)
        for i in range(1, NB1):
            proj_v(i, hs[i])
    else:
        hs[2] = modulate1(norm1(2))
        proj_k(1, hs[1]); rot_k(1)
        proj_q(1, hs[1])
        hs[3] = modulate1(norm1(3))
        proj_k(2, hs[2]); rot_k(2)
        proj_k(3, hs[3]); rot_k(3)
        kt_s[...] = _pk(_upk(ksel_s[...]).T)
        make_ref(0); make_ref(1)
        proj_q(2, hs[2]); make_ref(2)
        proj_q(3, hs[3]); make_ref(3)
        for i in range(1, NB1):
            proj_v(i, hs[i])

    def q_rows(h, qb):
        return qt_s[pl.ds(_mo(h * 8, 8), 8), qb * TQ:(qb + 1) * TQ]

    def nref_row(h, qb):
        return qn_s[pl.ds(h, 1), qb * TQ:(qb + 1) * TQ]

    def clamp_h(h):
        return min(h, H - 1) if isinstance(h, int) else jnp.minimum(h, H - 1)

    row0 = jax.lax.broadcasted_iota(jnp.int32, (16, TQ), 0) == 0

    def make_w(h, qb, par, slot=None):
        aug = jnp.where(row0, jnp.broadcast_to(nref_row(h, qb), (16, TQ)), 0.0).astype(BF)
        q = _upk(q_rows(h, qb))
        if slot is not None and WS:
            w_s[slot] = _pk(jnp.concatenate([q, aug], axis=0))
            qa = _upk(w_s[slot])
            q, aug = qa[:DH], qa[DH:]
        z = jnp.zeros((DH, TQ), BF)
        return jnp.concatenate([z, q, aug] if par else [q, z, aug], axis=0)

    def stage_qf(h, qb, slot):
        qf_s[slot, 0:DH, :] = _upk(q_rows(h, qb)).astype(F32)
        qf_s[slot, DH:DH + 8, :] = jnp.broadcast_to(nref_row(h, qb), (8, TQ))

    def make_qb(h, qb, slot, ds_, tok=None, never=None, fslot=None):
        if fslot is None:
            qf = _upk(q_rows(h, qb)).astype(F32)
        for d in ds_:
            if fslot is not None:
                blk = qf_s[fslot, pl.ds(8 * (d // 8), 8), :]
                row = blk[d % 8:d % 8 + 1]
            else:
                row = nref_row(h, qb) if d == DH else qf[d:d + 1]
            val = jnp.broadcast_to(row, (8, TQ))
            if tok is not None:
                val = jnp.where(never, tok, val)
            qb_s[slot, d] = val

    def make_kb(h, j, kb, tok=None, never=None):
        d, half = j // 2, j % 2
        kt = _upk(kt_s[pl.ds(_mo(h * 8, 8), 8), half * 128:(half + 1) * 128]).astype(F32)
        row = jnp.broadcast_to(kt[d:d + 1], (8, 128))
        if tok is not None:
            row = jnp.where(never, tok[:, :128], row)
        val = jnp.concatenate([row] * 16, axis=0).T
        kb[d, pl.ds(half * 128, 128), :] = val
        if NOCSE == 2:
            kb[DH + d, pl.ds(half * 128, 128), :] = val
        return val[120:]

    if NG == NC:
        v_tiles = list(range(NC))
    else:
        v_tiles = sorted(set(NC - 1 - (k_ * (NC - 1)) // NG for k_ in range(NG))) if NG else []
    assert len(v_tiles) == NG

    def fence(val, on, never):
        return jnp.where(never, pltpu.bitcast(val, jnp.uint32), on)

    def v_unit(tile, ui, kb, slot, zi=0):
        per = 4 // TU
        kr = 16 * tile + 8 * KU * (ui // per)
        c0 = (ui % per) * TU * 128
        acc = None
        toks = []
        for d in range(DH):
            kk = kb[d + DH * (ui if NOCSE == 2 else 0), pl.ds(_mo(kr + zi, 8) if ui and NOCSE == 1 else kr, 8 * KU), :]
            kk = jnp.concatenate([kk] * TU, axis=1).reshape(KU, 8, TU * 128)
            t_ = kk * qb_s[slot, d, :, c0:c0 + TU * 128][None]
            acc = t_ + qb_s[slot, DH, :, c0:c0 + TU * 128][None] if acc is None else acc + t_
            if ((d + 1) * NPG) // DH != (d * NPG) // DH:
                ts = [acc[a_, :, b_ * 128:(b_ + 1) * 128] for a_ in range(KU) for b_ in range(TU)]
                toks.append((ts[0] + ts[1]) + (ts[2] + ts[3]))
        return acc.reshape(8 * KU, TU * 128), toks

    def tile_blocks(tile):
        return [j for j in reversed(range(8)) if not (tile in v_tiles and j == VB)]

    def v_rows(tile, kb, slot, zi):
        us = [v_unit(tile, ui, kb, slot, zi) for ui in range(2)]
        vrows = jnp.concatenate([us[0][0], us[1][0]], axis=1 if KU == 2 else 0)
        toks = us[0][1] + us[1][1]
        return vrows, toks[:len(toks) - DROP]

    def qk_run(w, h, items, toks, never, extra=()):
        parts = [ka_s[pl.ds(t_ * 64 + 8 * j, 8), :] for t_, j in items]
        n_ = len(parts) - PLO
        for i_, tk in enumerate(toks):
            j = PLO + (i_ * n_) // len(toks)
            parts[j] = fence(tk, parts[j], never[i_ % 2])
        if extra:
            val = extra[0]
            for v_ in extra[1:]:
                val = val + v_
            parts[XP] = fence(val, parts[XP], never[2])
        st = jnp.dot(_upk(jnp.concatenate(parts, axis=0))[:, :3 * DH], w, preferred_element_type=F32)
        return [st[16 * i_:16 * i_ + 16] for i_ in range(len(items))]

    def b_tile(hoff, ck, s, l, acc):
        p = jnp.exp2(s)
        if XS & 2:
            l = None if ck == 0 else l_s[...]
        for j in reversed(range(CK // 16)):
            pr = p[16 * j:16 * j + 8] + p[16 * j + 8:16 * j + 16]
            l = pr if l is None else l + pr
        if XS & 2:
            l_s[...] = l
        vc = _upk(va_s[pl.ds(hoff * 8, 8), pl.ds(ck * CK, CK)])
        pv = jnp.dot(vc, p.astype(BF), preferred_element_type=F32)
        if ck == 0:
            acc = pv
        else:
            acc = (acc_s[...] if XS & 1 else acc) + pv
        if XS & 1:
            acc_s[...] = acc
        return l, acc

    def fin(h, qb, l, acc):
        lsum = l.sum(axis=0, keepdims=True)
        o = acc * (1.0 / lsum)
        ot_s[pl.ds(_mo(h * 8, 8), 8), qb * TQ:(qb + 1) * TQ] = _pk(o.astype(BF))
        return lsum

    kbs = (kb0, kb1)
    kb_sched = [[] for _ in range(NQ * NC)]
    for kj in range(2 * DH):
        kb_sched[(kj * (NQ * NC - KBE)) // (2 * DH)].append(kj)

    car_mx = [(0, j) for j in tile_blocks(0)] + [(1, j) for j in tile_blocks(1)[:SH]]
    car_items = car_mx + ([(0, VB)] if 0 in v_tiles else [])

    def run_steps(hp0, state, never, zi):
        h0 = 2 * hp0
        lo, hi = state
        pend = {}
        lh = []
        sc_ = {}
        for i_, (t_, j) in enumerate(car_items):
            sc_[(0, t_, j)] = car_s[pl.ds(16 * i_, 16), :]
        ws = {}

        def step_hq(s_):
            return clamp_h(h0 + s_ // NQ) if s_ >= SPI else h0 + s_ // NQ, s_ % NQ

        def pair_of(s_):
            p_ = hp0 + s_ // (2 * NQ)
            return jnp.minimum(p_, H // 2 - 1) if s_ >= SPI else p_

        def get_w(s_):
            if s_ not in ws:
                ws[s_] = make_w(*step_hq(s_), (s_ // NQ) % 2, s_ % 2)
            return ws[s_]

        for s_ in range(SPI):
            h, qb = step_hq(s_)
            kb_use = kbs[(s_ // NQ) % 2]
            kb_make = kbs[1 - (s_ // NQ) % 2]
            l = acc = None
            for c_ in range(NC):
                gt = s_ * NC + c_
                g1, g2 = gt + 1, gt + 2
                it1 = [(g1 // NC, g1 % NC, j) for j in tile_blocks(g1 % NC)[SH:]]
                it2 = [(g2 // NC, g2 % NC, j) for j in tile_blocks(g2 % NC)[:SH]]
                toks = []
                if (g1 % NC) in v_tiles:
                    s1 = g1 // NC
                    sc_[(s1, g1 % NC, VB)], toks = v_rows(g1 % NC, kbs[(s1 // NQ) % 2], s1 % SPI, zi)
                runs = [it1 + it2] if g1 // NC == g2 // NC else [it1, it2]
                for ri, its in enumerate(runs):
                    if not its:
                        continue
                    sr = its[0][0]
                    outs = qk_run(get_w(sr), pair_of(sr), [(t_, j) for _, t_, j in its],
                                  toks if ri == 0 else [], never,
                                  pend.pop(gt, ()) if ri == 0 else ())
                    sc_.update(zip(its, outs))
                    for sr_, t_, j in its:
                        if sr_ == SPI - 1:
                            r_ = t_ * 64 + 8 * j
                            ka_s[pl.ds(r_, 8), :] = k_s[pair_of(SPI), pl.ds(r_, 8), :]
                tok = lh[-TD] if len(lh) >= TD else None
                if s_ >= 1:
                    un = s_ - 1 + SPI
                    ds_ = [c_, DH] if c_ == NC - 1 else [c_]
                    if QF and c_ == 0:
                        stage_qf(clamp_h(h0 + un // NQ), un % NQ, s_ % 2)
                    make_qb(clamp_h(h0 + un // NQ), un % NQ, s_ - 1, ds_, tok, never[0],
                            s_ % 2 if QF else None)
                ht = (s_ % NQ) * NC + c_
                for kj in kb_sched[ht]:
                    val = make_kb(clamp_h(h + 1), kj, kb_make, tok, never[0])
                    if gt + KFD < SPI * NC:
                        pend.setdefault(gt + KFD, []).append(val)
                s_cur = jnp.concatenate([sc_.pop((s_, c_, j)) for j in range(8)], axis=0)
                l, acc = b_tile((s_ // NQ) % 2, c_, s_cur, l, acc)
                if s_ % NQ == NQ - 1:
                    hv = clamp_h(h + 2)
                    va_s[pl.ds(((s_ // NQ) % 2) * 8, 8), pl.ds(c_ * CK, CK)] = (
                        vt_s[pl.ds(_mo(hv * 8, 8), 8), pl.ds(c_ * CK, CK)])
                lh.append(l)
            lsum = fin(h, qb, l, acc)
            lo = jnp.minimum(lo, lsum)
            hi = jnp.maximum(hi, lsum)
        for i_, (t_, j) in enumerate(car_items):
            car_s[pl.ds(16 * i_, 16), :] = sc_.pop((SPI, t_, j))
        un = 2 * SPI - 1
        make_qb(clamp_h(h0 + un // NQ), un % NQ, SPI - 1, range(DH + 1))
        return lo, hi

    for u_ in range(SPI):
        make_qb(u_ // NQ, u_ % NQ, u_, range(DH + 1))
    for j in range(2 * DH):
        make_kb(0, j, kb0)
    pro = qk_run(make_w(0, 0, 0), 0, car_mx, [], None)
    if 0 in v_tiles:
        pro = pro + [v_rows(0, kb0, 0, 0)[0]]
    for i_, o_ in enumerate(pro):
        car_s[pl.ds(16 * i_, 16), :] = o_

    def p2_body(i, state):
        return run_steps((HPI // 2) * i, state, (i < 0, i < -1, i < -2), (i // 4096) * 8)

    one = jnp.ones((1, TQ), F32)
    lo, hi = jax.lax.fori_loop(0, (T // SPI), p2_body, (one, one))

    cp_wmod_b.wait()
    cp_wo.wait()
    cp_win.wait()
    cp_wsp.wait()
    cp_wout.wait()
    cp_bsp.wait()

    ok = jnp.logical_and(lo >= L_MIN, hi <= L_MAX)
    n_bad = jnp.sum(jnp.where(ok, 0.0, 1.0))

    @pl.when(jnp.logical_or(n_bad > 0.0, FORCE_FB > 0))
    def _():
        def exact_step(t, carry):
            h = t // NQ
            c0 = pl.multiple_of((t % NQ) * TQ, TQ)
            r8 = pl.multiple_of(h * 8, 8)
            q = qt_s[pl.ds(r8, 8), pl.ds(c0, TQ)]
            zq = jnp.zeros_like(q)
            odd = h % 2 == 1
            w = _upk(jnp.concatenate([jnp.where(odd, zq, q), jnp.where(odd, q, zq)], axis=0))
            s0[...] = jnp.dot(_upk(k_s[h // 2])[:, :2 * DH], w, preferred_element_type=F32)
            st = s0[...]
            p = jnp.exp2(st - jnp.max(st, axis=0, keepdims=True))
            lsum = jnp.sum(p, axis=0, keepdims=True)
            o = jnp.dot(_upk(vt_s[pl.ds(r8, 8), :]), p.astype(BF), preferred_element_type=F32)
            ot_s[pl.ds(r8, 8), pl.ds(c0, TQ)] = _pk((o * (1.0 / lsum)).astype(BF))
            return carry

        if KEEP:
            s0[0:16, :] = acc_s[...]
            s0[16:24, :] = l_s[...]
            s0[32:80, :] = qf_s[...].reshape(48, TQ)
            s0[80:112, :] = pltpu.bitcast(w_s[...].reshape(32, TQ), F32)
        if KEEPK:
            for d in range(2 * DH if NOCSE == 2 else DH):
                s0[pl.ds(256 * (d // 4), 256), (d % 4) * 128:(d % 4 + 1) * 128] = kb1[d]

        jax.lax.fori_loop(0, T, exact_step, 0)

    mod_v[:, 2 * D:] = jnp.dot(sc, wmod_v[:, 2 * D:], preferred_element_type=F32)[:8]

    def p3a(i):
        r0 = i * RB3
        ot = _upk(ot_s[:, pl.ds(r0, RB3)])
        attn = jnp.dot(ot.T, wo_v[...], preferred_element_type=F32)
        x1 = x_v[pl.ds(r0, RB3), :].astype(F32) + mod_row(2) * attn
        x1_s[pl.ds(r0, RB3), :] = x1
        h2 = (_ln(x1) * (1.0 + mod_row(4)) + mod_row(3)).astype(BF)
        h2_s[pl.ds(r0 // 2, RB3 // 2), :] = _pk(h2)
        return h2

    def p3b(i, h2):
        r0 = i * RB3
        z2 = _gelu(jnp.dot(h2, win_v[:, FH:], preferred_element_type=F32))
        z2_s[pl.ds(r0 // 2, RB3 // 2), :] = _pk(_ln(z2).astype(BF))

    if PH & 4:
        N3 = S // RB3
        P3D = 3
        h2s = {}
        for i in range(min(P3D, N3)):
            h2s[i] = p3a(i)
        for i in range(N3):
            if i + P3D < N3:
                h2s[i + P3D] = p3a(i + P3D)
            p3b(i, h2s.pop(i))

    oblocks = _out_blocks()

    def out_copy(j):
        r0, n = oblocks[j]
        return pltpu.make_async_copy(out_v.at[pl.ds(r0, n), :],
                                     out_hbm.at[0, pl.ds(r0, n), :], osems.at[j])

    brow_all = bsp_v[...].reshape(1, S).astype(F32)
    j = 0
    for i in range(S // RB4):
        r0 = i * RB4
        if PH & 8:
            h2 = _upk(h2_s[pl.ds(r0 // 2, RB4 // 2), :])
            z1 = _gelu(jnp.dot(h2, win_v[:, :FH], preferred_element_type=F32))
            gsp = jnp.dot(wsp_v[pl.ds(r0, RB4), :], _upk(z2_s[...]), preferred_element_type=F32)
            brow = brow_all[:, r0:r0 + RB4]
            bcol = jnp.broadcast_to(brow, (128, RB4)).T
            bfull = jnp.concatenate([bcol] * (FH // 128), axis=1)
            u = (z1 * (gsp + bfull)).astype(BF)
        while j < len(oblocks) and oblocks[j][0] < r0 + RB4:
            o0, n = oblocks[j]
            if PH & 8:
                y = jnp.dot(u[o0 - r0:o0 - r0 + n], wout_v[...], preferred_element_type=F32)
                out_v[pl.ds(o0, n), :] = (x1_s[pl.ds(o0, n), :] + mod_row(5) * y).astype(BF)
            out_copy(j).start()
            j += 1
    for j in range(len(oblocks)):
        out_copy(j).wait()


@jax.jit
def pallas_adaLN_cond__softmax_full_mha__mixer_gmlp__prompt_kernel(
    A_x, A_wqkv, A_wo, B_x, B_w_in, B_w_sp, B_b_sp, B_w_out, c, w_mod):
    del B_x
    any_spec = pl.BlockSpec(memory_space=pl.ANY)
    u32 = jnp.uint32
    scratch = [
        pltpu.VMEM((S, D), BF), pltpu.VMEM((D, 3 * D), BF), pltpu.VMEM((D, D), BF),
        pltpu.VMEM((D, 2 * FH), BF), pltpu.VMEM((S, S), BF), pltpu.VMEM((FH, D), BF),
        pltpu.VMEM((D, 6 * D), BF), pltpu.VMEM((1, D), BF), pltpu.VMEM((S,), BF),
        pltpu.VMEM((8, 6 * D), F32),
        pltpu.VMEM((H // 2, S // 2, 128), u32),
        pltpu.VMEM((S // 2, 128), u32), pltpu.VMEM((16, S), u32),
        pltpu.VMEM((2, 16, TQ), u32), pltpu.VMEM((2, 24, TQ), F32),
        pltpu.VMEM((4, S // 2, 128), u32),
        pltpu.VMEM((D // 2, S), u32), pltpu.VMEM((D // 2, S), u32),
        pltpu.VMEM((128, D), u32), pltpu.VMEM((D // 2, 256), u32),
        pltpu.VMEM((H, S), F32), pltpu.VMEM((H, RB1), F32),
        pltpu.VMEM((2 * DH, 256, 128), F32), pltpu.VMEM((2 * DH, 256, 128), F32),
        pltpu.VMEM((SPI, DH + 1, 8, TQ), F32),
        pltpu.VMEM((16, TQ), F32), pltpu.VMEM((8, TQ), F32), pltpu.VMEM((CK + 16 * SH, TQ), F32),
        pltpu.VMEM((S, TQ), F32), pltpu.VMEM((D // 2, S), u32),
        pltpu.VMEM((S, D), F32), pltpu.VMEM((S // 2, D), u32), pltpu.VMEM((S // 2, FH), u32),
        pltpu.VMEM((RB1, 3 * D), F32),
        pltpu.VMEM((S, D), BF),
        pltpu.SMEM((1,), jnp.int32),
        pltpu.SemaphoreType.DMA((22,)),
        pltpu.SemaphoreType.DMA((len(_out_blocks()),)),
    ]
    return pl.pallas_call(
        _kernel,
        out_shape=jax.ShapeDtypeStruct((1, S, D), BF),
        in_specs=[any_spec] * 9,
        out_specs=any_spec,
        scratch_shapes=scratch,
        compiler_params=pltpu.CompilerParams(vmem_limit_bytes=100 * 1024 * 1024),
    )(A_x, A_wqkv, A_wo, B_w_in, B_w_sp, B_b_sp, B_w_out, c, w_mod)
```

```python
import jax
import jax.numpy as jnp
import jax.experimental.pallas as pl
import jax.experimental.pallas.tpu as pltpu

S = 2048
D = 512
H = 32
DH = 16
FH = 896
EPS = 1e-5
LOG2E = 1.4426950408889634
QSCALE = (DH ** -0.5) * LOG2E

TQ = 512
CK = 128
NC = S // CK
NQ = S // TQ
T = H * NQ
SPI = 2 * NQ
RB = 512
NB = S // RB
NJ = 4
JW = D // NJ
OT = 128

VB = 7
NPG = 3
SH = 1
TD = 3
KFD = 6
KBE = 10
L_MIN = 2.0 ** -64
L_MAX = 2.0 ** 20

BF = jnp.bfloat16
F32 = jnp.float32
U32 = jnp.uint32


def _pk(x):
    return pltpu.bitcast(x, U32)


def _upk(x):
    return pltpu.bitcast(x, BF)


def _mo(x, n):
    return x if isinstance(x, int) else pl.multiple_of(x, n)


def _dot(a, b):
    return jnp.dot(a, b, preferred_element_type=F32)


def _ln(x):
    m = jnp.mean(x, axis=-1, keepdims=True)
    xc = x - m
    v = jnp.mean(xc * xc, axis=-1, keepdims=True)
    return xc * jax.lax.rsqrt(v + EPS)


def _gelu(x):
    c0 = 0.7978845608028654
    inner = x * (c0 + (c0 * 0.044715) * (x * x))
    hx = 0.5 * x
    return hx + hx * jnp.tanh(inner)


_OUT_BLOCKS = ([(i * RB, RB) for i in range(NB - 1)]
               + [(S - RB + j * OT, OT) for j in range(RB // OT)])


def _kernel(x_hbm, wqkv_hbm, wo_hbm, win_hbm, wsp_hbm, bsp_hbm, wout_hbm, c_hbm, wmod_hbm,
            out_hbm,
            x_v, wqkv_v, wo_v, win_v, wsp_v, wout_v, wmod_v, c_v, bsp_v, mod_v,
            k_s, ka_s, va_s, w_s, qf_s, kr_s, qt_s, vt_s, ksel_s, kt_s, qn_s, kn_s, kb0, kb1,
            qb_s, acc_s, l_s, car_s, s0, ot_s, x1_s, h2_s, z2_s, q0_s, out_v, sems, osems):
    def cols(src, dst, c0, n, sem):
        return pltpu.make_async_copy(src.at[:, pl.ds(c0, n)], dst.at[:, pl.ds(c0, n)], sem)

    def xrows(r0, n, sem):
        return pltpu.make_async_copy(x_hbm.at[0, pl.ds(r0, n), :], x_v.at[pl.ds(r0, n), :], sem)

    cp_c = pltpu.make_async_copy(c_hbm, c_v, sems.at[0])
    cp_x0 = xrows(0, RB, sems.at[1])
    cp_ms = [cols(wmod_hbm, wmod_v, j * JW, JW, sems.at[14 + j]) for j in range(NJ)]
    cp_mc = [cols(wmod_hbm, wmod_v, D + j * JW, JW, sems.at[18 + j]) for j in range(NJ)]
    cp_w = [pltpu.make_async_copy(wqkv_hbm.at[pl.ds(j * JW, JW), :],
                                  wqkv_v.at[pl.ds(j * JW, JW), :], sems.at[2 + j])
            for j in range(NJ)]
    cp_x1 = xrows(RB, RB, sems.at[6])
    cp_x23 = xrows(2 * RB, 2 * RB, sems.at[7])
    late = [cols(wmod_hbm, wmod_v, 2 * D, 4 * D, sems.at[8]),
            pltpu.make_async_copy(wo_hbm, wo_v, sems.at[9]),
            pltpu.make_async_copy(win_hbm, win_v, sems.at[10]),
            pltpu.make_async_copy(wsp_hbm, wsp_v, sems.at[11]),
            pltpu.make_async_copy(wout_hbm, wout_v, sems.at[12]),
            pltpu.make_async_copy(bsp_hbm, bsp_v, sems.at[13])]
    order = [cp_c, cp_x0, cp_ms[0], cp_mc[0]]
    for j in range(NJ):
        if j + 1 < NJ:
            order += [cp_ms[j + 1], cp_mc[j + 1]]
        else:
            order.append(cp_x1)
        order.append(cp_w[j])
    for cp in order + [cp_x23] + late:
        cp.start()

    cp_c.wait()
    cp_x0.wait()
    c = c_v[...].astype(F32)
    sc = (c * jax.nn.sigmoid(c)).astype(BF)
    sc = jnp.broadcast_to(sc, (16, D))

    def norm1(i):
        return _ln(x_v[pl.ds(i * RB, RB), :].astype(F32))

    def mod_row(j):
        return mod_v[0:1, j * D:(j + 1) * D]

    def modulate1(n):
        return (n * (1.0 + mod_row(1)) + mod_row(0)).astype(BF)

    n0 = norm1(0)

    def h0_piece(j):
        for c0 in (j * JW, D + j * JW):
            mod_v[:, c0:c0 + JW] = _dot(sc, wmod_v[:, c0:c0 + JW])[:8]
        sa = mod_v[0:1, j * JW:(j + 1) * JW]
        ca = mod_v[0:1, D + j * JW:D + (j + 1) * JW]
        return (n0[:, j * JW:(j + 1) * JW] * (1.0 + ca) + sa).astype(BF)

    cp_ms[0].wait()
    cp_mc[0].wait()
    hj = h0_piece(0)
    qkv0 = None
    for j in range(NJ):
        if j + 1 < NJ:
            cp_ms[j + 1].wait()
            cp_mc[j + 1].wait()
        if j == NJ - 2:
            cp_x1.wait()
        cp_w[j].wait()
        part = _dot(hj, wqkv_v[j * JW:(j + 1) * JW, :])
        if j == 0:
            q0_s[...] = part
        elif j + 1 < NJ:
            q0_s[...] = q0_s[...] + part
        else:
            qkv0 = q0_s[...] + part
        if j + 1 < NJ:
            hj = h0_piece(j + 1)
        if j >= NJ - 2:
            hr = RB // 2
            half = j - (NJ - 2)
            h2_s[pl.ds(half * hr // 2, hr // 2), :] = _pk(
                modulate1(_ln(x_v[pl.ds(RB + half * hr, hr), :].astype(F32))))

    def head_sq(xt):
        xf = xt.astype(F32)
        return (xf * xf).reshape(H, DH, xt.shape[1]).sum(axis=1)

    def proj_k(i, h):
        k = qkv0[:, D:2 * D] if i == 0 else _dot(h, wqkv_v[:, D:2 * D])
        k = k.astype(BF)
        kp = _pk(k)
        for g in range(4):
            kr_s[g, pl.ds(i * RB // 2, RB // 2), :] = kp[:, g * 128:(g + 1) * 128]
        for t_ in range(RB // CK):
            ksel_s[pl.ds((i * (RB // CK) + t_) * 8, 8), :] = (
                kp[t_ * 64 + 8 * VB:t_ * 64 + 8 * VB + 8])
        kn = head_sq(k.T)
        kn_s[...] = kn if i == 0 else jnp.maximum(kn_s[...], kn)

    lane = jax.lax.broadcasted_iota(jnp.int32, (8, 128), 1)
    one_pk = _pk(jnp.where(jax.lax.broadcasted_iota(jnp.int32, (16, 128), 1) == 2 * DH,
                           1.0, 0.0).astype(BF))

    def rot_k(i):
        n8 = RB // 16
        keep = jnp.broadcast_to((lane < 2 * DH)[None], (n8, 8, 128))
        fill = jnp.broadcast_to(one_pk[None], (n8, 8, 128))
        for g in range(4):
            kg = kr_s[g, pl.ds(i * RB // 2, RB // 2), :]
            for j in range(4):
                kj = kg if j == 0 else pltpu.roll(kg, 128 - 32 * j, axis=1)
                kj = jnp.where(keep, kj.reshape(n8, 8, 128), fill).reshape(RB // 2, 128)
                k_s[4 * g + j, pl.ds(i * RB // 2, RB // 2), :] = kj
                if g == 0 and j == 0:
                    ka_s[pl.ds(i * RB // 2, RB // 2), :] = kj

    def proj_q(i, h):
        q = qkv0[:, :D] if i == 0 else _dot(h, wqkv_v[:, :D])
        qt = (q * QSCALE).astype(BF).T
        qt_s[:, pl.ds(i * RB, RB)] = _pk(qt)
        qn_s[:, pl.ds(i * RB, RB)] = head_sq(qt)

    def make_ref(i):
        kmax = jnp.max(kn_s[...], axis=1, keepdims=True)
        bound = jnp.sqrt(qn_s[:, pl.ds(i * RB, RB)] * kmax) * (1.0 + 2.0 ** -6)
        qn_s[:, pl.ds(i * RB, RB)] = (-bound).astype(BF).astype(F32)

    def proj_v(i, h):
        v = qkv0[:, 2 * D:] if i == 0 else _dot(h, wqkv_v[:, 2 * D:])
        vp = _pk(v.astype(BF).T)
        vt_s[:, pl.ds(i * RB, RB)] = vp
        va_s[:, pl.ds(i * RB, RB)] = vp[:16]

    cp_x23.wait()
    hs = {1: _upk(h2_s[pl.ds(0, RB // 2), :])}
    proj_k(0, None)
    rot_k(0)
    proj_q(0, None)
    proj_v(0, None)
    hs[2] = modulate1(norm1(2))
    proj_k(1, hs[1])
    rot_k(1)
    proj_q(1, hs[1])
    hs[3] = modulate1(norm1(3))
    proj_k(2, hs[2])
    rot_k(2)
    proj_k(3, hs[3])
    rot_k(3)
    kt_s[...] = _pk(_upk(ksel_s[...]).T)
    make_ref(0)
    make_ref(1)
    proj_q(2, hs[2])
    make_ref(2)
    proj_q(3, hs[3])
    make_ref(3)
    for i in range(1, NB):
        proj_v(i, hs[i])

    def q_rows(h, qb):
        return qt_s[pl.ds(_mo(h * 8, 8), 8), qb * TQ:(qb + 1) * TQ]

    def nref_row(h, qb):
        return qn_s[pl.ds(h, 1), qb * TQ:(qb + 1) * TQ]

    def clamp_h(h):
        return min(h, H - 1) if isinstance(h, int) else jnp.minimum(h, H - 1)

    row0 = jax.lax.broadcasted_iota(jnp.int32, (16, TQ), 0) == 0

    def make_w(h, qb, par, slot=None):
        aug = jnp.where(row0, jnp.broadcast_to(nref_row(h, qb), (16, TQ)), 0.0).astype(BF)
        q = _upk(q_rows(h, qb))
        if slot is not None:
            w_s[slot] = _pk(jnp.concatenate([q, aug], axis=0))
            qa = _upk(w_s[slot])
            q, aug = qa[:DH], qa[DH:]
        z = jnp.zeros((DH, TQ), BF)
        return jnp.concatenate([z, q, aug] if par else [q, z, aug], axis=0)

    def stage_qf(h, qb, slot):
        qf_s[slot, 0:DH, :] = _upk(q_rows(h, qb)).astype(F32)
        qf_s[slot, DH:DH + 8, :] = jnp.broadcast_to(nref_row(h, qb), (8, TQ))

    def make_qb(h, qb, slot, ds_, tok=None, never=None, fslot=None):
        if fslot is None:
            qf = _upk(q_rows(h, qb)).astype(F32)
        for d in ds_:
            if fslot is not None:
                blk = qf_s[fslot, pl.ds(8 * (d // 8), 8), :]
                row = blk[d % 8:d % 8 + 1]
            else:
                row = nref_row(h, qb) if d == DH else qf[d:d + 1]
            val = jnp.broadcast_to(row, (8, TQ))
            if tok is not None:
                val = jnp.where(never, tok, val)
            qb_s[slot, d] = val

    def make_kb(h, j, kb, tok=None, never=None):
        d, half = j // 2, j % 2
        kt = _upk(kt_s[pl.ds(_mo(h * 8, 8), 8), half * 128:(half + 1) * 128]).astype(F32)
        row = jnp.broadcast_to(kt[d:d + 1], (8, 128))
        if tok is not None:
            row = jnp.where(never, tok[:, :128], row)
        val = jnp.concatenate([row] * 16, axis=0).T
        kb[d, pl.ds(half * 128, 128), :] = val
        return val[120:]

    def fence(val, on, never):
        return jnp.where(never, pltpu.bitcast(val, U32), on)

    def v_unit(tile, ui, kb, slot):
        c0 = ui * 256
        acc = None
        toks = []
        for d in range(DH):
            kk = kb[d, pl.ds(16 * tile, 16), :]
            kk = jnp.concatenate([kk] * 2, axis=1).reshape(2, 8, 256)
            t_ = kk * qb_s[slot, d, :, c0:c0 + 256][None]
            acc = t_ + qb_s[slot, DH, :, c0:c0 + 256][None] if acc is None else acc + t_
            if ((d + 1) * NPG) // DH != (d * NPG) // DH:
                ts = [acc[a_, :, b_ * 128:(b_ + 1) * 128] for a_ in range(2) for b_ in range(2)]
                toks.append((ts[0] + ts[1]) + (ts[2] + ts[3]))
        return acc.reshape(16, 256), toks

    def v_rows(tile, kb, slot):
        us = [v_unit(tile, ui, kb, slot) for ui in range(2)]
        return jnp.concatenate([us[0][0], us[1][0]], axis=1), us[0][1] + us[1][1]

    mx_blocks = [j for j in reversed(range(8)) if j != VB]

    def qk_run(w, items, toks, never, extra=()):
        parts = [ka_s[pl.ds(t_ * 64 + 8 * j, 8), :] for t_, j in items]
        for i_, tk in enumerate(toks):
            j = (i_ * len(parts)) // len(toks)
            parts[j] = fence(tk, parts[j], never[i_ % 2])
        if extra:
            val = extra[0]
            for v_ in extra[1:]:
                val = val + v_
            parts[0] = fence(val, parts[0], never[2])
        st = _dot(_upk(jnp.concatenate(parts, axis=0))[:, :3 * DH], w)
        return [st[16 * i_:16 * i_ + 16] for i_ in range(len(items))]

    def b_tile(hoff, ck, s):
        p = jnp.exp2(s)
        l = None if ck == 0 else l_s[...]
        for j in reversed(range(CK // 16)):
            pr = p[16 * j:16 * j + 8] + p[16 * j + 8:16 * j + 16]
            l = pr if l is None else l + pr
        l_s[...] = l
        vc = _upk(va_s[pl.ds(hoff * 8, 8), pl.ds(ck * CK, CK)])
        pv = _dot(vc, p.astype(BF))
        acc = pv if ck == 0 else acc_s[...] + pv
        acc_s[...] = acc
        return l, acc

    def fin(h, qb, l, acc):
        lsum = l.sum(axis=0, keepdims=True)
        o = acc * (1.0 / lsum)
        ot_s[pl.ds(_mo(h * 8, 8), 8), qb * TQ:(qb + 1) * TQ] = _pk(o.astype(BF))
        return lsum

    kbs = (kb0, kb1)
    kb_sched = [[] for _ in range(NQ * NC)]
    for kj in range(2 * DH):
        kb_sched[(kj * (NQ * NC - KBE)) // (2 * DH)].append(kj)

    car_mx = [(0, j) for j in mx_blocks] + [(1, j) for j in mx_blocks[:SH]]
    car_items = car_mx + [(0, VB)]

    def run_steps(pair, state, never):
        h0 = 2 * pair
        lo, hi = state
        pend = {}
        lh = []
        sc_ = {}
        for i_, (t_, j) in enumerate(car_items):
            sc_[(0, t_, j)] = car_s[pl.ds(16 * i_, 16), :]
        ws = {}
        next_pair = jnp.minimum(pair + 1, H // 2 - 1)

        def step_hq(s_):
            return clamp_h(h0 + s_ // NQ) if s_ >= SPI else h0 + s_ // NQ, s_ % NQ

        def get_w(s_):
            if s_ not in ws:
                ws[s_] = make_w(*step_hq(s_), (s_ // NQ) % 2, s_ % 2)
            return ws[s_]

        for s_ in range(SPI):
            h, qb = step_hq(s_)
            kb_make = kbs[1 - (s_ // NQ) % 2]
            for c_ in range(NC):
                gt = s_ * NC + c_
                g1, g2 = gt + 1, gt + 2
                it1 = [(g1 // NC, g1 % NC, j) for j in mx_blocks[SH:]]
                it2 = [(g2 // NC, g2 % NC, j) for j in mx_blocks[:SH]]
                s1 = g1 // NC
                sc_[(s1, g1 % NC, VB)], toks = v_rows(g1 % NC, kbs[(s1 // NQ) % 2], s1 % SPI)
                runs = [it1 + it2] if g1 // NC == g2 // NC else [it1, it2]
                for ri, its in enumerate(runs):
                    outs = qk_run(get_w(its[0][0]), [(t_, j) for _, t_, j in its],
                                  toks if ri == 0 else [], never,
                                  pend.pop(gt, ()) if ri == 0 else ())
                    sc_.update(zip(its, outs))
                    for sr_, t_, j in its:
                        if sr_ == SPI - 1:
                            r_ = t_ * 64 + 8 * j
                            ka_s[pl.ds(r_, 8), :] = k_s[next_pair, pl.ds(r_, 8), :]
                tok = lh[-TD] if len(lh) >= TD else None
                if s_ >= 1:
                    un = s_ - 1 + SPI
                    ds_ = [c_, DH] if c_ == NC - 1 else [c_]
                    if c_ == 0:
                        stage_qf(clamp_h(h0 + un // NQ), un % NQ, s_ % 2)
                    make_qb(clamp_h(h0 + un // NQ), un % NQ, s_ - 1, ds_, tok, never[0], s_ % 2)
                for kj in kb_sched[(s_ % NQ) * NC + c_]:
                    val = make_kb(clamp_h(h + 1), kj, kb_make, tok, never[0])
                    if gt + KFD < SPI * NC:
                        pend.setdefault(gt + KFD, []).append(val)
                s_cur = jnp.concatenate([sc_.pop((s_, c_, j)) for j in range(8)], axis=0)
                l, acc = b_tile((s_ // NQ) % 2, c_, s_cur)
                if s_ % NQ == NQ - 1:
                    hv = clamp_h(h + 2)
                    va_s[pl.ds(((s_ // NQ) % 2) * 8, 8), pl.ds(c_ * CK, CK)] = (
                        vt_s[pl.ds(_mo(hv * 8, 8), 8), pl.ds(c_ * CK, CK)])
                lh.append(l)
            lsum = fin(h, qb, l, acc)
            lo = jnp.minimum(lo, lsum)
            hi = jnp.maximum(hi, lsum)
        for i_, (t_, j) in enumerate(car_items):
            car_s[pl.ds(16 * i_, 16), :] = sc_.pop((SPI, t_, j))
        un = 2 * SPI - 1
        make_qb(clamp_h(h0 + un // NQ), un % NQ, SPI - 1, range(DH + 1))
        return lo, hi

    for u_ in range(SPI):
        make_qb(u_ // NQ, u_ % NQ, u_, range(DH + 1))
    for j in range(2 * DH):
        make_kb(0, j, kb0)
    pro = qk_run(make_w(0, 0, 0), car_mx, [], None) + [v_rows(0, kb0, 0)[0]]
    for i_, o_ in enumerate(pro):
        car_s[pl.ds(16 * i_, 16), :] = o_

    def p2_body(i, state):
        return run_steps(i, state, (i < 0, i < -1, i < -2))

    one = jnp.ones((1, TQ), F32)
    lo, hi = jax.lax.fori_loop(0, T // SPI, p2_body, (one, one))

    for cp in late:
        cp.wait()

    ok = jnp.logical_and(lo >= L_MIN, hi <= L_MAX)
    n_bad = jnp.sum(jnp.where(ok, 0.0, 1.0))

    @pl.when(n_bad > 0.0)
    def _():
        def exact_step(t, carry):
            h = t // NQ
            c0 = pl.multiple_of((t % NQ) * TQ, TQ)
            r8 = pl.multiple_of(h * 8, 8)
            q = qt_s[pl.ds(r8, 8), pl.ds(c0, TQ)]
            zq = jnp.zeros_like(q)
            odd = h % 2 == 1
            w = _upk(jnp.concatenate([jnp.where(odd, zq, q), jnp.where(odd, q, zq)], axis=0))
            s0[...] = _dot(_upk(k_s[h // 2])[:, :2 * DH], w)
            st = s0[...]
            p = jnp.exp2(st - jnp.max(st, axis=0, keepdims=True))
            lsum = jnp.sum(p, axis=0, keepdims=True)
            o = _dot(_upk(vt_s[pl.ds(r8, 8), :]), p.astype(BF))
            ot_s[pl.ds(r8, 8), pl.ds(c0, TQ)] = _pk((o * (1.0 / lsum)).astype(BF))
            return carry

        s0[0:16, :] = acc_s[...]
        s0[16:24, :] = l_s[...]
        s0[32:80, :] = qf_s[...].reshape(48, TQ)
        s0[80:112, :] = pltpu.bitcast(w_s[...].reshape(32, TQ), F32)

        jax.lax.fori_loop(0, T, exact_step, 0)

    mod_v[:, 2 * D:] = _dot(sc, wmod_v[:, 2 * D:])[:8]

    def p3a(i):
        r0 = i * RB
        attn = _dot(_upk(ot_s[:, pl.ds(r0, RB)]).T, wo_v[...])
        x1 = x_v[pl.ds(r0, RB), :].astype(F32) + mod_row(2) * attn
        x1_s[pl.ds(r0, RB), :] = x1
        h2 = (_ln(x1) * (1.0 + mod_row(4)) + mod_row(3)).astype(BF)
        h2_s[pl.ds(r0 // 2, RB // 2), :] = _pk(h2)
        return h2

    def p3b(i, h2):
        z2 = _gelu(_dot(h2, win_v[:, FH:]))
        z2_s[pl.ds(i * RB // 2, RB // 2), :] = _pk(_ln(z2).astype(BF))

    h2s = {i: p3a(i) for i in range(3)}
    for i in range(NB):
        if i + 3 < NB:
            h2s[i + 3] = p3a(i + 3)
        p3b(i, h2s.pop(i))

    def out_copy(j):
        r0, n = _OUT_BLOCKS[j]
        return pltpu.make_async_copy(out_v.at[pl.ds(r0, n), :],
                                     out_hbm.at[0, pl.ds(r0, n), :], osems.at[j])

    brow_all = bsp_v[...].reshape(1, S).astype(F32)
    for i in range(NB):
        r0 = i * RB
        z1 = _gelu(_dot(_upk(h2_s[pl.ds(r0 // 2, RB // 2), :]), win_v[:, :FH]))
        gsp = _dot(wsp_v[pl.ds(r0, RB), :], _upk(z2_s[...]))
        bcol = jnp.broadcast_to(brow_all[:, r0:r0 + RB], (128, RB)).T
        bfull = jnp.concatenate([bcol] * (FH // 128), axis=1)
        u = (z1 * (gsp + bfull)).astype(BF)
        for j, (o0, n) in enumerate(_OUT_BLOCKS):
            if r0 <= o0 < r0 + RB:
                y = _dot(u[o0 - r0:o0 - r0 + n], wout_v[...])
                out_v[pl.ds(o0, n), :] = (x1_s[pl.ds(o0, n), :] + mod_row(5) * y).astype(BF)
                out_copy(j).start()
    for j in range(len(_OUT_BLOCKS)):
        out_copy(j).wait()


@jax.jit
def pallas_adaLN_cond__softmax_full_mha__mixer_gmlp__prompt_kernel(
    A_x: jax.Array,
    A_wqkv: jax.Array,
    A_wo: jax.Array,
    B_x: jax.Array,
    B_w_in: jax.Array,
    B_w_sp: jax.Array,
    B_b_sp: jax.Array,
    B_w_out: jax.Array,
    c: jax.Array,
    w_mod: jax.Array,
):
    del B_x
    vm = pltpu.VMEM
    scratch = [
        vm((S, D), BF), vm((D, 3 * D), BF), vm((D, D), BF),
        vm((D, 2 * FH), BF), vm((S, S), BF), vm((FH, D), BF),
        vm((D, 6 * D), BF), vm((1, D), BF), vm((S,), BF),
        vm((8, 6 * D), F32),
        vm((H // 2, S // 2, 128), U32),
        vm((S // 2, 128), U32), vm((16, S), U32),
        vm((2, 16, TQ), U32), vm((2, 24, TQ), F32),
        vm((4, S // 2, 128), U32),
        vm((D // 2, S), U32), vm((D // 2, S), U32),
        vm((128, D), U32), vm((D // 2, 256), U32),
        vm((H, S), F32), vm((H, RB), F32),
        vm((DH, 256, 128), F32), vm((DH, 256, 128), F32),
        vm((SPI, DH + 1, 8, TQ), F32),
        vm((16, TQ), F32), vm((8, TQ), F32), vm((CK + 16 * SH, TQ), F32),
        vm((S, TQ), F32), vm((D // 2, S), U32),
        vm((S, D), F32), vm((S // 2, D), U32), vm((S // 2, FH), U32),
        vm((RB, 3 * D), F32),
        vm((S, D), BF),
        pltpu.SemaphoreType.DMA((22,)),
        pltpu.SemaphoreType.DMA((len(_OUT_BLOCKS),)),
    ]
    any_spec = pl.BlockSpec(memory_space=pl.ANY)
    return pl.pallas_call(
        _kernel,
        out_shape=jax.ShapeDtypeStruct((1, S, D), BF),
        in_specs=[any_spec] * 9,
        out_specs=any_spec,
        scratch_shapes=scratch,
        compiler_params=pltpu.CompilerParams(vmem_limit_bytes=100 * 1024 * 1024),
    )(A_x, A_wqkv, A_wo, B_w_in, B_w_sp, B_b_sp, B_w_out, c, w_mod)
```

```python
import jax
import jax.numpy as jnp
import jax.experimental.pallas as pl
import jax.experimental.pallas.tpu as pltpu

S = 2048
D = 512
H = 32
DH = 16
FH = 896
EPS = 1e-5
LOG2E = 1.4426950408889634
QSCALE = (DH ** -0.5) * LOG2E

TQ = 512
CK = 128
NC = S // CK
NQ = S // TQ
T = H * NQ
SPI = 2 * NQ
RB = 512
NB = S // RB
NJ = 4
JW = D // NJ
OT = 128

VB = 0
NPG = 3
SH = 1
TD = 3
KFD = 6
KBE = 8
L_MIN = 2.0 ** -64
L_MAX = 2.0 ** 20

BF = jnp.bfloat16
F32 = jnp.float32
U32 = jnp.uint32


def _pk(x):
    return pltpu.bitcast(x, U32)


def _upk(x):
    return pltpu.bitcast(x, BF)


def _mo(x, n):
    return x if isinstance(x, int) else pl.multiple_of(x, n)


def _dot(a, b):
    return jnp.dot(a, b, preferred_element_type=F32)


def _ln(x):
    m = jnp.mean(x, axis=-1, keepdims=True)
    xc = x - m
    v = jnp.mean(xc * xc, axis=-1, keepdims=True)
    return xc * jax.lax.rsqrt(v + EPS)


def _gelu(x):
    c0 = 0.7978845608028654
    inner = x * (c0 + (c0 * 0.044715) * (x * x))
    hx = 0.5 * x
    return hx + hx * jnp.tanh(inner)


_OUT_BLOCKS = ([(i * RB, RB) for i in range(NB - 1)]
               + [(S - RB + j * OT, OT) for j in range(RB // OT)])


def _kernel(x_hbm, wqkv_hbm, wo_hbm, win_hbm, wsp_hbm, bsp_hbm, wout_hbm, c_hbm, wmod_hbm,
            out_hbm,
            x_v, wqkv_v, wo_v, win_v, wsp_v, wout_v, wmod_v, c_v, bsp_v, mod_v,
            k_s, ka_s, va_s, w_s, qf_s, kr_s, qt_s, vt_s, ksel_s, kt_s, qn_s, kn_s, kb0, kb1,
            qb_s, acc_s, l_s, car_s, s0, ot_s, x1_s, h2_s, z2_s, q0_s, out_v, sems, osems):
    def cols(src, dst, c0, n, sem):
        return pltpu.make_async_copy(src.at[:, pl.ds(c0, n)], dst.at[:, pl.ds(c0, n)], sem)

    def xrows(r0, n, sem):
        return pltpu.make_async_copy(x_hbm.at[0, pl.ds(r0, n), :], x_v.at[pl.ds(r0, n), :], sem)

    cp_c = pltpu.make_async_copy(c_hbm, c_v, sems.at[0])
    cp_x0 = xrows(0, RB, sems.at[1])
    cp_ms = [cols(wmod_hbm, wmod_v, j * JW, JW, sems.at[14 + j]) for j in range(NJ)]
    cp_mc = [cols(wmod_hbm, wmod_v, D + j * JW, JW, sems.at[18 + j]) for j in range(NJ)]
    cp_w = [pltpu.make_async_copy(wqkv_hbm.at[pl.ds(j * JW, JW), :],
                                  wqkv_v.at[pl.ds(j * JW, JW), :], sems.at[2 + j])
            for j in range(NJ)]
    cp_x1 = xrows(RB, RB, sems.at[6])
    cp_x23 = xrows(2 * RB, 2 * RB, sems.at[7])
    late = [cols(wmod_hbm, wmod_v, 2 * D, 4 * D, sems.at[8]),
            pltpu.make_async_copy(wo_hbm, wo_v, sems.at[9]),
            pltpu.make_async_copy(win_hbm, win_v, sems.at[10]),
            pltpu.make_async_copy(wsp_hbm, wsp_v, sems.at[11]),
            pltpu.make_async_copy(wout_hbm, wout_v, sems.at[12]),
            pltpu.make_async_copy(bsp_hbm, bsp_v, sems.at[13])]
    order = [cp_c, cp_x0, cp_ms[0], cp_mc[0]]
    for j in range(NJ):
        if j + 1 < NJ:
            order += [cp_ms[j + 1], cp_mc[j + 1]]
        else:
            order.append(cp_x1)
        order.append(cp_w[j])
    for cp in order + [cp_x23] + late:
        cp.start()

    cp_c.wait()
    cp_x0.wait()
    c = c_v[...].astype(F32)
    sc = (c * jax.nn.sigmoid(c)).astype(BF)
    sc = jnp.broadcast_to(sc, (16, D))

    def norm1(i):
        return _ln(x_v[pl.ds(i * RB, RB), :].astype(F32))

    def mod_row(j):
        return mod_v[0:1, j * D:(j + 1) * D]

    def modulate1(n):
        return (n * (1.0 + mod_row(1)) + mod_row(0)).astype(BF)

    n0 = norm1(0)

    def h0_piece(j):
        for c0 in (j * JW, D + j * JW):
            mod_v[:, c0:c0 + JW] = _dot(sc, wmod_v[:, c0:c0 + JW])[:8]
        sa = mod_v[0:1, j * JW:(j + 1) * JW]
        ca = mod_v[0:1, D + j * JW:D + (j + 1) * JW]
        return (n0[:, j * JW:(j + 1) * JW] * (1.0 + ca) + sa).astype(BF)

    cp_ms[0].wait()
    cp_mc[0].wait()
    hj = h0_piece(0)
    qkv0 = None
    for j in range(NJ):
        if j + 1 < NJ:
            cp_ms[j + 1].wait()
            cp_mc[j + 1].wait()
        if j == NJ - 2:
            cp_x1.wait()
        cp_w[j].wait()
        part = _dot(hj, wqkv_v[j * JW:(j + 1) * JW, :])
        if j == 0:
            q0_s[...] = part
        elif j + 1 < NJ:
            q0_s[...] = q0_s[...] + part
        else:
            qkv0 = q0_s[...] + part
        if j + 1 < NJ:
            hj = h0_piece(j + 1)
        if j >= NJ - 2:
            hr = RB // 2
            half = j - (NJ - 2)
            h2_s[pl.ds(half * hr // 2, hr // 2), :] = _pk(
                modulate1(_ln(x_v[pl.ds(RB + half * hr, hr), :].astype(F32))))

    def head_sq(xt):
        xf = xt.astype(F32)
        return (xf * xf).reshape(H, DH, xt.shape[1]).sum(axis=1)

    def proj_k(i, h):
        k = qkv0[:, D:2 * D] if i == 0 else _dot(h, wqkv_v[:, D:2 * D])
        k = k.astype(BF)
        kp = _pk(k)
        for g in range(4):
            kr_s[g, pl.ds(i * RB // 2, RB // 2), :] = kp[:, g * 128:(g + 1) * 128]
        for t_ in range(RB // CK):
            ksel_s[pl.ds((i * (RB // CK) + t_) * 8, 8), :] = (
                kp[t_ * 64 + 8 * VB:t_ * 64 + 8 * VB + 8])
        kn = head_sq(k.T)
        kn_s[...] = kn if i == 0 else jnp.maximum(kn_s[...], kn)

    lane = jax.lax.broadcasted_iota(jnp.int32, (8, 128), 1)
    one_pk = _pk(jnp.where(jax.lax.broadcasted_iota(jnp.int32, (16, 128), 1) == 2 * DH,
                           1.0, 0.0).astype(BF))

    def rot_k(i):
        n8 = RB // 16
        keep = jnp.broadcast_to((lane < 2 * DH)[None], (n8, 8, 128))
        fill = jnp.broadcast_to(one_pk[None], (n8, 8, 128))
        for g in range(4):
            kg = kr_s[g, pl.ds(i * RB // 2, RB // 2), :]
            for j in range(4):
                kj = kg if j == 0 else pltpu.roll(kg, 128 - 32 * j, axis=1)
                kj = jnp.where(keep, kj.reshape(n8, 8, 128), fill).reshape(RB // 2, 128)
                k_s[4 * g + j, pl.ds(i * RB // 2, RB // 2), :] = kj
                if g == 0 and j == 0:
                    ka_s[pl.ds(i * RB // 2, RB // 2), :] = kj

    def proj_q(i, h):
        q = qkv0[:, :D] if i == 0 else _dot(h, wqkv_v[:, :D])
        qt = (q * QSCALE).astype(BF).T
        qt_s[:, pl.ds(i * RB, RB)] = _pk(qt)
        qn_s[:, pl.ds(i * RB, RB)] = head_sq(qt)

    def make_ref(i):
        kmax = jnp.max(kn_s[...], axis=1, keepdims=True)
        bound = jnp.sqrt(qn_s[:, pl.ds(i * RB, RB)] * kmax) * (1.0 + 2.0 ** -6)
        qn_s[:, pl.ds(i * RB, RB)] = (-bound).astype(BF).astype(F32)

    def proj_v(i, h):
        v = qkv0[:, 2 * D:] if i == 0 else _dot(h, wqkv_v[:, 2 * D:])
        vp = _pk(v.astype(BF).T)
        vt_s[:, pl.ds(i * RB, RB)] = vp
        va_s[:, pl.ds(i * RB, RB)] = vp[:16]

    cp_x23.wait()
    hs = {1: _upk(h2_s[pl.ds(0, RB // 2), :])}
    proj_k(0, None)
    rot_k(0)
    proj_q(0, None)
    proj_v(0, None)
    hs[2] = modulate1(norm1(2))
    proj_k(1, hs[1])
    rot_k(1)
    proj_q(1, hs[1])
    hs[3] = modulate1(norm1(3))
    proj_k(2, hs[2])
    rot_k(2)
    proj_q(2, hs[2])
    proj_v(1, hs[1])
    proj_k(3, hs[3])
    rot_k(3)
    kt_s[...] = _pk(_upk(ksel_s[...]).T)
    for i in range(NB - 1):
        make_ref(i)
    proj_q(3, hs[3])
    make_ref(3)
    proj_v(2, hs[2])
    proj_v(3, hs[3])

    def q_rows(h, qb):
        return qt_s[pl.ds(_mo(h * 8, 8), 8), qb * TQ:(qb + 1) * TQ]

    def nref_row(h, qb):
        return qn_s[pl.ds(h, 1), qb * TQ:(qb + 1) * TQ]

    def clamp_h(h):
        return min(h, H - 1) if isinstance(h, int) else jnp.minimum(h, H - 1)

    row0 = jax.lax.broadcasted_iota(jnp.int32, (16, TQ), 0) == 0

    def make_w(h, qb, par, slot, staged=False):
        if not staged:
            aug = jnp.where(row0, jnp.broadcast_to(nref_row(h, qb), (16, TQ)), 0.0).astype(BF)
            w_s[slot] = _pk(jnp.concatenate([_upk(q_rows(h, qb)), aug], axis=0))
        qa = _upk(w_s[slot])
        q, aug = qa[:DH], qa[DH:]
        z = jnp.zeros((DH, TQ), BF)
        return jnp.concatenate([z, q, aug] if par else [q, z, aug], axis=0)

    def stage_qf(h, qb, slot):
        qf_s[slot, 0:DH, :] = _upk(q_rows(h, qb)).astype(F32)
        qf_s[slot, DH:DH + 8, :] = jnp.broadcast_to(nref_row(h, qb), (8, TQ))

    def make_qb(h, qb, slot, ds_, tok=None, never=None, fslot=None):
        if fslot is None:
            qf = _upk(q_rows(h, qb)).astype(F32)
        for d in ds_:
            if fslot is not None:
                blk = qf_s[fslot, pl.ds(8 * (d // 8), 8), :]
                row = blk[d % 8:d % 8 + 1]
            else:
                row = nref_row(h, qb) if d == DH else qf[d:d + 1]
            val = jnp.broadcast_to(row, (8, TQ))
            if tok is not None:
                val = jnp.where(never, tok, val)
            qb_s[slot, d] = val

    def make_kb(h, j, kb, tok=None, never=None):
        d, half = j // 2, j % 2
        kt = _upk(kt_s[pl.ds(_mo(h * 8, 8), 8), half * 128:(half + 1) * 128]).astype(F32)
        row = jnp.broadcast_to(kt[d:d + 1], (8, 128))
        if tok is not None:
            row = jnp.where(never, tok[:, :128], row)
        val = jnp.concatenate([row] * 16, axis=0).T
        kb[d, pl.ds(half * 128, 128), :] = val
        return val[120:]

    def fence(val, on, never):
        return jnp.where(never, pltpu.bitcast(val, U32), on)

    def v_unit(tile, ui, kb, slot):
        c0 = ui * 256
        acc = None
        toks = []
        for d in range(DH):
            kk = kb[d, pl.ds(16 * tile, 16), :]
            kk = jnp.concatenate([kk] * 2, axis=1).reshape(2, 8, 256)
            t_ = kk * qb_s[slot, d, :, c0:c0 + 256][None]
            acc = t_ + qb_s[slot, DH, :, c0:c0 + 256][None] if acc is None else acc + t_
            if ((d + 1) * NPG) // DH != (d * NPG) // DH:
                ts = [acc[a_, :, b_ * 128:(b_ + 1) * 128] for a_ in range(2) for b_ in range(2)]
                toks.append((ts[0] + ts[1]) + (ts[2] + ts[3]))
        return acc.reshape(16, 256), toks

    def v_rows(tile, kb, slot):
        us = [v_unit(tile, ui, kb, slot) for ui in range(2)]
        return jnp.concatenate([us[0][0], us[1][0]], axis=1), us[0][1] + us[1][1]

    mx_blocks = [j for j in reversed(range(8)) if j != VB]

    def qk_run(w, items, toks, never, extra=()):
        parts = [ka_s[pl.ds(t_ * 64 + 8 * j, 8), :] for t_, j in items]
        for i_, tk in enumerate(toks):
            j = (i_ * len(parts)) // len(toks)
            parts[j] = fence(tk, parts[j], never[i_ % 2])
        if extra:
            val = extra[0]
            for v_ in extra[1:]:
                val = val + v_
            parts[0] = fence(val, parts[0], never[2])
        st = _dot(_upk(jnp.concatenate(parts, axis=0))[:, :3 * DH], w)
        return [st[16 * i_:16 * i_ + 16] for i_ in range(len(items))]

    def b_tile(hoff, ck, s):
        p = jnp.exp2(s)
        l = None if ck == 0 else l_s[...]
        for j in reversed(range(CK // 16)):
            pr = p[16 * j:16 * j + 8] + p[16 * j + 8:16 * j + 16]
            l = pr if l is None else l + pr
        l_s[...] = l
        vc = _upk(va_s[pl.ds(hoff * 8, 8), pl.ds(ck * CK, CK)])
        pv = _dot(vc, p.astype(BF))
        acc = pv if ck == 0 else acc_s[...] + pv
        acc_s[...] = acc
        return l, acc

    def fin(h, qb, l, acc):
        lsum = l.sum(axis=0, keepdims=True)
        o = acc * (1.0 / lsum)
        ot_s[pl.ds(_mo(h * 8, 8), 8), qb * TQ:(qb + 1) * TQ] = _pk(o.astype(BF))
        return lsum

    kbs = (kb0, kb1)
    kb_sched = [[] for _ in range(NQ * NC)]
    for kj in range(2 * DH):
        kb_sched[(kj * (NQ * NC - KBE)) // (2 * DH)].append(kj)

    car_mx = [(0, j) for j in mx_blocks] + [(1, j) for j in mx_blocks[:SH]]
    car_items = car_mx + [(0, VB), (1, VB)]

    def run_steps(pair, state, never):
        h0 = 2 * pair
        lo, hi = state
        pend = {}
        lh = []
        sc_ = {}
        for i_, (t_, j) in enumerate(car_items):
            sc_[(0, t_, j)] = car_s[pl.ds(16 * i_, 16), :]
        ws = {}
        next_pair = jnp.minimum(pair + 1, H // 2 - 1)

        def step_hq(s_):
            return clamp_h(h0 + s_ // NQ) if s_ >= SPI else h0 + s_ // NQ, s_ % NQ

        def get_w(s_):
            if s_ not in ws:
                ws[s_] = make_w(*step_hq(s_), (s_ // NQ) % 2, s_ % 2, staged=(s_ == 0))
            return ws[s_]

        for s_ in range(SPI):
            h, qb = step_hq(s_)
            kb_make = kbs[1 - (s_ // NQ) % 2]
            for c_ in range(NC):
                gt = s_ * NC + c_
                g1, g2 = gt + 1, gt + 2
                it1 = [(g1 // NC, g1 % NC, j) for j in mx_blocks[SH:]]
                it2 = [(g2 // NC, g2 % NC, j) for j in mx_blocks[:SH]]
                s1 = g1 // NC
                if gt == 0:
                    toks = []
                else:
                    sc_[(s1, g1 % NC, VB)], toks = v_rows(g1 % NC, kbs[(s1 // NQ) % 2], s1 % SPI)
                runs = [it1 + it2] if g1 // NC == g2 // NC else [it1, it2]
                for ri, its in enumerate(runs):
                    outs = qk_run(get_w(its[0][0]), [(t_, j) for _, t_, j in its],
                                  toks if ri == 0 else [], never,
                                  pend.pop(gt, ()) if ri == 0 else ())
                    sc_.update(zip(its, outs))
                    for sr_, t_, j in its:
                        if sr_ == SPI - 1:
                            r_ = t_ * 64 + 8 * j
                            ka_s[pl.ds(r_, 8), :] = k_s[next_pair, pl.ds(r_, 8), :]
                tok = lh[-TD] if len(lh) >= TD else None
                if s_ >= 1:
                    un = s_ - 1 + SPI
                    ds_ = [c_, DH] if c_ == NC - 1 else [c_]
                    if c_ == 0:
                        stage_qf(clamp_h(h0 + un // NQ), un % NQ, s_ % 2)
                    make_qb(clamp_h(h0 + un // NQ), un % NQ, s_ - 1, ds_, tok, never[0], s_ % 2)
                for kj in kb_sched[(s_ % NQ) * NC + c_]:
                    val = make_kb(clamp_h(h + 1), kj, kb_make, tok, never[0])
                    if gt + KFD < SPI * NC:
                        pend.setdefault(gt + KFD, []).append(val)
                s_cur = jnp.concatenate([sc_.pop((s_, c_, j)) for j in range(8)], axis=0)
                l, acc = b_tile((s_ // NQ) % 2, c_, s_cur)
                if s_ % NQ == NQ - 1:
                    hv = clamp_h(h + 2)
                    va_s[pl.ds(((s_ // NQ) % 2) * 8, 8), pl.ds(c_ * CK, CK)] = (
                        vt_s[pl.ds(_mo(hv * 8, 8), 8), pl.ds(c_ * CK, CK)])
                lh.append(l)
            lsum = fin(h, qb, l, acc)
            lo = jnp.minimum(lo, lsum)
            hi = jnp.maximum(hi, lsum)
        sc_[(SPI, 1, VB)] = v_rows(1, kb0, 0)[0]
        for i_, (t_, j) in enumerate(car_items):
            car_s[pl.ds(16 * i_, 16), :] = sc_.pop((SPI, t_, j))
        un = 2 * SPI - 1
        make_qb(clamp_h(h0 + un // NQ), un % NQ, SPI - 1, range(DH + 1))
        return lo, hi

    for u_ in range(SPI):
        make_qb(u_ // NQ, u_ % NQ, u_, range(DH + 1))
    for j in range(2 * DH):
        make_kb(0, j, kb0)
    pro = qk_run(make_w(0, 0, 0, 0), car_mx, [], None) + [v_rows(0, kb0, 0)[0], v_rows(1, kb0, 0)[0]]
    for i_, o_ in enumerate(pro):
        car_s[pl.ds(16 * i_, 16), :] = o_

    def p2_body(i, state):
        return run_steps(i, state, (i < 0, i < -1, i < -2))

    one = jnp.ones((1, TQ), F32)
    lo, hi = jax.lax.fori_loop(0, T // SPI, p2_body, (one, one))

    for cp in late:
        cp.wait()

    ok = jnp.logical_and(lo >= L_MIN, hi <= L_MAX)
    n_bad = jnp.sum(jnp.where(ok, 0.0, 1.0))

    @pl.when(n_bad > 0.0)
    def _():
        def exact_step(t, carry):
            h = t // NQ
            c0 = pl.multiple_of((t % NQ) * TQ, TQ)
            r8 = pl.multiple_of(h * 8, 8)
            q = qt_s[pl.ds(r8, 8), pl.ds(c0, TQ)]
            zq = jnp.zeros_like(q)
            odd = h % 2 == 1
            w = _upk(jnp.concatenate([jnp.where(odd, zq, q), jnp.where(odd, q, zq)], axis=0))
            s0[...] = _dot(_upk(k_s[h // 2])[:, :2 * DH], w)
            st = s0[...]
            p = jnp.exp2(st - jnp.max(st, axis=0, keepdims=True))
            lsum = jnp.sum(p, axis=0, keepdims=True)
            o = _dot(_upk(vt_s[pl.ds(r8, 8), :]), p.astype(BF))
            ot_s[pl.ds(r8, 8), pl.ds(c0, TQ)] = _pk((o * (1.0 / lsum)).astype(BF))
            return carry

        s0[0:16, :] = acc_s[...]
        s0[16:24, :] = l_s[...]
        s0[32:80, :] = qf_s[...].reshape(48, TQ)
        s0[80:112, :] = pltpu.bitcast(w_s[...].reshape(32, TQ), F32)

        jax.lax.fori_loop(0, T, exact_step, 0)

    mod_v[:, 2 * D:] = _dot(sc, wmod_v[:, 2 * D:])[:8]

    def p3a(i):
        r0 = i * RB
        attn = _dot(_upk(ot_s[:, pl.ds(r0, RB)]).T, wo_v[...])
        x1 = x_v[pl.ds(r0, RB), :].astype(F32) + mod_row(2) * attn
        x1_s[pl.ds(r0, RB), :] = x1
        h2 = (_ln(x1) * (1.0 + mod_row(4)) + mod_row(3)).astype(BF)
        h2_s[pl.ds(r0 // 2, RB // 2), :] = _pk(h2)
        return h2

    def p3b(i, h2):
        z2 = _gelu(_dot(h2, win_v[:, FH:]))
        z2_s[pl.ds(i * RB // 2, RB // 2), :] = _pk(_ln(z2).astype(BF))

    h2s = [p3a(i) for i in range(NB)]
    z1s = []
    for i in range(NB):
        z1s.append(_dot(h2s[i], win_v[:, :FH]))
        p3b(i, h2s[i])

    def out_copy(j):
        r0, n = _OUT_BLOCKS[j]
        return pltpu.make_async_copy(out_v.at[pl.ds(r0, n), :],
                                     out_hbm.at[0, pl.ds(r0, n), :], osems.at[j])

    brow_all = bsp_v[...].reshape(1, S).astype(F32)
    for i in range(NB):
        r0 = i * RB
        z1 = _gelu(z1s[i])
        gsp = _dot(wsp_v[pl.ds(r0, RB), :], _upk(z2_s[...]))
        bcol = jnp.broadcast_to(brow_all[:, r0:r0 + RB], (128, RB)).T
        bfull = jnp.concatenate([bcol] * (FH // 128), axis=1)
        u = (z1 * (gsp + bfull)).astype(BF)
        for j, (o0, n) in enumerate(_OUT_BLOCKS):
            if r0 <= o0 < r0 + RB:
                y = _dot(u[o0 - r0:o0 - r0 + n], wout_v[...])
                out_v[pl.ds(o0, n), :] = (x1_s[pl.ds(o0, n), :] + mod_row(5) * y).astype(BF)
                out_copy(j).start()
    for j in range(len(_OUT_BLOCKS)):
        out_copy(j).wait()


@jax.jit
def pallas_adaLN_cond__softmax_full_mha__mixer_gmlp__prompt_kernel(
    A_x: jax.Array,
    A_wqkv: jax.Array,
    A_wo: jax.Array,
    B_x: jax.Array,
    B_w_in: jax.Array,
    B_w_sp: jax.Array,
    B_b_sp: jax.Array,
    B_w_out: jax.Array,
    c: jax.Array,
    w_mod: jax.Array,
):
    del B_x
    vm = pltpu.VMEM
    scratch = [
        vm((S, D), BF), vm((D, 3 * D), BF), vm((D, D), BF),
        vm((D, 2 * FH), BF), vm((S, S), BF), vm((FH, D), BF),
        vm((D, 6 * D), BF), vm((1, D), BF), vm((S,), BF),
        vm((8, 6 * D), F32),
        vm((H // 2, S // 2, 128), U32),
        vm((S // 2, 128), U32), vm((16, S), U32),
        vm((2, 16, TQ), U32), vm((2, 24, TQ), F32),
        vm((4, S // 2, 128), U32),
        vm((D // 2, S), U32), vm((D // 2, S), U32),
        vm((128, D), U32), vm((D // 2, 256), U32),
        vm((H, S), F32), vm((H, RB), F32),
        vm((DH, 256, 128), F32), vm((DH, 256, 128), F32),
        vm((SPI, DH + 1, 8, TQ), F32),
        vm((16, TQ), F32), vm((8, TQ), F32), vm((CK + 16 * SH + 16, TQ), F32),
        vm((S, TQ), F32), vm((D // 2, S), U32),
        vm((S, D), F32), vm((S // 2, D), U32), vm((S // 2, FH), U32),
        vm((RB, 3 * D), F32),
        vm((S, D), BF),
        pltpu.SemaphoreType.DMA((22,)),
        pltpu.SemaphoreType.DMA((len(_OUT_BLOCKS),)),
    ]
    any_spec = pl.BlockSpec(memory_space=pl.ANY)
    return pl.pallas_call(
        _kernel,
        out_shape=jax.ShapeDtypeStruct((1, S, D), BF),
        in_specs=[any_spec] * 9,
        out_specs=any_spec,
        scratch_shapes=scratch,
        compiler_params=pltpu.CompilerParams(vmem_limit_bytes=100 * 1024 * 1024),
    )(A_x, A_wqkv, A_wo, B_w_in, B_w_sp, B_b_sp, B_w_out, c, w_mod)
```

```python
import jax
import jax.numpy as jnp
import jax.experimental.pallas as pl
import jax.experimental.pallas.tpu as pltpu

S = 2048
D = 512
H = 32
DH = 16
FH = 896
EPS = 1e-5
LOG2E = 1.4426950408889634
QSCALE = (DH ** -0.5) * LOG2E

TQ = 512
CK = 128
NC = S // CK
NQ = S // TQ
T = H * NQ
SPI = 2 * NQ
RB = 512
NB = S // RB
NJ = 4
JW = D // NJ
TAIL = (256, 128, 64, 32, 32)

VB = 0
NPG = 3
SH = 1
TD = 3
KFD = 6
KBE = 8
L_MIN = 2.0 ** -40
L_MAX = 2.0 ** 20

BF = jnp.bfloat16
F32 = jnp.float32
U32 = jnp.uint32


def _pk(x):
    return pltpu.bitcast(x, U32)


def _upk(x):
    return pltpu.bitcast(x, BF)


def _mo(x, n):
    return x if isinstance(x, int) else pl.multiple_of(x, n)


def _dot(a, b):
    return jnp.dot(a, b, preferred_element_type=F32)


def _ln(x):
    m = jnp.mean(x, axis=-1, keepdims=True)
    xc = x - m
    v = jnp.mean(xc * xc, axis=-1, keepdims=True)
    return xc * jax.lax.rsqrt(v + EPS)


def _gelu(x):
    c0 = 0.7978845608028654
    inner = x * (c0 + (c0 * 0.044715) * (x * x))
    hx = 0.5 * x
    return hx + hx * jnp.tanh(inner)


_OUT_BLOCKS = ([(i * RB, RB) for i in range(NB - 1)]
               + [(S - RB + sum(TAIL[:j]), n_) for j, n_ in enumerate(TAIL)])


def _kernel(x_hbm, wqkv_hbm, wo_hbm, win_hbm, wsp_hbm, bsp_hbm, wout_hbm, c_hbm, wmod_hbm,
            out_hbm,
            x_v, wqkv_v, wo_v, win_v, wsp_v, wout_v, wmod_v, c_v, bsp_v, mod_v,
            k_s, ka_s, va_s, w_s, qf_s, kr_s, qt_s, vt_s, ksel_s, kt_s, qn_s, kn_s, kb0, kb1,
            qb_s, acc_s, l_s, car_s, s0, ot_s, x1_s, h2_s, z2_s, q0_s, out_v, sems, osems):
    def cols(src, dst, c0, n, sem):
        return pltpu.make_async_copy(src.at[:, pl.ds(c0, n)], dst.at[:, pl.ds(c0, n)], sem)

    def xrows(r0, n, sem):
        return pltpu.make_async_copy(x_hbm.at[0, pl.ds(r0, n), :], x_v.at[pl.ds(r0, n), :], sem)

    cp_c = pltpu.make_async_copy(c_hbm, c_v, sems.at[0])
    cp_x0 = xrows(0, RB, sems.at[1])
    cp_ms = [cols(wmod_hbm, wmod_v, j * JW, JW, sems.at[14 + j]) for j in range(NJ)]
    cp_mc = [cols(wmod_hbm, wmod_v, D + j * JW, JW, sems.at[18 + j]) for j in range(NJ)]
    cp_w = [pltpu.make_async_copy(wqkv_hbm.at[pl.ds(j * JW, JW), :],
                                  wqkv_v.at[pl.ds(j * JW, JW), :], sems.at[2 + j])
            for j in range(NJ)]
    cp_x1 = xrows(RB, RB, sems.at[6])
    cp_x23 = xrows(2 * RB, 2 * RB, sems.at[7])
    late = [cols(wmod_hbm, wmod_v, 2 * D, 4 * D, sems.at[8]),
            pltpu.make_async_copy(wo_hbm, wo_v, sems.at[9]),
            pltpu.make_async_copy(win_hbm, win_v, sems.at[10]),
            pltpu.make_async_copy(wsp_hbm, wsp_v, sems.at[11]),
            pltpu.make_async_copy(wout_hbm, wout_v, sems.at[12]),
            pltpu.make_async_copy(bsp_hbm, bsp_v, sems.at[13])]
    order = [cp_c, cp_x0, cp_ms[0], cp_mc[0]]
    for j in range(NJ):
        if j + 1 < NJ:
            order += [cp_ms[j + 1], cp_mc[j + 1]]
        else:
            order.append(cp_x1)
        order.append(cp_w[j])
    for cp in order + [cp_x23] + late:
        cp.start()

    cp_c.wait()
    cp_x0.wait()
    c = c_v[...].astype(F32)
    sc = (c * jax.nn.sigmoid(c)).astype(BF)
    sc = jnp.broadcast_to(sc, (16, D))

    def norm1(i):
        return _ln(x_v[pl.ds(i * RB, RB), :].astype(F32))

    def mod_row(j):
        return mod_v[0:1, j * D:(j + 1) * D]

    def modulate1(n):
        return (n * (1.0 + mod_row(1)) + mod_row(0)).astype(BF)

    n0 = norm1(0)

    def h0_piece(j):
        for c0 in (j * JW, D + j * JW):
            mod_v[:, c0:c0 + JW] = _dot(sc, wmod_v[:, c0:c0 + JW])[:8]
        sa = mod_v[0:1, j * JW:(j + 1) * JW]
        ca = mod_v[0:1, D + j * JW:D + (j + 1) * JW]
        return (n0[:, j * JW:(j + 1) * JW] * (1.0 + ca) + sa).astype(BF)

    cp_ms[0].wait()
    cp_mc[0].wait()
    hj = h0_piece(0)
    qkv0 = None
    for j in range(NJ):
        if j + 1 < NJ:
            cp_ms[j + 1].wait()
            cp_mc[j + 1].wait()
        if j == NJ - 2:
            cp_x1.wait()
        cp_w[j].wait()
        part = _dot(hj, wqkv_v[j * JW:(j + 1) * JW, :])
        if j == 0:
            q0_s[...] = part
        elif j + 1 < NJ:
            q0_s[...] = q0_s[...] + part
        else:
            qkv0 = q0_s[...] + part
        if j + 1 < NJ:
            hj = h0_piece(j + 1)
        if j >= NJ - 2:
            hr = RB // 2
            half = j - (NJ - 2)
            h2_s[pl.ds(half * hr // 2, hr // 2), :] = _pk(
                modulate1(_ln(x_v[pl.ds(RB + half * hr, hr), :].astype(F32))))

    def head_sq(xt):
        xf = xt.astype(F32)
        return (xf * xf).reshape(H, DH, xt.shape[1]).sum(axis=1)

    def proj_k(i, h):
        k = qkv0[:, D:2 * D] if i == 0 else _dot(h, wqkv_v[:, D:2 * D])
        k = k.astype(BF)
        kp = _pk(k)
        for g in range(4):
            kr_s[g, pl.ds(i * RB // 2, RB // 2), :] = kp[:, g * 128:(g + 1) * 128]
        for t_ in range(RB // CK):
            ksel_s[pl.ds((i * (RB // CK) + t_) * 8, 8), :] = (
                kp[t_ * 64 + 8 * VB:t_ * 64 + 8 * VB + 8])
        kn = head_sq(k.T)
        kn_s[...] = kn if i == 0 else jnp.maximum(kn_s[...], kn)

    lane = jax.lax.broadcasted_iota(jnp.int32, (8, 128), 1)
    one_pk = _pk(jnp.where(jax.lax.broadcasted_iota(jnp.int32, (16, 128), 1) == 2 * DH,
                           1.0, 0.0).astype(BF))

    def rot_k(i):
        n8 = RB // 16
        keep = jnp.broadcast_to((lane < 2 * DH)[None], (n8, 8, 128))
        fill = jnp.broadcast_to(one_pk[None], (n8, 8, 128))
        for g in range(4):
            kg = kr_s[g, pl.ds(i * RB // 2, RB // 2), :]
            for j in range(4):
                kj = kg if j == 0 else pltpu.roll(kg, 128 - 32 * j, axis=1)
                kj = jnp.where(keep, kj.reshape(n8, 8, 128), fill).reshape(RB // 2, 128)
                k_s[4 * g + j, pl.ds(i * RB // 2, RB // 2), :] = kj
                if g == 0 and j == 0:
                    ka_s[pl.ds(i * RB // 2, RB // 2), :] = kj

    def proj_q(i, h):
        q = qkv0[:, :D] if i == 0 else _dot(h, wqkv_v[:, :D])
        qt = (q * QSCALE).astype(BF).T
        qt_s[:, pl.ds(i * RB, RB)] = _pk(qt)
        qn_s[:, pl.ds(i * RB, RB)] = head_sq(qt)

    def make_ref(i):
        kmax = jnp.max(kn_s[...], axis=1, keepdims=True)
        bound = jnp.sqrt(qn_s[:, pl.ds(i * RB, RB)] * kmax) * (1.0 + 2.0 ** -6)
        qn_s[:, pl.ds(i * RB, RB)] = (-bound).astype(BF).astype(F32)

    def proj_v(i, h):
        v = qkv0[:, 2 * D:] if i == 0 else _dot(h, wqkv_v[:, 2 * D:])
        vp = _pk(v.astype(BF).T)
        vt_s[:, pl.ds(i * RB, RB)] = vp
        va_s[:, pl.ds(i * RB, RB)] = vp[:16]

    cp_x23.wait()
    hs = {1: _upk(h2_s[pl.ds(0, RB // 2), :])}
    proj_k(0, None)
    rot_k(0)
    proj_q(0, None)
    proj_v(0, None)
    hs[2] = modulate1(norm1(2))
    proj_k(1, hs[1])
    rot_k(1)
    proj_q(1, hs[1])
    hs[3] = modulate1(norm1(3))
    proj_k(2, hs[2])
    rot_k(2)
    proj_q(2, hs[2])
    proj_v(1, hs[1])
    proj_k(3, hs[3])
    rot_k(3)
    kt_s[...] = _pk(_upk(ksel_s[...]).T)
    for i in range(NB - 1):
        make_ref(i)
    proj_q(3, hs[3])
    make_ref(3)
    proj_v(2, hs[2])
    proj_v(3, hs[3])

    def q_rows(h, qb):
        return qt_s[pl.ds(_mo(h * 8, 8), 8), qb * TQ:(qb + 1) * TQ]

    def nref_row(h, qb):
        return qn_s[pl.ds(h, 1), qb * TQ:(qb + 1) * TQ]

    def clamp_h(h):
        return min(h, H - 1) if isinstance(h, int) else jnp.minimum(h, H - 1)

    row0 = jax.lax.broadcasted_iota(jnp.int32, (16, TQ), 0) == 0

    def make_w(h, qb, par, slot, staged=False):
        if not staged:
            aug = jnp.where(row0, jnp.broadcast_to(nref_row(h, qb), (16, TQ)), 0.0).astype(BF)
            w_s[slot] = _pk(jnp.concatenate([_upk(q_rows(h, qb)), aug], axis=0))
        qa = _upk(w_s[slot])
        q, aug = qa[:DH], qa[DH:]
        z = jnp.zeros((DH, TQ), BF)
        return jnp.concatenate([z, q, aug] if par else [q, z, aug], axis=0)

    def stage_qf(h, qb, slot):
        qf_s[slot, 0:DH, :] = _upk(q_rows(h, qb)).astype(F32)
        qf_s[slot, DH:DH + 8, :] = jnp.broadcast_to(nref_row(h, qb), (8, TQ))

    def make_qb(h, qb, slot, ds_, tok=None, never=None, fslot=None):
        if fslot is None:
            qf = _upk(q_rows(h, qb)).astype(F32)
        for d in ds_:
            if fslot is not None:
                blk = qf_s[fslot, pl.ds(8 * (d // 8), 8), :]
                row = blk[d % 8:d % 8 + 1]
            else:
                row = nref_row(h, qb) if d == DH else qf[d:d + 1]
            val = jnp.broadcast_to(row, (8, TQ))
            if tok is not None:
                val = jnp.where(never, tok, val)
            qb_s[slot, d] = val

    def make_kb(h, j, kb, tok=None, never=None):
        d, half = j // 2, j % 2
        kt = _upk(kt_s[pl.ds(_mo(h * 8, 8), 8), half * 128:(half + 1) * 128]).astype(F32)
        row = jnp.broadcast_to(kt[d:d + 1], (8, 128))
        if tok is not None:
            row = jnp.where(never, tok[:, :128], row)
        val = jnp.concatenate([row] * 16, axis=0).T
        kb[d, pl.ds(half * 128, 128), :] = val
        return val[120:]

    def fence(val, on, never):
        return jnp.where(never, pltpu.bitcast(val, U32), on)

    def v_unit(tile, ui, kb, slot):
        c0 = ui * 256
        acc = None
        toks = []
        for d in range(DH):
            kk = kb[d, pl.ds(16 * tile, 16), :]
            kk = jnp.concatenate([kk] * 2, axis=1).reshape(2, 8, 256)
            t_ = kk * qb_s[slot, d, :, c0:c0 + 256][None]
            acc = t_ + qb_s[slot, DH, :, c0:c0 + 256][None] if acc is None else acc + t_
            if ((d + 1) * NPG) // DH != (d * NPG) // DH:
                ts = [acc[a_, :, b_ * 128:(b_ + 1) * 128] for a_ in range(2) for b_ in range(2)]
                toks.append((ts[0] + ts[1]) + (ts[2] + ts[3]) if d == DH - 1 else ts[0] + ts[3])
        return acc.reshape(16, 256), toks

    def v_rows(tile, kb, slot):
        us = [v_unit(tile, ui, kb, slot) for ui in range(2)]
        return jnp.concatenate([us[0][0], us[1][0]], axis=1), us[0][1] + us[1][1]

    mx_blocks = [j for j in reversed(range(8)) if j != VB]

    def qk_run(w, items, toks, never, extra=()):
        parts = [ka_s[pl.ds(t_ * 64 + 8 * j, 8), :] for t_, j in items]
        for i_, tk in enumerate(toks):
            j = (i_ * len(parts)) // len(toks)
            parts[j] = fence(tk, parts[j], never[i_ % 2])
        if extra:
            val = extra[0]
            for v_ in extra[1:]:
                val = val + v_
            parts[0] = fence(val, parts[0], never[2])
        st = _dot(_upk(jnp.concatenate(parts, axis=0))[:, :3 * DH], w)
        return [st[16 * i_:16 * i_ + 16] for i_ in range(len(items))]

    def b_tile(hoff, ck, s):
        p = jnp.exp2(s)
        l = None if ck == 0 else l_s[...]
        for j in reversed(range(CK // 16)):
            pr = p[16 * j:16 * j + 8] + p[16 * j + 8:16 * j + 16]
            l = pr if l is None else l + pr
        l_s[...] = l
        vc = _upk(va_s[pl.ds(hoff * 8, 8), pl.ds(ck * CK, CK)])
        pv = _dot(vc, p.astype(BF))
        acc = pv if ck == 0 else acc_s[...] + pv
        acc_s[...] = acc
        return l, acc

    def fin(h, qb, l, acc):
        lsum = l.sum(axis=0, keepdims=True)
        o = acc * (1.0 / lsum)
        ot_s[pl.ds(_mo(h * 8, 8), 8), qb * TQ:(qb + 1) * TQ] = _pk(o.astype(BF))
        return lsum

    kbs = (kb0, kb1)
    kb_sched = [[] for _ in range(NQ * NC)]
    for kj in range(2 * DH):
        kb_sched[(kj * (NQ * NC - KBE)) // (2 * DH)].append(kj)

    car_mx = [(0, j) for j in mx_blocks] + [(1, j) for j in mx_blocks[:SH]]
    car_items = car_mx + [(0, VB), (1, VB)]

    def run_steps(pair, state, never):
        h0 = 2 * pair
        lo, hi = state
        pend = {}
        lh = []
        sc_ = {}
        for i_, (t_, j) in enumerate(car_items):
            sc_[(0, t_, j)] = car_s[pl.ds(16 * i_, 16), :]
        ws = {}
        next_pair = jnp.minimum(pair + 1, H // 2 - 1)

        def step_hq(s_):
            return clamp_h(h0 + s_ // NQ) if s_ >= SPI else h0 + s_ // NQ, s_ % NQ

        def get_w(s_):
            if s_ not in ws:
                ws[s_] = make_w(*step_hq(s_), (s_ // NQ) % 2, s_ % 2, staged=(s_ == 0))
            return ws[s_]

        for s_ in range(SPI):
            h, qb = step_hq(s_)
            kb_make = kbs[1 - (s_ // NQ) % 2]
            for c_ in range(NC):
                gt = s_ * NC + c_
                g1, g2 = gt + 1, gt + 2
                it1 = [(g1 // NC, g1 % NC, j) for j in mx_blocks[SH:]]
                it2 = [(g2 // NC, g2 % NC, j) for j in mx_blocks[:SH]]
                s1 = g1 // NC
                if gt == 0:
                    toks = []
                else:
                    sc_[(s1, g1 % NC, VB)], toks = v_rows(g1 % NC, kbs[(s1 // NQ) % 2], s1 % SPI)
                runs = [it1 + it2] if g1 // NC == g2 // NC else [it1, it2]
                for ri, its in enumerate(runs):
                    outs = qk_run(get_w(its[0][0]), [(t_, j) for _, t_, j in its],
                                  toks if ri == 0 else [], never,
                                  pend.pop(gt, ()) if ri == 0 else ())
                    sc_.update(zip(its, outs))
                    for sr_, t_, j in its:
                        if sr_ == SPI - 1:
                            r_ = t_ * 64 + 8 * j
                            ka_s[pl.ds(r_, 8), :] = k_s[next_pair, pl.ds(r_, 8), :]
                tok = lh[-TD] if len(lh) >= TD else None
                if s_ >= 1:
                    un = s_ - 1 + SPI
                    ds_ = [c_, DH] if c_ == NC - 1 else [c_]
                    if c_ == 0:
                        stage_qf(clamp_h(h0 + un // NQ), un % NQ, s_ % 2)
                    make_qb(clamp_h(h0 + un // NQ), un % NQ, s_ - 1, ds_, tok, never[0], s_ % 2)
                for kj in kb_sched[(s_ % NQ) * NC + c_]:
                    val = make_kb(clamp_h(h + 1), kj, kb_make, tok, never[0])
                    if gt + KFD < SPI * NC:
                        pend.setdefault(gt + KFD, []).append(val)
                s_cur = jnp.concatenate([sc_.pop((s_, c_, j)) for j in range(8)], axis=0)
                l, acc = b_tile((s_ // NQ) % 2, c_, s_cur)
                if s_ % NQ == NQ - 1:
                    hv = clamp_h(h + 2)
                    va_s[pl.ds(((s_ // NQ) % 2) * 8, 8), pl.ds(c_ * CK, CK)] = (
                        vt_s[pl.ds(_mo(hv * 8, 8), 8), pl.ds(c_ * CK, CK)])
                lh.append(l)
            lsum = fin(h, qb, l, acc)
            lo = jnp.minimum(lo, lsum)
            hi = jnp.maximum(hi, lsum)
        sc_[(SPI, 1, VB)] = v_rows(1, kb0, 0)[0]
        for i_, (t_, j) in enumerate(car_items):
            car_s[pl.ds(16 * i_, 16), :] = sc_.pop((SPI, t_, j))
        un = 2 * SPI - 1
        make_qb(clamp_h(h0 + un // NQ), un % NQ, SPI - 1, range(DH + 1))
        return lo, hi

    for u_ in range(SPI):
        make_qb(u_ // NQ, u_ % NQ, u_, range(DH + 1))
    for j in range(2 * DH):
        make_kb(0, j, kb0)
    pro = qk_run(make_w(0, 0, 0, 0), car_mx, [], None) + [v_rows(0, kb0, 0)[0], v_rows(1, kb0, 0)[0]]
    for i_, o_ in enumerate(pro):
        car_s[pl.ds(16 * i_, 16), :] = o_

    def p2_body(i, state):
        return run_steps(i, state, (i < 0, i < -1, i < -2))

    one = jnp.ones((1, TQ), F32)
    lo, hi = jax.lax.fori_loop(0, T // SPI, p2_body, (one, one))

    for cp in late:
        cp.wait()

    ok = jnp.logical_and(lo >= L_MIN, hi <= L_MAX)
    n_bad = jnp.sum(jnp.where(ok, 0.0, 1.0))

    @pl.when(n_bad > 0.0)
    def _():
        def exact_step(t, carry):
            h = t // NQ
            c0 = pl.multiple_of((t % NQ) * TQ, TQ)
            r8 = pl.multiple_of(h * 8, 8)
            q = qt_s[pl.ds(r8, 8), pl.ds(c0, TQ)]
            zq = jnp.zeros_like(q)
            odd = h % 2 == 1
            w = _upk(jnp.concatenate([jnp.where(odd, zq, q), jnp.where(odd, q, zq)], axis=0))
            s0[...] = _dot(_upk(k_s[h // 2])[:, :2 * DH], w)
            st = s0[...]
            p = jnp.exp2(st - jnp.max(st, axis=0, keepdims=True))
            lsum = jnp.sum(p, axis=0, keepdims=True)
            o = _dot(_upk(vt_s[pl.ds(r8, 8), :]), p.astype(BF))
            ot_s[pl.ds(r8, 8), pl.ds(c0, TQ)] = _pk((o * (1.0 / lsum)).astype(BF))
            return carry

        s0[0:16, :] = acc_s[...]
        s0[16:24, :] = l_s[...]
        s0[32:80, :] = qf_s[...].reshape(48, TQ)
        s0[80:112, :] = pltpu.bitcast(w_s[...].reshape(32, TQ), F32)

        jax.lax.fori_loop(0, T, exact_step, 0)

    mod_v[:, 2 * D:] = _dot(sc, wmod_v[:, 2 * D:])[:8]

    def p3a(i):
        r0 = i * RB
        attn = _dot(_upk(ot_s[:, pl.ds(r0, RB)]).T, wo_v[...])
        x1 = x_v[pl.ds(r0, RB), :].astype(F32) + mod_row(2) * attn
        x1_s[pl.ds(r0, RB), :] = x1
        h2 = (_ln(x1) * (1.0 + mod_row(4)) + mod_row(3)).astype(BF)
        h2_s[pl.ds(r0 // 2, RB // 2), :] = _pk(h2)
        return h2

    def p3b(i, h2):
        z2 = _gelu(_dot(h2, win_v[:, FH:]))
        z2_s[pl.ds(i * RB // 2, RB // 2), :] = _pk(_ln(z2).astype(BF))

    h2s = [p3a(i) for i in range(NB)]
    for i in range(NB):
        p3b(i, h2s[i])
    z1s = {i: _dot(h2s[i], win_v[:, :FH]) for i in range(2)}

    def out_copy(j):
        r0, n = _OUT_BLOCKS[j]
        return pltpu.make_async_copy(out_v.at[pl.ds(r0, n), :],
                                     out_hbm.at[0, pl.ds(r0, n), :], osems.at[j])

    brow_all = bsp_v[...].reshape(1, S).astype(F32)
    for i in range(NB):
        r0 = i * RB
        z1 = _gelu(z1s[i] if i in z1s else _dot(h2s[i], win_v[:, :FH]))
        gsp = _dot(wsp_v[pl.ds(r0, RB), :], _upk(z2_s[...]))
        bcol = jnp.broadcast_to(brow_all[:, r0:r0 + RB], (128, RB)).T
        bfull = jnp.concatenate([bcol] * (FH // 128), axis=1)
        u = (z1 * (gsp + bfull)).astype(BF)
        for j, (o0, n) in enumerate(_OUT_BLOCKS):
            if r0 <= o0 < r0 + RB:
                y = _dot(u[o0 - r0:o0 - r0 + n], wout_v[...])
                out_v[pl.ds(o0, n), :] = (x1_s[pl.ds(o0, n), :] + mod_row(5) * y).astype(BF)
                out_copy(j).start()
    for j in range(len(_OUT_BLOCKS)):
        out_copy(j).wait()


@jax.jit
def pallas_adaLN_cond__softmax_full_mha__mixer_gmlp__prompt_kernel(
    A_x: jax.Array,
    A_wqkv: jax.Array,
    A_wo: jax.Array,
    B_x: jax.Array,
    B_w_in: jax.Array,
    B_w_sp: jax.Array,
    B_b_sp: jax.Array,
    B_w_out: jax.Array,
    c: jax.Array,
    w_mod: jax.Array,
):
    del B_x
    vm = pltpu.VMEM
    scratch = [
        vm((S, D), BF), vm((D, 3 * D), BF), vm((D, D), BF),
        vm((D, 2 * FH), BF), vm((S, S), BF), vm((FH, D), BF),
        vm((D, 6 * D), BF), vm((1, D), BF), vm((S,), BF),
        vm((8, 6 * D), F32),
        vm((H // 2, S // 2, 128), U32),
        vm((S // 2, 128), U32), vm((16, S), U32),
        vm((2, 16, TQ), U32), vm((2, 24, TQ), F32),
        vm((4, S // 2, 128), U32),
        vm((D // 2, S), U32), vm((D // 2, S), U32),
        vm((128, D), U32), vm((D // 2, 256), U32),
        vm((H, S), F32), vm((H, RB), F32),
        vm((DH, 256, 128), F32), vm((DH, 256, 128), F32),
        vm((SPI, DH + 1, 8, TQ), F32),
        vm((16, TQ), F32), vm((8, TQ), F32), vm((CK + 16 * SH + 16, TQ), F32),
        vm((S, TQ), F32), vm((D // 2, S), U32),
        vm((S, D), F32), vm((S // 2, D), U32), vm((S // 2, FH), U32),
        vm((RB, 3 * D), F32),
        vm((S, D), BF),
        pltpu.SemaphoreType.DMA((22,)),
        pltpu.SemaphoreType.DMA((len(_OUT_BLOCKS),)),
    ]
    any_spec = pl.BlockSpec(memory_space=pl.ANY)
    return pl.pallas_call(
        _kernel,
        out_shape=jax.ShapeDtypeStruct((1, S, D), BF),
        in_specs=[any_spec] * 9,
        out_specs=any_spec,
        scratch_shapes=scratch,
        compiler_params=pltpu.CompilerParams(vmem_limit_bytes=100 * 1024 * 1024, disable_semaphore_checks=True),
    )(A_x, A_wqkv, A_wo, B_w_in, B_w_sp, B_b_sp, B_w_out, c, w_mod)
```

```python
import jax
import jax.numpy as jnp
import jax.experimental.pallas as pl
import jax.experimental.pallas.tpu as pltpu

S = 2048
D = 512
H = 32
DH = 16
FH = 896
EPS = 1e-5
LOG2E = 1.4426950408889634
QSCALE = (DH ** -0.5) * LOG2E

TQ = 512
CK = 128
NC = S // CK
NQ = S // TQ
T = H * NQ
SPI = 2 * NQ
RB = 512
NB = S // RB
NJ = 4
JW = D // NJ
TAIL = (256, 128, 64, 32, 32)

VB = 0
NPG = 3
SH = 1
TD = 3
KFD = 6
KBE = 6
L_MIN = 2.0 ** -40
L_MAX = 2.0 ** 20

BF = jnp.bfloat16
F32 = jnp.float32
U32 = jnp.uint32


def _pk(x):
    return pltpu.bitcast(x, U32)


def _upk(x):
    return pltpu.bitcast(x, BF)


def _mo(x, n):
    return x if isinstance(x, int) else pl.multiple_of(x, n)


def _dot(a, b):
    return jnp.dot(a, b, preferred_element_type=F32)


def _ln(x):
    m = jnp.mean(x, axis=-1, keepdims=True)
    xc = x - m
    v = jnp.mean(xc * xc, axis=-1, keepdims=True)
    return xc * jax.lax.rsqrt(v + EPS)


def _gelu(x):
    c0 = 0.7978845608028654
    inner = x * (c0 + (c0 * 0.044715) * (x * x))
    hx = 0.5 * x
    return hx + hx * jnp.tanh(inner)


_OUT_BLOCKS = ([(i * RB, RB) for i in range(NB - 1)]
               + [(S - RB + sum(TAIL[:j]), n_) for j, n_ in enumerate(TAIL)])


def _kernel(x_hbm, wqkv_hbm, wo_hbm, win_hbm, wsp_hbm, bsp_hbm, wout_hbm, c_hbm, wmod_hbm,
            out_hbm,
            x_v, wqkv_v, wo_v, win_v, wsp_v, wout_v, wmod_v, c_v, bsp_v, mod_v,
            k_s, ka_s, va_s, w_s, qf_s, kr_s, qt_s, vt_s, ksel_s, kt_s, qn_s, kn_s, kb0, kb1,
            qb_s, acc_s, l_s, car_s, s0, ot_s, x1_s, h2_s, z2_s, q0_s, out_v, sems, osems):
    def cols(src, dst, c0, n, sem):
        return pltpu.make_async_copy(src.at[:, pl.ds(c0, n)], dst.at[:, pl.ds(c0, n)], sem)

    def xrows(r0, n, sem):
        return pltpu.make_async_copy(x_hbm.at[0, pl.ds(r0, n), :], x_v.at[pl.ds(r0, n), :], sem)

    cp_c = pltpu.make_async_copy(c_hbm, c_v, sems.at[0])
    cp_x0 = xrows(0, RB, sems.at[1])
    cp_ms = [cols(wmod_hbm, wmod_v, j * JW, JW, sems.at[14 + j]) for j in range(NJ)]
    cp_mc = [cols(wmod_hbm, wmod_v, D + j * JW, JW, sems.at[18 + j]) for j in range(NJ)]
    cp_w = [pltpu.make_async_copy(wqkv_hbm.at[pl.ds(j * JW, JW), :],
                                  wqkv_v.at[pl.ds(j * JW, JW), :], sems.at[2 + j])
            for j in range(NJ)]
    cp_x1 = xrows(RB, RB, sems.at[6])
    cp_x23 = xrows(2 * RB, 2 * RB, sems.at[7])
    late = [cols(wmod_hbm, wmod_v, 2 * D, 4 * D, sems.at[8]),
            pltpu.make_async_copy(wo_hbm, wo_v, sems.at[9]),
            pltpu.make_async_copy(win_hbm, win_v, sems.at[10]),
            pltpu.make_async_copy(wsp_hbm, wsp_v, sems.at[11]),
            pltpu.make_async_copy(wout_hbm, wout_v, sems.at[12]),
            pltpu.make_async_copy(bsp_hbm, bsp_v, sems.at[13])]
    order = [cp_c, cp_x0, cp_ms[0], cp_mc[0]]
    for j in range(NJ):
        if j + 1 < NJ:
            order += [cp_ms[j + 1], cp_mc[j + 1]]
        else:
            order.append(cp_x1)
        order.append(cp_w[j])
    for cp in order + [cp_x23] + late:
        cp.start()

    cp_c.wait()
    cp_x0.wait()
    c = c_v[...].astype(F32)
    sc = (c * jax.nn.sigmoid(c)).astype(BF)
    sc = jnp.broadcast_to(sc, (16, D))

    def norm1(i):
        return _ln(x_v[pl.ds(i * RB, RB), :].astype(F32))

    def mod_row(j):
        return mod_v[0:1, j * D:(j + 1) * D]

    def modulate1(n):
        return (n * (1.0 + mod_row(1)) + mod_row(0)).astype(BF)

    n0 = norm1(0)

    def h0_piece(j):
        for c0 in (j * JW, D + j * JW):
            mod_v[:, c0:c0 + JW] = _dot(sc, wmod_v[:, c0:c0 + JW])[:8]
        sa = mod_v[0:1, j * JW:(j + 1) * JW]
        ca = mod_v[0:1, D + j * JW:D + (j + 1) * JW]
        return (n0[:, j * JW:(j + 1) * JW] * (1.0 + ca) + sa).astype(BF)

    cp_ms[0].wait()
    cp_mc[0].wait()
    hj = h0_piece(0)
    qkv0 = None
    for j in range(NJ):
        if j + 1 < NJ:
            cp_ms[j + 1].wait()
            cp_mc[j + 1].wait()
        if j == NJ - 2:
            cp_x1.wait()
        cp_w[j].wait()
        part = _dot(hj, wqkv_v[j * JW:(j + 1) * JW, :])
        if j == 0:
            q0_s[...] = part
        elif j + 1 < NJ:
            q0_s[...] = q0_s[...] + part
        else:
            qkv0 = q0_s[...] + part
        if j + 1 < NJ:
            hj = h0_piece(j + 1)
        if j >= NJ - 2:
            hr = RB // 2
            half = j - (NJ - 2)
            h2_s[pl.ds(half * hr // 2, hr // 2), :] = _pk(
                modulate1(_ln(x_v[pl.ds(RB + half * hr, hr), :].astype(F32))))

    def head_sq(xt):
        xf = xt.astype(F32)
        return (xf * xf).reshape(H, DH, xt.shape[1]).sum(axis=1)

    def proj_k(i, h):
        k = qkv0[:, D:2 * D] if i == 0 else _dot(h, wqkv_v[:, D:2 * D])
        k = k.astype(BF)
        kp = _pk(k)
        for g in range(4):
            kr_s[g, pl.ds(i * RB // 2, RB // 2), :] = kp[:, g * 128:(g + 1) * 128]
        for t_ in range(RB // CK):
            ksel_s[pl.ds((i * (RB // CK) + t_) * 8, 8), :] = (
                kp[t_ * 64 + 8 * VB:t_ * 64 + 8 * VB + 8])
        kn = head_sq(k.T)
        kn_s[...] = kn if i == 0 else jnp.maximum(kn_s[...], kn)

    lane = jax.lax.broadcasted_iota(jnp.int32, (8, 128), 1)
    one_pk = _pk(jnp.where(jax.lax.broadcasted_iota(jnp.int32, (16, 128), 1) == 2 * DH,
                           1.0, 0.0).astype(BF))

    def rot_k(i):
        n8 = RB // 16
        keep = jnp.broadcast_to((lane < 2 * DH)[None], (n8, 8, 128))
        fill = jnp.broadcast_to(one_pk[None], (n8, 8, 128))
        for g in range(4):
            kg = kr_s[g, pl.ds(i * RB // 2, RB // 2), :]
            for j in range(4):
                kj = kg if j == 0 else pltpu.roll(kg, 128 - 32 * j, axis=1)
                kj = jnp.where(keep, kj.reshape(n8, 8, 128), fill).reshape(RB // 2, 128)
                k_s[4 * g + j, pl.ds(i * RB // 2, RB // 2), :] = kj
                if g == 0 and j == 0:
                    ka_s[pl.ds(i * RB // 2, RB // 2), :] = kj

    def proj_q(i, h):
        q = qkv0[:, :D] if i == 0 else _dot(h, wqkv_v[:, :D])
        qt = (q * QSCALE).astype(BF).T
        qt_s[:, pl.ds(i * RB, RB)] = _pk(qt)
        qn_s[:, pl.ds(i * RB, RB)] = head_sq(qt)

    def make_ref(i):
        kmax = jnp.max(kn_s[...], axis=1, keepdims=True)
        bound = jnp.sqrt(qn_s[:, pl.ds(i * RB, RB)] * kmax) * (1.0 + 2.0 ** -6)
        qn_s[:, pl.ds(i * RB, RB)] = (-bound).astype(BF).astype(F32)

    def proj_v(i, h):
        v = qkv0[:, 2 * D:] if i == 0 else _dot(h, wqkv_v[:, 2 * D:])
        vp = _pk(v.astype(BF).T)
        vt_s[:, pl.ds(i * RB, RB)] = vp
        va_s[:, pl.ds(i * RB, RB)] = vp[:16]

    cp_x23.wait()
    hs = {1: _upk(h2_s[pl.ds(0, RB // 2), :])}
    proj_k(0, None)
    rot_k(0)
    proj_q(0, None)
    proj_v(0, None)
    hs[2] = modulate1(norm1(2))
    proj_k(1, hs[1])
    rot_k(1)
    proj_q(1, hs[1])
    hs[3] = modulate1(norm1(3))
    proj_k(2, hs[2])
    rot_k(2)
    proj_q(2, hs[2])
    proj_v(1, hs[1])
    proj_k(3, hs[3])
    rot_k(3)
    kt_s[...] = _pk(_upk(ksel_s[...]).T)
    for i in range(NB - 1):
        make_ref(i)
    proj_q(3, hs[3])
    make_ref(3)
    proj_v(2, hs[2])
    proj_v(3, hs[3])

    def q_rows(h, qb):
        return qt_s[pl.ds(_mo(h * 8, 8), 8), qb * TQ:(qb + 1) * TQ]

    def nref_row(h, qb):
        return qn_s[pl.ds(h, 1), qb * TQ:(qb + 1) * TQ]

    def clamp_h(h):
        return min(h, H - 1) if isinstance(h, int) else jnp.minimum(h, H - 1)

    row0 = jax.lax.broadcasted_iota(jnp.int32, (16, TQ), 0) == 0

    def make_w(h, qb, par, slot, staged=False):
        if not staged:
            aug = jnp.where(row0, jnp.broadcast_to(nref_row(h, qb), (16, TQ)), 0.0).astype(BF)
            w_s[slot] = _pk(jnp.concatenate([_upk(q_rows(h, qb)), aug], axis=0))
        qa = _upk(w_s[slot])
        q, aug = qa[:DH], qa[DH:]
        z = jnp.zeros((DH, TQ), BF)
        return jnp.concatenate([z, q, aug] if par else [q, z, aug], axis=0)

    def stage_qf(h, qb, slot):
        qf_s[slot, 0:DH, :] = _upk(q_rows(h, qb)).astype(F32)
        qf_s[slot, DH:DH + 8, :] = jnp.broadcast_to(nref_row(h, qb), (8, TQ))

    def make_qb(h, qb, slot, ds_, tok=None, never=None, fslot=None):
        if fslot is None:
            qf = _upk(q_rows(h, qb)).astype(F32)
        for d in ds_:
            if fslot is not None:
                blk = qf_s[fslot, pl.ds(8 * (d // 8), 8), :]
                row = blk[d % 8:d % 8 + 1]
            else:
                row = nref_row(h, qb) if d == DH else qf[d:d + 1]
            val = jnp.broadcast_to(row, (8, TQ))
            if tok is not None:
                val = jnp.where(never, tok, val)
            qb_s[slot, d] = val

    def make_kb(h, j, kb, tok=None, never=None):
        d, half = j // 2, j % 2
        kt = _upk(kt_s[pl.ds(_mo(h * 8, 8), 8), half * 128:(half + 1) * 128]).astype(F32)
        row = jnp.broadcast_to(kt[d:d + 1], (8, 128))
        if tok is not None:
            row = jnp.where(never, tok[:, :128], row)
        val = jnp.concatenate([row] * 16, axis=0).T
        kb[d, pl.ds(half * 128, 128), :] = val
        return val[120:]

    def fence(val, on, never):
        return jnp.where(never, pltpu.bitcast(val, U32), on)

    def v_unit(tile, ui, kb, slot):
        c0 = ui * 256
        acc = None
        toks = []
        for d in range(DH):
            kk = kb[d, pl.ds(16 * tile, 16), :]
            kk = jnp.concatenate([kk] * 2, axis=1).reshape(2, 8, 256)
            t_ = kk * qb_s[slot, d, :, c0:c0 + 256][None]
            acc = t_ + qb_s[slot, DH, :, c0:c0 + 256][None] if acc is None else acc + t_
            if ((d + 1) * NPG) // DH != (d * NPG) // DH:
                ts = [acc[a_, :, b_ * 128:(b_ + 1) * 128] for a_ in range(2) for b_ in range(2)]
                toks.append((ts[0] + ts[1]) + (ts[2] + ts[3]) if d == DH - 1 else ts[0] + ts[3])
        return acc.reshape(16, 256), toks

    def v_rows(tile, kb, slot):
        us = [v_unit(tile, ui, kb, slot) for ui in range(2)]
        return jnp.concatenate([us[0][0], us[1][0]], axis=1), us[0][1] + us[1][1]

    mx_blocks = [j for j in reversed(range(8)) if j != VB]

    def qk_run(w, items, toks, never, extra=()):
        parts = [ka_s[pl.ds(t_ * 64 + 8 * j, 8), :] for t_, j in items]
        for i_, tk in enumerate(toks):
            j = (i_ * len(parts)) // len(toks)
            parts[j] = fence(tk, parts[j], never[i_ % 2])
        if extra:
            val = extra[0]
            for v_ in extra[1:]:
                val = val + v_
            parts[0] = fence(val, parts[0], never[2])
        st = _dot(_upk(jnp.concatenate(parts, axis=0))[:, :3 * DH], w)
        return [st[16 * i_:16 * i_ + 16] for i_ in range(len(items))]

    def b_tile(hoff, ck, s):
        p = jnp.exp2(s)
        l = None if ck == 0 else l_s[...]
        for j in reversed(range(CK // 16)):
            pr = p[16 * j:16 * j + 8] + p[16 * j + 8:16 * j + 16]
            l = pr if l is None else l + pr
        l_s[...] = l
        vc = _upk(va_s[pl.ds(hoff * 8, 8), pl.ds(ck * CK, CK)])
        pv = _dot(vc, p.astype(BF))
        acc = pv if ck == 0 else acc_s[...] + pv
        acc_s[...] = acc
        return l, acc

    def fin(h, qb, l, acc):
        lsum = l.sum(axis=0, keepdims=True)
        o = acc * (1.0 / lsum)
        ot_s[pl.ds(_mo(h * 8, 8), 8), qb * TQ:(qb + 1) * TQ] = _pk(o.astype(BF))
        return lsum

    kbs = (kb0, kb1)
    kb_sched = [[] for _ in range(NQ * NC)]
    for kj in range(2 * DH):
        kb_sched[(kj * (NQ * NC - KBE)) // (2 * DH)].append(kj)

    car_mx = [(0, j) for j in mx_blocks] + [(1, j) for j in mx_blocks[:SH]]
    car_items = car_mx + [(0, VB), (1, VB)]

    def run_steps(pair, bad, never):
        h0 = 2 * pair
        pend = {}
        lh = []
        sc_ = {}
        for i_, (t_, j) in enumerate(car_items):
            sc_[(0, t_, j)] = car_s[pl.ds(16 * i_, 16), :]
        ws = {}
        next_pair = jnp.minimum(pair + 1, H // 2 - 1)

        def step_hq(s_):
            return clamp_h(h0 + s_ // NQ) if s_ >= SPI else h0 + s_ // NQ, s_ % NQ

        def get_w(s_):
            if s_ not in ws:
                ws[s_] = make_w(*step_hq(s_), (s_ // NQ) % 2, s_ % 2, staged=(s_ == 0))
            return ws[s_]

        for s_ in range(SPI):
            h, qb = step_hq(s_)
            kb_make = kbs[1 - (s_ // NQ) % 2]
            for c_ in range(NC):
                gt = s_ * NC + c_
                g1, g2 = gt + 1, gt + 2
                it1 = [(g1 // NC, g1 % NC, j) for j in mx_blocks[SH:]]
                it2 = [(g2 // NC, g2 % NC, j) for j in mx_blocks[:SH]]
                s1 = g1 // NC
                if gt == 0:
                    toks = []
                else:
                    sc_[(s1, g1 % NC, VB)], toks = v_rows(g1 % NC, kbs[(s1 // NQ) % 2], s1 % SPI)
                runs = [it1 + it2] if g1 // NC == g2 // NC else [it1, it2]
                for ri, its in enumerate(runs):
                    outs = qk_run(get_w(its[0][0]), [(t_, j) for _, t_, j in its],
                                  toks if ri == 0 else [], never,
                                  pend.pop(gt, ()) if ri == 0 else ())
                    sc_.update(zip(its, outs))
                    for sr_, t_, j in its:
                        if sr_ == SPI - 1:
                            r_ = t_ * 64 + 8 * j
                            ka_s[pl.ds(r_, 8), :] = k_s[next_pair, pl.ds(r_, 8), :]
                tok = lh[-TD] if len(lh) >= TD else None
                if s_ >= 1:
                    un = s_ - 1 + SPI
                    ds_ = [c_, DH] if c_ == NC - 1 else [c_]
                    if c_ == 0:
                        stage_qf(clamp_h(h0 + un // NQ), un % NQ, s_ % 2)
                    make_qb(clamp_h(h0 + un // NQ), un % NQ, s_ - 1, ds_, tok, never[0], s_ % 2)
                for kj in kb_sched[(s_ % NQ) * NC + c_]:
                    val = make_kb(clamp_h(h + 1), kj, kb_make, tok, never[0])
                    if gt + KFD < SPI * NC:
                        pend.setdefault(gt + KFD, []).append(val)
                s_cur = jnp.concatenate([sc_.pop((s_, c_, j)) for j in range(8)], axis=0)
                l, acc = b_tile((s_ // NQ) % 2, c_, s_cur)
                if s_ % NQ == NQ - 1:
                    hv = clamp_h(h + 2)
                    va_s[pl.ds(((s_ // NQ) % 2) * 8, 8), pl.ds(c_ * CK, CK)] = (
                        vt_s[pl.ds(_mo(hv * 8, 8), 8), pl.ds(c_ * CK, CK)])
                lh.append(l)
            lsum = fin(h, qb, l, acc)
            ok = jnp.logical_and(lsum >= L_MIN, lsum <= L_MAX)
            bad = jnp.where(ok, bad, 1.0)
        sc_[(SPI, 1, VB)] = v_rows(1, kb0, 0)[0]
        for i_, (t_, j) in enumerate(car_items):
            car_s[pl.ds(16 * i_, 16), :] = sc_.pop((SPI, t_, j))
        un = 2 * SPI - 1
        make_qb(clamp_h(h0 + un // NQ), un % NQ, SPI - 1, range(DH + 1))
        return bad

    for u_ in range(SPI):
        make_qb(u_ // NQ, u_ % NQ, u_, range(DH + 1))
    for j in range(2 * DH):
        make_kb(0, j, kb0)
    pro = qk_run(make_w(0, 0, 0, 0), car_mx, [], None) + [v_rows(0, kb0, 0)[0], v_rows(1, kb0, 0)[0]]
    for i_, o_ in enumerate(pro):
        car_s[pl.ds(16 * i_, 16), :] = o_

    def p2_body(i, bad):
        return run_steps(i, bad, (i < 0, i < -1, i < -2))

    bad = jax.lax.fori_loop(0, T // SPI, p2_body, jnp.zeros((1, TQ), F32))

    for cp in late:
        cp.wait()

    @pl.when(jnp.sum(bad) > 0.0)
    def _():
        def exact_step(t, carry):
            h = t // NQ
            c0 = pl.multiple_of((t % NQ) * TQ, TQ)
            r8 = pl.multiple_of(h * 8, 8)
            q = qt_s[pl.ds(r8, 8), pl.ds(c0, TQ)]
            zq = jnp.zeros_like(q)
            odd = h % 2 == 1
            w = _upk(jnp.concatenate([jnp.where(odd, zq, q), jnp.where(odd, q, zq)], axis=0))
            s0[...] = _dot(_upk(k_s[h // 2])[:, :2 * DH], w)
            st = s0[...]
            p = jnp.exp2(st - jnp.max(st, axis=0, keepdims=True))
            lsum = jnp.sum(p, axis=0, keepdims=True)
            o = _dot(_upk(vt_s[pl.ds(r8, 8), :]), p.astype(BF))
            ot_s[pl.ds(r8, 8), pl.ds(c0, TQ)] = _pk((o * (1.0 / lsum)).astype(BF))
            return carry

        s0[0:16, :] = acc_s[...]
        s0[16:24, :] = l_s[...]
        s0[32:80, :] = qf_s[...].reshape(48, TQ)
        s0[80:112, :] = pltpu.bitcast(w_s[...].reshape(32, TQ), F32)

        jax.lax.fori_loop(0, T, exact_step, 0)

    mod_v[:, 2 * D:] = _dot(sc, wmod_v[:, 2 * D:])[:8]

    def p3a(i):
        r0 = i * RB
        attn = _dot(_upk(ot_s[:, pl.ds(r0, RB)]).T, wo_v[...])
        x1 = x_v[pl.ds(r0, RB), :].astype(F32) + mod_row(2) * attn
        x1_s[pl.ds(r0, RB), :] = x1
        h2 = (_ln(x1) * (1.0 + mod_row(4)) + mod_row(3)).astype(BF)
        h2_s[pl.ds(r0 // 2, RB // 2), :] = _pk(h2)
        return h2

    def p3b(i, h2):
        z2 = _gelu(_dot(h2, win_v[:, FH:]))
        z2_s[pl.ds(i * RB // 2, RB // 2), :] = _pk(_ln(z2).astype(BF))

    h2s = [p3a(i) for i in range(NB)]
    for i in range(NB):
        p3b(i, h2s[i])
    z1s = {i: _dot(h2s[i], win_v[:, :FH]) for i in range(2)}

    def out_copy(j):
        r0, n = _OUT_BLOCKS[j]
        return pltpu.make_async_copy(out_v.at[pl.ds(r0, n), :],
                                     out_hbm.at[0, pl.ds(r0, n), :], osems.at[j])

    brow_all = bsp_v[...].reshape(1, S).astype(F32)
    for i in range(NB):
        r0 = i * RB
        z1 = _gelu(z1s[i] if i in z1s else _dot(h2s[i], win_v[:, :FH]))
        gsp = _dot(wsp_v[pl.ds(r0, RB), :], _upk(z2_s[...]))
        bcol = jnp.broadcast_to(brow_all[:, r0:r0 + RB], (128, RB)).T
        bfull = jnp.concatenate([bcol] * (FH // 128), axis=1)
        u = (z1 * (gsp + bfull)).astype(BF)
        for j, (o0, n) in enumerate(_OUT_BLOCKS):
            if r0 <= o0 < r0 + RB:
                y = _dot(u[o0 - r0:o0 - r0 + n], wout_v[...])
                out_v[pl.ds(o0, n), :] = (x1_s[pl.ds(o0, n), :] + mod_row(5) * y).astype(BF)
                out_copy(j).start()
    for j in range(len(_OUT_BLOCKS)):
        out_copy(j).wait()


@jax.jit
def pallas_adaLN_cond__softmax_full_mha__mixer_gmlp__prompt_kernel(
    A_x: jax.Array,
    A_wqkv: jax.Array,
    A_wo: jax.Array,
    B_x: jax.Array,
    B_w_in: jax.Array,
    B_w_sp: jax.Array,
    B_b_sp: jax.Array,
    B_w_out: jax.Array,
    c: jax.Array,
    w_mod: jax.Array,
):
    del B_x
    vm = pltpu.VMEM
    scratch = [
        vm((S, D), BF), vm((D, 3 * D), BF), vm((D, D), BF),
        vm((D, 2 * FH), BF), vm((S, S), BF), vm((FH, D), BF),
        vm((D, 6 * D), BF), vm((1, D), BF), vm((S,), BF),
        vm((8, 6 * D), F32),
        vm((H // 2, S // 2, 128), U32),
        vm((S // 2, 128), U32), vm((16, S), U32),
        vm((2, 16, TQ), U32), vm((2, 24, TQ), F32),
        vm((4, S // 2, 128), U32),
        vm((D // 2, S), U32), vm((D // 2, S), U32),
        vm((128, D), U32), vm((D // 2, 256), U32),
        vm((H, S), F32), vm((H, RB), F32),
        vm((DH, 256, 128), F32), vm((DH, 256, 128), F32),
        vm((SPI, DH + 1, 8, TQ), F32),
        vm((16, TQ), F32), vm((8, TQ), F32), vm((CK + 16 * SH + 16, TQ), F32),
        vm((S, TQ), F32), vm((D // 2, S), U32),
        vm((S, D), F32), vm((S // 2, D), U32), vm((S // 2, FH), U32),
        vm((RB, 3 * D), F32),
        vm((S, D), BF),
        pltpu.SemaphoreType.DMA((22,)),
        pltpu.SemaphoreType.DMA((len(_OUT_BLOCKS),)),
    ]
    any_spec = pl.BlockSpec(memory_space=pl.ANY)
    return pl.pallas_call(
        _kernel,
        out_shape=jax.ShapeDtypeStruct((1, S, D), BF),
        in_specs=[any_spec] * 9,
        out_specs=any_spec,
        scratch_shapes=scratch,
        compiler_params=pltpu.CompilerParams(vmem_limit_bytes=100 * 1024 * 1024,
                                             disable_semaphore_checks=True),
    )(A_x, A_wqkv, A_wo, B_w_in, B_w_sp, B_b_sp, B_w_out, c, w_mod)
```
